```python
import jax
import jax.numpy as jnp

def _softmax(x, axis=-1):
    return jax.nn.softmax(x, axis=axis)
def _gelu(x):
    return jax.nn.gelu(x, approximate=True)
def _silu(x):
    return jax.nn.silu(x)
def _sigmoid(x):
    return jax.nn.sigmoid(x)
def _layernorm(x, axis=-1, eps=1e-5):
    m = jnp.mean(x, axis=axis, keepdims=True)
    v = jnp.var(x, axis=axis, keepdims=True)
    return (x - m) / jnp.sqrt(v + eps)
def _scatter_add(tgt, idx, src, axis=0):
    return tgt.at[idx].add(src)
def _segment_sum(src, seg, n):
    return jax.ops.segment_sum(src, seg, n)
class _Rng:
    def __init__(self, key):
        self._k = key
    def _next(self):
        self._k, sub = jax.random.split(self._k)
        return sub
    def normal(self, shape):
        return jax.random.normal(self._next(), shape, dtype=jnp.bfloat16)
    def randint(self, lo, hi, shape):
        return jax.random.randint(self._next(), shape, lo, hi, dtype=jnp.int32)
    def uniform(self, shape, lo=0.0, hi=1.0):
        return jax.random.uniform(self._next(), shape, jnp.bfloat16, lo, hi)
    def permutation(self, n):
        return jax.random.permutation(self._next(), n)


kernel_name = 'gated_mix__sliding_local_dilated__compressed_kv_cla__prompt'

def setup_inputs():
    _rng = _Rng(jax.random.key(int.from_bytes(__import__("os").urandom(4), "little")))
    _w = (lambda a: (lambda t: t.astype(jnp.bfloat16) if jnp.issubdtype(t.dtype, jnp.floating) else t)(jnp.asarray(a)))
    def _A_setup():
        B, S, D = 1, 2048, 576
        return {
            "x": _w((lambda *s: _rng.normal(s) * 0.05)(B, S, D)),
            "wqkv": _w((lambda *s: _rng.normal(s) * 0.05)(D, 3 * D)),
            "wo": _w((lambda *s: _rng.normal(s) * 0.05)(D, D)),
        }
    _A_in = _A_setup()

    def _B_setup():
        B, H, Sq, Sk, D, M = 1, 32, 2048, 2048, 128, 576
        Dc = 4 * D
        return {
            "x": _w((lambda *s: _rng.normal(s) * 0.05)(B, Sq, M)),
            "c_kv": _w((lambda *s: _rng.normal(s) * 0.05)(B, Sk, Dc)),
            "w_q": _w((lambda *s: _rng.normal(s) * 0.05)(M, H, D) * (M ** -0.5)),
            "w_uk": _w((lambda *s: _rng.normal(s) * 0.05)(Dc, H, D) * (Dc ** -0.5)),
            "w_uv": _w((lambda *s: _rng.normal(s) * 0.05)(Dc, H, D) * (Dc ** -0.5)),
            "w_o": _w((lambda *s: _rng.normal(s) * 0.05)(H, D, M) * ((H * D) ** -0.5)),
        }
    _B_in = _B_setup()

    return {
        "A_x": _A_in["x"],
        "A_wqkv": _A_in["wqkv"],
        "A_wo": _A_in["wo"],
        "B_x": _B_in["x"],
        "B_c_kv": _B_in["c_kv"],
        "B_w_q": _B_in["w_q"],
        "B_w_uk": _B_in["w_uk"],
        "B_w_uv": _B_in["w_uv"],
        "B_w_o": _B_in["w_o"],
        "gate_w": _w((lambda *s: _rng.normal(s) * 0.05)(576)),
    }

def reference(A_x, A_wqkv, A_wo, B_x, B_c_kv, B_w_q, B_w_uk, B_w_uv, B_w_o, gate_w):
    def _A_ref(x, wqkv, wo):
        B, S, D = x.shape
        H = 32; Dh = D // H
        W, dil = 8, 2
        qkv = (lambda x, *d: x.transpose(*d))((x @ wqkv).reshape(B, S, 3, H, Dh), 2, 0, 3, 1, 4)
        q, k, v = qkv[0], qkv[1], qkv[2]
        scale = Dh ** -0.5
        pos = jnp.arange(S)
        off = jnp.arange(W) * dil
        idx = pos[:, None] - off[None, :]
        mask = idx >= 0
        idx_c = jnp.where(mask, idx, 0).reshape(-1)
        kg = k[:, :, idx_c, :].reshape(B, H, S, W, Dh)
        vg = v[:, :, idx_c, :].reshape(B, H, S, W, Dh)
        logits = jnp.einsum("bhsd,bhswd->bhsw", q, kg) * scale
        logits = jnp.where(mask[None, None, :, :], logits, -1e9)
        attn = _softmax(logits, axis=-1)
        o = jnp.einsum("bhsw,bhswd->bhsd", attn, vg)
        return (lambda x, *d: x.transpose(*d))(o, 0, 2, 1, 3).reshape(B, S, D) @ wo

    def _B_ref(x, c_kv, w_q, w_uk, w_uv, w_o):
        B, Sq, M = x.shape[0], x.shape[1], x.shape[2]
        Sk = c_kv.shape[1]
        H, D = w_q.shape[1], w_q.shape[2]
        q = jnp.einsum("bqm,mhd->bhqd", x, w_q)
        k = jnp.einsum("bkc,chd->bhkd", c_kv, w_uk)
        v = jnp.einsum("bkc,chd->bhkd", c_kv, w_uv)
        scores = jnp.einsum("bhqd,bhkd->bhqk", q, k) * (D ** -0.5)
        off = Sk - Sq
        qi = jnp.arange(Sq)[:, None]
        kj = jnp.arange(Sk)[None, :]
        cmask = kj <= (qi + off)
        scores = jnp.where(cmask[None, None], scores, -1e9)
        p = _softmax(scores, axis=-1)
        ctx = jnp.einsum("bhqk,bhkd->bhqd", p, v)
        return jnp.einsum("bhqd,hdm->bqm", ctx, w_o)

    x = A_x
    g = _sigmoid((x * gate_w).sum(-1, keepdims=True))
    a = _A_ref(x, A_wqkv, A_wo)
    b = _B_ref(x, B_c_kv, B_w_q, B_w_uk, B_w_uv, B_w_o)
    return g * a + (1 - g) * b
```

```python
import functools
import math

import jax
import jax.numpy as jnp
import jax.experimental.pallas as pl
import jax.experimental.pallas.tpu as pltpu

F32 = jnp.float32
BF16 = jnp.bfloat16

S = 2048
M = 576
MP = 640
NT_M = MP // 128
H = 32
D = 128
DC = 512
DHA = 18
WIN = 8
DIL = 2
HALO = 16
LOG2E = math.log2(math.e)
NEG = -1e9

RA = 256
HG = 8
NG = H // HG
RP = 1024
TQ = 256
TB = 128
HU = 2
RO = 512

NN = (((1,), (0,)), ((), ()))
NT = (((1,), (1,)), ((), ()))


def _dot(a, b, dims=NN):
    return jax.lax.dot_general(a, b, dims, preferred_element_type=F32)


def _lane_partial(s, op):
    acc = s[:, 0:128]
    for j in range(1, s.shape[1] // 128):
        acc = op(acc, s[:, j * 128:(j + 1) * 128])
    return acc


def _segments(r0):
    nsub = TQ // TB
    segs = []
    if r0 > 0:
        segs.append((0, TQ, 0, r0, False))
    for j in range(nsub):
        segs.append((j * TB, (j + 1) * TB, r0 + j * TB, r0 + (j + 1) * TB, True))
        if (j + 1) * TB < TQ:
            segs.append(((j + 1) * TB, TQ, r0 + j * TB, r0 + (j + 1) * TB, False))
    return segs


def _attn_scores(q_ref, k_ref, r0, tri):
    nsub = TQ // TB
    segs = _segments(r0)
    ss = []
    for (a, b, c, d, msk) in segs:
        s = _dot(q_ref[r0 + a:r0 + b, :], k_ref[c:d, :], NT)
        if msk:
            s = jnp.where(tri, s, NEG * LOG2E)
        ss.append(s)
    ms = []
    for i in range(nsub):
        m = None
        for (a, b, c, d, msk), s in zip(segs, ss):
            if a <= i * TB and (i + 1) * TB <= b:
                sm = _lane_partial(s[i * TB - a:(i + 1) * TB - a], jnp.maximum)
                m = sm if m is None else jnp.maximum(m, sm)
        ms.append(jnp.max(m, axis=1, keepdims=True))
    return ss, ms


def _attn_values(v_ref, omg_ref, r0, ss, ms):
    nsub = TQ // TB
    segs = _segments(r0)
    ls = [None] * nsub
    os_ = [None] * nsub
    for (a, b, c, d, msk), s in zip(segs, ss):
        m = jnp.concatenate(ms[a // TB:b // TB], axis=0) if b - a > TB else ms[a // TB]
        p = jnp.exp2(s - m)
        l = _lane_partial(p, jnp.add)
        o = _dot(p.astype(BF16), v_ref[c:d, :])
        for i in range(a // TB, b // TB):
            li = l[i * TB - a:(i + 1) * TB - a]
            oi = o[i * TB - a:(i + 1) * TB - a]
            ls[i] = li if ls[i] is None else ls[i] + li
            os_[i] = oi if os_[i] is None else os_[i] + oi
    outs = []
    for i, (o, l) in enumerate(zip(os_, ls)):
        l = jnp.sum(l, axis=1, keepdims=True)
        r = pl.reciprocal(l, approx=True)
        r = r * (2.0 - l * r)
        omg = omg_ref[r0 + i * TB:r0 + (i + 1) * TB, :]
        outs.append(o * (omg * r))
    return outs


def _kernel(x_hbm, wqkv_hbm, woa_hbm, c_hbm, wq_hbm, wuk_hbm, wuv_hbm, wob_hbm, gate_ref,
            out_hbm,
            x_s, wqkv_s, woa_s, c_s, wq_raw, wuk_raw, wuv_raw, wob_s,
            wt_s, wpt_s, wof_s, woap_s, kl_s, vl_s, acc_s, omg_s,
            wq_s, wkv_s, q_s, k_s, v_s, ctx_s, out_s, sems, osems):
    copies = {
        "wqkv": pltpu.make_async_copy(wqkv_hbm, wqkv_s.at[pl.ds(0, M)], sems.at[0]),
        "x": pltpu.make_async_copy(x_hbm, x_s, sems.at[1]),
        "woa": pltpu.make_async_copy(woa_hbm, woa_s, sems.at[2]),
        "wq": pltpu.make_async_copy(wq_hbm, wq_raw, sems.at[3]),
        "wuk": pltpu.make_async_copy(wuk_hbm, wuk_raw, sems.at[4]),
        "wuv": pltpu.make_async_copy(wuv_hbm, wuv_raw, sems.at[5]),
        "c": pltpu.make_async_copy(c_hbm, c_s, sems.at[6]),
        "wob": pltpu.make_async_copy(wob_hbm, wob_s, sems.at[7]),
    }
    for cp in copies.values():
        cp.start()

    wqkv_s[M:MP, :] = jnp.zeros((MP - M, 3 * M), BF16)
    zero_halo = jnp.zeros((HALO, 128), F32)
    for j in range(NT_M):
        kl_s[j, 0:HALO, :] = zero_halo
        vl_s[j, 0:HALO, :] = zero_halo
    eye = (jax.lax.broadcasted_iota(jnp.int32, (128, 128), 0)
           == jax.lax.broadcasted_iota(jnp.int32, (128, 128), 1)).astype(BF16)

    copies["wqkv"].wait()
    ncol = 3 * M
    for t in range(pl.cdiv(ncol, 128)):
        c0 = t * 128
        wd = min(128, ncol - c0)
        wt = _dot(eye[0:wd, 0:wd], wqkv_s[:, c0:c0 + wd], NT)
        for j in range(NT_M):
            wt_s[j, c0:c0 + wd, :] = wt[:, j * 128:(j + 1) * 128]
    for sec in range(3):
        for d in range(DHA):
            for j in range(NT_M):
                rows = wt_s[j, pl.ds(sec * M + d, H, stride=DHA), :]
                wj = min(128, M - j * 128)
                wpt_s[sec, d * H:(d + 1) * H, j * 128:j * 128 + wj] = rows[:, 0:wj].astype(BF16)
    wpt_s[0, M:MP, :] = jnp.broadcast_to(gate_ref[...].reshape(1, M), (MP - M, M))
    wpt_s[1, M:MP, :] = jnp.zeros((MP - M, M), BF16)
    wpt_s[2, M:MP, :] = jnp.zeros((MP - M, M), BF16)

    copies["woa"].wait()
    woa = woa_s[...].astype(F32)
    for j in range(NT_M):
        wj = min(128, M - j * 128)
        blk = woa[:, j * 128:j * 128 + wj]
        if wj < 128:
            blk = jnp.concatenate([blk, jnp.zeros((M, 128 - wj), F32)], axis=1)
        wof_s[j] = blk
    for d in range(DHA):
        for j in range(NT_M):
            wj = min(128, M - j * 128)
            rows = wof_s[j, pl.ds(d, H, stride=DHA), :]
            woap_s[d * H:(d + 1) * H, j * 128:j * 128 + wj] = rows[:, 0:wj].astype(BF16)
    woap_s[M:MP, :] = jnp.zeros((MP - M, M), BF16)

    copies["x"].wait()

    lane = jax.lax.broadcasted_iota(jnp.int32, (RA, 128), 1)
    rowi = jax.lax.broadcasted_iota(jnp.int32, (RA, 128), 0)
    a_scale = (DHA ** -0.5) * LOG2E

    def a_proj(c):
        r0 = c * RA
        xq = x_s[r0:r0 + RA, :]
        q = _dot(xq, wpt_s[0], NT)
        k = _dot(xq, wpt_s[1], NT)
        v = _dot(xq, wpt_s[2], NT)
        for j in range(NT_M):
            kl_s[j, HALO + r0:HALO + r0 + RA, :] = k[:, j * 128:(j + 1) * 128]
            vl_s[j, HALO + r0:HALO + r0 + RA, :] = v[:, j * 128:(j + 1) * 128]
        gl = q[:, (NT_M - 1) * 128:]
        gl = jnp.where(lane >= 64, gl, pltpu.roll(gl, 64, 1))
        g = jax.nn.sigmoid(gl)
        omg_s[r0:r0 + RA, :] = 1.0 - g
        qt = [q[:, j * 128:(j + 1) * 128] * a_scale for j in range(NT_M)]
        return qt, g

    def a_local(c, qt):
        r0 = c * RA
        logits = []
        for w in range(WIN):
            off = HALO + r0 - w * DIL
            s = None
            for j in range(NT_M):
                t = qt[j] * kl_s[j, off:off + RA, :]
                s = t if s is None else s + t
            s = s + pltpu.roll(s, 64, 1)
            s = s + pltpu.roll(s, 32, 1)
            if r0 < w * DIL:
                s = jnp.where(rowi + r0 >= w * DIL, s, NEG * LOG2E)
            logits.append(s)
        m = functools.reduce(jnp.maximum, logits)
        ps = [jnp.exp2(s - m) for s in logits]
        l = functools.reduce(jnp.add, ps)
        r = pl.reciprocal(l, approx=True)
        r = r * (2.0 - l * r)
        ot = []
        for j in range(NT_M):
            o = None
            for w in range(WIN):
                off = HALO + r0 - w * DIL
                t = ps[w] * vl_s[j, off:off + RA, :]
                o = t if o is None else o + t
            ot.append((o * r).astype(BF16))
        return jnp.concatenate(ot, axis=1)

    def a_out(c, o, g):
        r0 = c * RA
        a = _dot(o, woap_s[...])
        gw = jnp.concatenate([g] * NT_M, axis=1)[:, 0:M]
        acc_s[r0:r0 + RA, :] = a * gw

    nca = S // RA
    st = {}
    for t in range(nca + 2):
        if t < nca:
            st[t] = a_proj(t)
        if 0 <= t - 1 < nca:
            qt, g = st[t - 1]
            st[t - 1] = (a_local(t - 1, qt), g)
        if 0 <= t - 2 < nca:
            o, g = st.pop(t - 2)
            a_out(t - 2, o, g)

    def relayout(raw, nrow, dst, col_base, per_group):
        w32 = raw.bitcast(jnp.uint32)
        for pr in range(H // 2):
            u = w32[pl.ds(pr, nrow, stride=H // 2), :]
            lo = pltpu.bitcast(u << 16, F32).astype(BF16)
            hi = pltpu.bitcast(u & jnp.uint32(0xFFFF0000), F32).astype(BF16)
            for h, val in ((2 * pr, lo), (2 * pr + 1, hi)):
                g, i = divmod(h, HG)
                c0 = col_base + i * D
                dst[g, :, c0:c0 + D] = val

    copies["wq"].wait()
    relayout(wq_raw, M, wq_s, 0, HG)
    copies["wuk"].wait()
    relayout(wuk_raw, DC, wkv_s, 0, HG)
    copies["wuv"].wait()
    relayout(wuv_raw, DC, wkv_s, HG * D, HG)
    copies["c"].wait()

    b_scale = (D ** -0.5) * LOG2E
    row = jax.lax.broadcasted_iota(jnp.int32, (TB, TB), 0)
    col = jax.lax.broadcasted_iota(jnp.int32, (TB, TB), 1)
    tri = col <= row

    def group_body(g, carry):
        def proj_body(rc, c2):
            r0 = pl.multiple_of(rc * RP, RP)
            q = _dot(x_s[pl.ds(r0, RP), :], wq_s[g]) * b_scale
            kv = _dot(c_s[pl.ds(r0, RP), :], wkv_s[g])
            for i in range(HG):
                q_s[i, pl.ds(r0, RP), :] = q[:, i * D:(i + 1) * D].astype(BF16)
                k_s[i, pl.ds(r0, RP), :] = kv[:, i * D:(i + 1) * D].astype(BF16)
                v_s[i, pl.ds(r0, RP), :] = kv[:, (HG + i) * D:(HG + i + 1) * D].astype(BF16)
            return c2

        jax.lax.fori_loop(0, S // RP, proj_body, 0)

        def attn_body(it, c2):
            items = [(u, r) for u in range(HU) for r in range(S // TQ)[::-1]]
            pend = {}
            for t in range(len(items) + 1):
                if t < len(items):
                    u, r = items[t]
                    hh = it * HU + u
                    pend[items[t]] = _attn_scores(q_s.at[hh], k_s.at[hh], r * TQ, tri)
                if t >= 1:
                    u, r = items[t - 1]
                    hh = it * HU + u
                    r0 = r * TQ
                    outs = _attn_values(v_s.at[hh], omg_s, r0, *pend.pop(items[t - 1]))
                    for j, o in enumerate(outs):
                        ctx_s[g * HG + hh, r0 + j * TB:r0 + (j + 1) * TB, :] = o.astype(BF16)
            return c2

        jax.lax.fori_loop(0, HG // HU, attn_body, 0)
        return carry

    jax.lax.fori_loop(0, NG, group_body, 0)

    copies["wob"].wait()

    def out_copy(i):
        r0 = i * RO
        if not isinstance(i, int):
            r0 = pl.multiple_of(r0, RO)
        return pltpu.make_async_copy(out_s.at[pl.ds(r0, RO)], out_hbm.at[0, pl.ds(r0, RO)], osems.at[i])

    def out_body(i, carry):
        r0 = pl.multiple_of(i * RO, RO)
        lhs = jnp.concatenate([ctx_s[h, pl.ds(r0, RO), :] for h in range(H)], axis=1)
        b = _dot(lhs, wob_s[...])
        out_s[pl.ds(r0, RO), :] = (acc_s[pl.ds(r0, RO), :] + b).astype(BF16)
        out_copy(i).start()
        return carry

    jax.lax.fori_loop(0, S // RO, out_body, 0)
    for i in range(S // RO):
        out_copy(i).wait()


@jax.jit
def pallas_gated_mix__sliding_local_dilated__compressed_kv_cla__prompt_kernel(
    A_x: jax.Array,
    A_wqkv: jax.Array,
    A_wo: jax.Array,
    B_x: jax.Array,
    B_c_kv: jax.Array,
    B_w_q: jax.Array,
    B_w_uk: jax.Array,
    B_w_uv: jax.Array,
    B_w_o: jax.Array,
    gate_w: jax.Array,
):
    del B_x
    x = A_x.reshape(S, M)
    c = B_c_kv.reshape(S, DC)
    wq = B_w_q.reshape(M * H, D)
    wuk = B_w_uk.reshape(DC * H, D)
    wuv = B_w_uv.reshape(DC * H, D)
    wob = B_w_o.reshape(H * D, M)

    any_spec = pl.BlockSpec(memory_space=pl.ANY)
    scratch = [
        pltpu.VMEM((S, M), BF16),
        pltpu.VMEM((MP, 3 * M), BF16),
        pltpu.VMEM((M, M), BF16),
        pltpu.VMEM((S, DC), BF16),
        pltpu.VMEM((M * H, D), BF16),
        pltpu.VMEM((DC * H, D), BF16),
        pltpu.VMEM((DC * H, D), BF16),
        pltpu.VMEM((H * D, M), BF16),
        pltpu.VMEM((NT_M, 14 * 128, 128), F32),
        pltpu.VMEM((3, MP, M), BF16),
        pltpu.VMEM((NT_M, M, 128), F32),
        pltpu.VMEM((MP, M), BF16),
        pltpu.VMEM((NT_M, HALO + S, 128), F32),
        pltpu.VMEM((NT_M, HALO + S, 128), F32),
        pltpu.VMEM((S, M), F32),
        pltpu.VMEM((S, 128), F32),
        pltpu.VMEM((NG, M, HG * D), BF16),
        pltpu.VMEM((NG, DC, 2 * HG * D), BF16),
        pltpu.VMEM((HG, S, D), BF16),
        pltpu.VMEM((HG, S, D), BF16),
        pltpu.VMEM((HG, S, D), BF16),
        pltpu.VMEM((H, S, D), BF16),
        pltpu.VMEM((S, M), BF16),
        pltpu.SemaphoreType.DMA((8,)),
        pltpu.SemaphoreType.DMA((S // RO,)),
    ]
    return pl.pallas_call(
        _kernel,
        out_shape=jax.ShapeDtypeStruct((1, S, M), BF16),
        in_specs=[any_spec] * 8 + [pl.BlockSpec(memory_space=pltpu.VMEM)],
        out_specs=any_spec,
        scratch_shapes=scratch,
        compiler_params=pltpu.CompilerParams(vmem_limit_bytes=120 * 1024 * 1024),
        name="gated_mix",
    )(x, A_wqkv, A_wo, c, wq, wuk, wuv, wob, gate_w)
```

```python
import functools
import math

import jax
import jax.numpy as jnp
import jax.experimental.pallas as pl
import jax.experimental.pallas.tpu as pltpu

F32 = jnp.float32
BF16 = jnp.bfloat16

S = 2048
M = 576
MP = 640
NT_M = MP // 128
H = 32
D = 128
DC = 512
DHA = 18
WIN = 8
DIL = 2
HALO = 16
LOG2E = math.log2(math.e)
NEG = -1e9

RA = 256
RS = 32
HG = 8
NG = H // HG
RP = 1024
TQ = 256
TB = 128
HU = 2
RO = 512
PITCH = 24
RELAY_START = 4

NN = (((1,), (0,)), ((), ()))
NT = (((1,), (1,)), ((), ()))


def _dot(a, b, dims=NN):
    return jax.lax.dot_general(a, b, dims, preferred_element_type=F32)


def _lane_partial(s, op):
    acc = s[:, 0:128]
    for j in range(1, s.shape[1] // 128):
        acc = op(acc, s[:, j * 128:(j + 1) * 128])
    return acc


def _recip(l):
    r = pl.reciprocal(l, approx=True)
    return r * (2.0 - l * r)


def _segments(r0):
    nsub = TQ // TB
    segs = []
    if r0 > 0:
        segs.append((0, TQ, 0, r0, False))
    for j in range(nsub):
        segs.append((j * TB, (j + 1) * TB, r0 + j * TB, r0 + (j + 1) * TB, True))
        if (j + 1) * TB < TQ:
            segs.append(((j + 1) * TB, TQ, r0 + j * TB, r0 + (j + 1) * TB, False))
    return segs


def _attn_scores(q_ref, k_ref, r0, tri):
    nsub = TQ // TB
    segs = _segments(r0)
    ss = []
    for (a, b, c, d, msk) in segs:
        s = _dot(q_ref[r0 + a:r0 + b, :], k_ref[c:d, :], NT)
        if msk:
            s = jnp.where(tri, s, NEG * LOG2E)
        ss.append(s)
    ms = []
    for i in range(nsub):
        m = None
        for (a, b, c, d, msk), s in zip(segs, ss):
            if a <= i * TB and (i + 1) * TB <= b:
                sm = _lane_partial(s[i * TB - a:(i + 1) * TB - a], jnp.maximum)
                m = sm if m is None else jnp.maximum(m, sm)
        ms.append(jnp.max(m, axis=1, keepdims=True))
    return ss, ms


def _attn_values(v_ref, r0, ss, ms):
    nsub = TQ // TB
    segs = _segments(r0)
    ls = [None] * nsub
    os_ = [None] * nsub
    for (a, b, c, d, msk), s in zip(segs, ss):
        m = jnp.concatenate(ms[a // TB:b // TB], axis=0) if b - a > TB else ms[a // TB]
        p = jnp.exp2(s - m)
        l = _lane_partial(p, jnp.add)
        o = _dot(p.astype(BF16), v_ref[c:d, :])
        for i in range(a // TB, b // TB):
            li = l[i * TB - a:(i + 1) * TB - a]
            oi = o[i * TB - a:(i + 1) * TB - a]
            ls[i] = li if ls[i] is None else ls[i] + li
            os_[i] = oi if os_[i] is None else os_[i] + oi
    return [o * _recip(jnp.sum(l, axis=1, keepdims=True)) for o, l in zip(os_, ls)]


def _kernel(xt_hbm, wqkv_hbm, woa_hbm, c_hbm, wq_hbm, wuk_hbm, wuv_hbm, wob_hbm, gate_hbm,
            out_hbm,
            xt_s, x_s, wqkv_s, woa_s, c_s, wq_raw, wuk_raw, wuv_raw, wob_s, gate_s,
            wt_s, wpt_s, wof_s, woap_s, woapt_s, kl_s, vl_s, acc_s, g_s,
            wq_s, wk_s, wv_s, q_s, k_s, v_s, ctx_s, out_s, sems, osems):
    def staged(w_hbm, raw, nrow):
        return w_hbm.bitcast(jnp.uint32), raw.reshape(nrow, PITCH, D).at[:, 0:H // 2, :]

    copies = {
        "wqkv": pltpu.make_async_copy(wqkv_hbm, wqkv_s.at[pl.ds(0, M)], sems.at[0]),
        "x": pltpu.make_async_copy(xt_hbm, xt_s, sems.at[1]),
        "gate": pltpu.make_async_copy(gate_hbm, gate_s, sems.at[8]),
        "woa": pltpu.make_async_copy(woa_hbm, woa_s, sems.at[2]),
        "wq": pltpu.make_async_copy(*staged(wq_hbm, wq_raw, M), sems.at[3]),
        "wuk": pltpu.make_async_copy(*staged(wuk_hbm, wuk_raw, DC), sems.at[4]),
        "wuv": pltpu.make_async_copy(*staged(wuv_hbm, wuv_raw, DC), sems.at[5]),
        "c": pltpu.make_async_copy(c_hbm, c_s, sems.at[6]),
        "wob": pltpu.make_async_copy(wob_hbm, wob_s, sems.at[7]),
    }
    copies["wqkv"].start(priority=0)
    for name in ("x", "gate", "woa"):
        copies[name].start(priority=1)

    def make_eye():
        return (jax.lax.broadcasted_iota(jnp.int32, (128, 128), 0)
                == jax.lax.broadcasted_iota(jnp.int32, (128, 128), 1)).astype(BF16)

    def a_prep():
        wqkv_s[M:MP, :] = jnp.zeros((MP - M, 3 * M), BF16)
        zero_halo = jnp.zeros((HALO, 128), F32)
        for j in range(NT_M):
            kl_s[j, 0:HALO, :] = zero_halo
            vl_s[j, 0:HALO, :] = zero_halo
        for sec in range(3):
            wpt_s[sec, M:MP, :] = jnp.zeros((MP - M, M), BF16)
        woap_s[M:MP, :] = jnp.zeros((MP - M, M), BF16)
        eye = make_eye()

        copies["wqkv"].wait()
        ncol = 3 * M
        for t in range(pl.cdiv(ncol, 128)):
            c0 = t * 128
            wd = min(128, ncol - c0)
            wt = _dot(eye[0:wd, 0:wd], wqkv_s[:, c0:c0 + wd], NT)
            for j in range(NT_M):
                wt_s[j, c0:c0 + wd, :] = wt[:, j * 128:(j + 1) * 128]
        for sec in range(3):
            for d in range(DHA):
                for j in range(NT_M):
                    rows = wt_s[j, pl.ds(sec * M + d, H, stride=DHA), :]
                    wj = min(128, M - j * 128)
                    wpt_s[sec, d * H:(d + 1) * H, j * 128:j * 128 + wj] = rows[:, 0:wj].astype(BF16)
        for name in ("x", "gate", "woa"):
            copies[name].wait()
        for name in ("wq", "wuk", "wuv"):
            copies[name].start()

    def a_prep_wo():
        eye = make_eye()
        woa = woa_s[...].astype(F32)
        for j in range(NT_M):
            wj = min(128, M - j * 128)
            blk = woa[:, j * 128:j * 128 + wj]
            if wj < 128:
                blk = jnp.concatenate([blk, jnp.zeros((M, 128 - wj), F32)], axis=1)
            wof_s[j] = blk
        for d in range(DHA):
            for j in range(NT_M):
                wj = min(128, M - j * 128)
                rows = wof_s[j, pl.ds(d, H, stride=DHA), :]
                woap_s[d * H:(d + 1) * H, j * 128:j * 128 + wj] = rows[:, 0:wj].astype(BF16)
        for j in range(NT_M):
            wj = min(128, M - j * 128)
            woapt_s[j * 128:j * 128 + wj, :] = _dot(
                eye[0:wj, 0:wj], woap_s[:, j * 128:j * 128 + wj], NT).astype(BF16)

    def a_xpose(c):
        eye = make_eye()
        r0 = c * RA
        for t in range(r0 // 128, (r0 + RA) // 128):
            x_s[t * 128:(t + 1) * 128, :] = _dot(eye, xt_s[:, t * 128:(t + 1) * 128], NT).astype(BF16)
        gw = jnp.broadcast_to(gate_s[...].reshape(1, M), (16, M))
        g_s[:, r0:r0 + RA] = jax.nn.sigmoid(_dot(gw, xt_s[:, r0:r0 + RA]))

    a_scale = (DHA ** -0.5) * LOG2E

    def a_proj(c, fill):
        r0 = c * RA
        xq = x_s[r0:r0 + RA, :]
        q = _dot(xq, wpt_s[0], NT)
        fill()
        k = _dot(xq, wpt_s[1], NT)
        for j in range(NT_M):
            kl_s[j, HALO + r0:HALO + r0 + RA, :] = k[:, j * 128:(j + 1) * 128]
        fill()
        v = _dot(xq, wpt_s[2], NT)
        for j in range(NT_M):
            vl_s[j, HALO + r0:HALO + r0 + RA, :] = v[:, j * 128:(j + 1) * 128]
        fill()
        return [q[:, j * 128:(j + 1) * 128] * a_scale for j in range(NT_M)]

    def a_local_sub(r0, qt):
        logits = []
        for w in range(WIN):
            off = HALO + r0 - w * DIL
            s = None
            for j in range(NT_M):
                t = qt[j] * kl_s[j, off:off + RS, :]
                s = t if s is None else s + t
            s = s + pltpu.roll(s, 64, 1)
            s = s + pltpu.roll(s, 32, 1)
            if r0 < w * DIL:
                rowi = jax.lax.broadcasted_iota(jnp.int32, (RS, 128), 0)
                s = jnp.where(rowi + r0 >= w * DIL, s, NEG * LOG2E)
            logits.append(s)
        m = functools.reduce(jnp.maximum, logits)
        ps = [jnp.exp2(s - m) for s in logits]
        r = _recip(functools.reduce(jnp.add, ps))
        ot = []
        for j in range(NT_M):
            o = None
            for w in range(WIN):
                off = HALO + r0 - w * DIL
                t = ps[w] * vl_s[j, off:off + RS, :]
                o = t if o is None else o + t
            ot.append((o * r).astype(BF16))
        return jnp.concatenate(ot, axis=1)

    def a_local(c, qt, fill):
        r0 = c * RA
        outs = []
        for sb in range(RA // RS):
            outs.append(a_local_sub(r0 + sb * RS, [q[sb * RS:(sb + 1) * RS] for q in qt]))
            if sb % 4 == 3:
                fill()
        return jnp.concatenate(outs, axis=0)

    def a_out(c, o):
        r0 = c * RA
        at = _dot(woapt_s[...], o, NT)
        acc_s[:, r0:r0 + RA] = at * g_s[0:1, r0:r0 + RA]

    def a_main():
        nca = S // RA
        st = {}
        pending = []
        per_fill = [0]

        def fill():
            for _ in range(per_fill[0]):
                if pending:
                    pending.pop(0)()

        a_xpose(0)
        for t in range(nca + 2):
            if t == RELAY_START:
                for name in ("wq", "wuk", "wuv"):
                    copies[name].wait()
                for name in ("c", "wob"):
                    copies[name].start()
                pending.extend(relayout_units())
                nfill = (nca - RELAY_START) * 5 + 2
                per_fill[0] = pl.cdiv(len(pending), nfill)
            if t + 1 < nca:
                a_xpose(t + 1)
            if t < nca:
                st[t] = a_proj(t, fill)
            if t == 0:
                a_prep_wo()
            if 0 <= t - 1 < nca:
                st[t - 1] = a_local(t - 1, st[t - 1], fill)
            if 0 <= t - 2 < nca:
                a_out(t - 2, st.pop(t - 2))
        while pending:
            pending.pop(0)()

    def relayout_pair(raw, nrow, dst, pr):
        u = raw[pl.ds(pr, nrow, stride=PITCH), :]
        dst[2 * pr] = pltpu.bitcast(u << 16, F32).astype(BF16)
        dst[2 * pr + 1] = pltpu.bitcast(u & jnp.uint32(0xFFFF0000), F32).astype(BF16)

    def relayout_units():
        units = []
        for raw, nrow, dst in ((wq_raw, M, wq_s), (wuk_raw, DC, wk_s), (wuv_raw, DC, wv_s)):
            for pr in range(H // 2):
                units.append(functools.partial(relayout_pair, raw, nrow, dst, pr))
        return units

    b_scale = (D ** -0.5) * LOG2E

    def group_body(g, carry):
        def proj_body(rc, c2):
            r0 = pl.multiple_of(rc * RP, RP)
            wq = jnp.concatenate([wq_s[g * HG + i] for i in range(HG)], axis=1)
            wkv = jnp.concatenate([wk_s[g * HG + i] for i in range(HG)]
                                  + [wv_s[g * HG + i] for i in range(HG)], axis=1)
            q = _dot(x_s[pl.ds(r0, RP), :], wq) * b_scale
            kv = _dot(c_s[pl.ds(r0, RP), :], wkv)
            for i in range(HG):
                q_s[i, pl.ds(r0, RP), :] = q[:, i * D:(i + 1) * D].astype(BF16)
                k_s[i, pl.ds(r0, RP), :] = kv[:, i * D:(i + 1) * D].astype(BF16)
                v_s[i, pl.ds(r0, RP), :] = kv[:, (HG + i) * D:(HG + i + 1) * D].astype(BF16)
            return c2

        with jax.named_scope("B_proj"):
            jax.lax.fori_loop(0, S // RP, proj_body, 0)

        def attn_body(it, c2):
            row = jax.lax.broadcasted_iota(jnp.int32, (TB, TB), 0)
            col = jax.lax.broadcasted_iota(jnp.int32, (TB, TB), 1)
            tri = col <= row
            items = [(u, r) for u in range(HU) for r in range(S // TQ)[::-1]]
            pend = {}
            for t in range(len(items) + 1):
                if t < len(items):
                    u, r = items[t]
                    hh = it * HU + u
                    pend[items[t]] = _attn_scores(q_s.at[hh], k_s.at[hh], r * TQ, tri)
                if t >= 1:
                    u, r = items[t - 1]
                    hh = it * HU + u
                    r0 = r * TQ
                    outs = _attn_values(v_s.at[hh], r0, *pend.pop(items[t - 1]))
                    for j, o in enumerate(outs):
                        ctx_s[g * HG + hh, r0 + j * TB:r0 + (j + 1) * TB, :] = o.astype(BF16)
            return c2

        with jax.named_scope("B_attn"):
            jax.lax.fori_loop(0, HG // HU, attn_body, 0)
        return carry

    def out_copy(i):
        r0 = i * RO
        if not isinstance(i, int):
            r0 = pl.multiple_of(r0, RO)
        return pltpu.make_async_copy(out_s.at[:, pl.ds(r0, RO)], out_hbm.at[0, :, pl.ds(r0, RO)], osems.at[i])

    def out_body(i, carry):
        r0 = pl.multiple_of(i * RO, RO)
        ctx = jnp.concatenate([ctx_s[h, pl.ds(r0, RO), :] for h in range(H)], axis=1)
        wo = jnp.concatenate([wob_s[h] for h in range(H)], axis=1)
        bt = _dot(wo, ctx, NT)
        omg = 1.0 - g_s[0:1, pl.ds(r0, RO)]
        out_s[:, pl.ds(r0, RO)] = (acc_s[:, pl.ds(r0, RO)] + omg * bt).astype(BF16)
        out_copy(i).start()
        return carry

    with jax.named_scope("A_prep"):
        a_prep()
    with jax.named_scope("A_main"):
        a_main()
        copies["c"].wait()
    jax.lax.fori_loop(0, NG, group_body, 0)
    with jax.named_scope("B_out"):
        copies["wob"].wait()
        jax.lax.fori_loop(0, S // RO, out_body, 0)
        for i in range(S // RO):
            out_copy(i).wait()


@jax.jit
def pallas_gated_mix__sliding_local_dilated__compressed_kv_cla__prompt_kernel(
    A_x: jax.Array,
    A_wqkv: jax.Array,
    A_wo: jax.Array,
    B_x: jax.Array,
    B_c_kv: jax.Array,
    B_w_q: jax.Array,
    B_w_uk: jax.Array,
    B_w_uv: jax.Array,
    B_w_o: jax.Array,
    gate_w: jax.Array,
):
    del B_x
    xt = jnp.swapaxes(A_x, 1, 2).reshape(M, S)
    c = B_c_kv.reshape(S, DC)
    wob = jnp.swapaxes(B_w_o, 1, 2)

    any_spec = pl.BlockSpec(memory_space=pl.ANY)
    scratch = [
        pltpu.VMEM((M, S), BF16),
        pltpu.VMEM((S, M), BF16),
        pltpu.VMEM((MP, 3 * M), BF16),
        pltpu.VMEM((M, M), BF16),
        pltpu.VMEM((S, DC), BF16),
        pltpu.VMEM((M * PITCH, D), jnp.uint32),
        pltpu.VMEM((DC * PITCH, D), jnp.uint32),
        pltpu.VMEM((DC * PITCH, D), jnp.uint32),
        pltpu.VMEM((H, M, D), BF16),
        pltpu.VMEM((M,), BF16),
        pltpu.VMEM((NT_M, 14 * 128, 128), F32),
        pltpu.VMEM((3, MP, M), BF16),
        pltpu.VMEM((NT_M, M, 128), F32),
        pltpu.VMEM((MP, M), BF16),
        pltpu.VMEM((M, MP), BF16),
        pltpu.VMEM((NT_M, HALO + S, 128), F32),
        pltpu.VMEM((NT_M, HALO + S, 128), F32),
        pltpu.VMEM((M, S), F32),
        pltpu.VMEM((16, S), F32),
        pltpu.VMEM((H, M, D), BF16),
        pltpu.VMEM((H, DC, D), BF16),
        pltpu.VMEM((H, DC, D), BF16),
        pltpu.VMEM((HG, S, D), BF16),
        pltpu.VMEM((HG, S, D), BF16),
        pltpu.VMEM((HG, S, D), BF16),
        pltpu.VMEM((H, S, D), BF16),
        pltpu.VMEM((M, S), BF16),
        pltpu.SemaphoreType.DMA((9,)),
        pltpu.SemaphoreType.DMA((S // RO,)),
    ]
    out_t = pl.pallas_call(
        _kernel,
        out_shape=jax.ShapeDtypeStruct((1, M, S), BF16),
        in_specs=[any_spec] * 9,
        out_specs=any_spec,
        scratch_shapes=scratch,
        compiler_params=pltpu.CompilerParams(vmem_limit_bytes=120 * 1024 * 1024),
        name="gated_mix",
    )(xt, A_wqkv, A_wo, c, B_w_q, B_w_uk, B_w_uv, wob, gate_w)
    return jnp.swapaxes(out_t, 1, 2)
```

```python
import functools
import math

import jax
import jax.numpy as jnp
import jax.experimental.pallas as pl
import jax.experimental.pallas.tpu as pltpu

F32 = jnp.float32
BF16 = jnp.bfloat16

S = 2048
M = 576
MP = 640
NT_M = MP // 128
H = 32
D = 128
DC = 512
DHA = 18
WIN = 8
DIL = 2
HALO = 16
LOG2E = math.log2(math.e)
NEG = -1e9

RA = 256
RS = 32
HG = 8
NG = H // HG
RP = 1024
TQ = 256
TB = 128
HU = 2
RO = 512
NPAIR = H // 2

NN = (((1,), (0,)), ((), ()))
NT = (((1,), (1,)), ((), ()))


def _dot(a, b, dims=NN):
    return jax.lax.dot_general(a, b, dims, preferred_element_type=F32)


def _lane_partial(s, op):
    acc = s[:, 0:128]
    for j in range(1, s.shape[1] // 128):
        acc = op(acc, s[:, j * 128:(j + 1) * 128])
    return acc


def _recip(l):
    r = pl.reciprocal(l, approx=True)
    return r * (2.0 - l * r)


def _segments(r0):
    nsub = TQ // TB
    segs = []
    if r0 > 0:
        segs.append((0, TQ, 0, r0, False))
    for j in range(nsub):
        segs.append((j * TB, (j + 1) * TB, r0 + j * TB, r0 + (j + 1) * TB, True))
        if (j + 1) * TB < TQ:
            segs.append(((j + 1) * TB, TQ, r0 + j * TB, r0 + (j + 1) * TB, False))
    return segs


def _attn_scores(q_ref, k_ref, r0, tri):
    nsub = TQ // TB
    segs = _segments(r0)
    ss = []
    for (a, b, c, d, msk) in segs:
        s = _dot(q_ref[r0 + a:r0 + b, :], k_ref[c:d, :], NT)
        if msk:
            s = jnp.where(tri, s, NEG * LOG2E)
        ss.append(s)
    ms = []
    for i in range(nsub):
        m = None
        for (a, b, c, d, msk), s in zip(segs, ss):
            if a <= i * TB and (i + 1) * TB <= b:
                sm = _lane_partial(s[i * TB - a:(i + 1) * TB - a], jnp.maximum)
                m = sm if m is None else jnp.maximum(m, sm)
        ms.append(jnp.max(m, axis=1, keepdims=True))
    return ss, ms


def _attn_values(v_ref, r0, ss, ms):
    nsub = TQ // TB
    segs = _segments(r0)
    ls = [None] * nsub
    os_ = [None] * nsub
    for (a, b, c, d, msk), s in zip(segs, ss):
        m = jnp.concatenate(ms[a // TB:b // TB], axis=0) if b - a > TB else ms[a // TB]
        p = jnp.exp2(s - m)
        l = _lane_partial(p, jnp.add)
        o = _dot(p.astype(BF16), v_ref[c:d, :])
        for i in range(a // TB, b // TB):
            li = l[i * TB - a:(i + 1) * TB - a]
            oi = o[i * TB - a:(i + 1) * TB - a]
            ls[i] = li if ls[i] is None else ls[i] + li
            os_[i] = oi if os_[i] is None else os_[i] + oi
    return [o * _recip(jnp.sum(l, axis=1, keepdims=True)) for o, l in zip(os_, ls)]


def _kernel(xt_hbm, wqkv_hbm, woa_hbm, c_hbm, wq_hbm, wuk_hbm, wuv_hbm, wob_hbm, gate_hbm,
            out_hbm,
            xt_s, x_s, wqkv_s, woa_s, c_s, wq_raw, wuk_raw, wuv_raw, wob_s, gate_s,
            wt_s, wpt_s, wof_s, woap_s, woapt_s, kl_s, vl_s, acc_s, g_s,
            q_s, k_s, v_s, ctx_s, out_s, sems, wsems, osems):
    copies = {
        "wqkv": pltpu.make_async_copy(wqkv_hbm, wqkv_s.at[pl.ds(0, M)], sems.at[0]),
        "x": pltpu.make_async_copy(xt_hbm, xt_s, sems.at[1]),
        "gate": pltpu.make_async_copy(gate_hbm, gate_s, sems.at[2]),
        "woa": pltpu.make_async_copy(woa_hbm, woa_s, sems.at[3]),
        "c": pltpu.make_async_copy(c_hbm, c_s, sems.at[4]),
        "wob": pltpu.make_async_copy(wob_hbm, wob_s, sems.at[5]),
    }
    pair_copies = []
    for wi, (w_hbm, raw) in enumerate(((wq_hbm, wq_raw), (wuk_hbm, wuk_raw), (wuv_hbm, wuv_raw))):
        w32 = w_hbm.bitcast(jnp.uint32)
        for j in range(NPAIR):
            pair_copies.append(pltpu.make_async_copy(
                w32.at[:, j, :], raw.at[j], wsems.at[wi * NPAIR + j]))
    copies["wqkv"].start(priority=0)
    for name in ("x", "gate", "woa"):
        copies[name].start(priority=1)

    def make_eye():
        return (jax.lax.broadcasted_iota(jnp.int32, (128, 128), 0)
                == jax.lax.broadcasted_iota(jnp.int32, (128, 128), 1)).astype(BF16)

    def a_prep():
        wqkv_s[M:MP, :] = jnp.zeros((MP - M, 3 * M), BF16)
        zero_halo = jnp.zeros((HALO, 128), F32)
        for j in range(NT_M):
            kl_s[j, 0:HALO, :] = zero_halo
            vl_s[j, 0:HALO, :] = zero_halo
        for sec in range(3):
            wpt_s[sec, M:MP, :] = jnp.zeros((MP - M, M), BF16)
        woap_s[M:MP, :] = jnp.zeros((MP - M, M), BF16)
        eye = make_eye()

        copies["wqkv"].wait()
        ncol = 3 * M
        for t in range(pl.cdiv(ncol, 128)):
            c0 = t * 128
            wd = min(128, ncol - c0)
            wt = _dot(eye[0:wd, 0:wd], wqkv_s[:, c0:c0 + wd], NT)
            for j in range(NT_M):
                wt_s[j, c0:c0 + wd, :] = wt[:, j * 128:(j + 1) * 128]
        for sec in range(3):
            for d in range(DHA):
                for j in range(NT_M):
                    rows = wt_s[j, pl.ds(sec * M + d, H, stride=DHA), :]
                    wj = min(128, M - j * 128)
                    wpt_s[sec, d * H:(d + 1) * H, j * 128:j * 128 + wj] = rows[:, 0:wj].astype(BF16)
        for name in ("x", "gate", "woa"):
            copies[name].wait()
        copies["c"].start()
        for j in range(NPAIR):
            for wi in range(3):
                pair_copies[wi * NPAIR + j].start()
        copies["wob"].start()

    def a_prep_wo():
        eye = make_eye()
        woa = woa_s[...].astype(F32)
        for j in range(NT_M):
            wj = min(128, M - j * 128)
            blk = woa[:, j * 128:j * 128 + wj]
            if wj < 128:
                blk = jnp.concatenate([blk, jnp.zeros((M, 128 - wj), F32)], axis=1)
            wof_s[j] = blk
        for d in range(DHA):
            for j in range(NT_M):
                wj = min(128, M - j * 128)
                rows = wof_s[j, pl.ds(d, H, stride=DHA), :]
                woap_s[d * H:(d + 1) * H, j * 128:j * 128 + wj] = rows[:, 0:wj].astype(BF16)
        for j in range(NT_M):
            wj = min(128, M - j * 128)
            woapt_s[j * 128:j * 128 + wj, :] = _dot(
                eye[0:wj, 0:wj], woap_s[:, j * 128:j * 128 + wj], NT).astype(BF16)

    def a_xpose(c):
        eye = make_eye()
        r0 = c * RA
        for t in range(r0 // 128, (r0 + RA) // 128):
            x_s[t * 128:(t + 1) * 128, :] = _dot(eye, xt_s[:, t * 128:(t + 1) * 128], NT).astype(BF16)
        gw = jnp.broadcast_to(gate_s[...].reshape(1, M), (16, M))
        g_s[:, r0:r0 + RA] = jax.nn.sigmoid(_dot(gw, xt_s[:, r0:r0 + RA]))

    a_scale = (DHA ** -0.5) * LOG2E

    def a_proj(c):
        r0 = c * RA
        xq = x_s[r0:r0 + RA, :]
        q = _dot(xq, wpt_s[0], NT)
        k = _dot(xq, wpt_s[1], NT)
        for j in range(NT_M):
            kl_s[j, HALO + r0:HALO + r0 + RA, :] = k[:, j * 128:(j + 1) * 128]
        v = _dot(xq, wpt_s[2], NT)
        for j in range(NT_M):
            vl_s[j, HALO + r0:HALO + r0 + RA, :] = v[:, j * 128:(j + 1) * 128]
        return [q[:, j * 128:(j + 1) * 128] * a_scale for j in range(NT_M)]

    def a_local_sub(r0, qt):
        logits = []
        for w in range(WIN):
            off = HALO + r0 - w * DIL
            s = None
            for j in range(NT_M):
                t = qt[j] * kl_s[j, off:off + RS, :]
                s = t if s is None else s + t
            s = s + pltpu.roll(s, 64, 1)
            s = s + pltpu.roll(s, 32, 1)
            if r0 < w * DIL:
                rowi = jax.lax.broadcasted_iota(jnp.int32, (RS, 128), 0)
                s = jnp.where(rowi + r0 >= w * DIL, s, NEG * LOG2E)
            logits.append(s)
        m = functools.reduce(jnp.maximum, logits)
        ps = [jnp.exp2(s - m) for s in logits]
        r = _recip(functools.reduce(jnp.add, ps))
        ot = []
        for j in range(NT_M):
            o = None
            for w in range(WIN):
                off = HALO + r0 - w * DIL
                t = ps[w] * vl_s[j, off:off + RS, :]
                o = t if o is None else o + t
            ot.append((o * r).astype(BF16))
        return jnp.concatenate(ot, axis=1)

    def a_local(c, qt):
        r0 = c * RA
        outs = []
        for sb in range(RA // RS):
            outs.append(a_local_sub(r0 + sb * RS, [q[sb * RS:(sb + 1) * RS] for q in qt]))
        return jnp.concatenate(outs, axis=0)

    def a_out(c, o):
        r0 = c * RA
        at = _dot(woapt_s[...], o, NT)
        acc_s[:, r0:r0 + RA] = at * g_s[0:1, r0:r0 + RA]

    def a_main():
        nca = S // RA
        st = {}
        a_xpose(0)
        for t in range(nca + 2):
            if t + 1 < nca:
                a_xpose(t + 1)
            if t < nca:
                st[t] = a_proj(t)
            if t == 0:
                a_prep_wo()
            if 0 <= t - 1 < nca:
                st[t - 1] = a_local(t - 1, st[t - 1])
            if 0 <= t - 2 < nca:
                a_out(t - 2, st.pop(t - 2))

    def group_weights(raw, g):
        cols = []
        for b in range(HG // 2):
            u = raw[g * (HG // 2) + b]
            cols.append(pltpu.bitcast(u << 16, F32).astype(BF16))
            cols.append(pltpu.bitcast(u & jnp.uint32(0xFFFF0000), F32).astype(BF16))
        return jnp.concatenate(cols, axis=1)

    b_scale = (D ** -0.5) * LOG2E

    def group_body(g, carry):
        def proj_body(rc, c2):
            r0 = pl.multiple_of(rc * RP, RP)
            wq = group_weights(wq_raw, g)
            wkv = jnp.concatenate([group_weights(wuk_raw, g), group_weights(wuv_raw, g)], axis=1)
            q = _dot(x_s[pl.ds(r0, RP), :], wq) * b_scale
            kv = _dot(c_s[pl.ds(r0, RP), :], wkv)
            for i in range(HG):
                q_s[i, pl.ds(r0, RP), :] = q[:, i * D:(i + 1) * D].astype(BF16)
                k_s[i, pl.ds(r0, RP), :] = kv[:, i * D:(i + 1) * D].astype(BF16)
                v_s[i, pl.ds(r0, RP), :] = kv[:, (HG + i) * D:(HG + i + 1) * D].astype(BF16)
            return c2

        with jax.named_scope("B_proj"):
            jax.lax.fori_loop(0, S // RP, proj_body, 0)

        def attn_body(it, c2):
            row = jax.lax.broadcasted_iota(jnp.int32, (TB, TB), 0)
            col = jax.lax.broadcasted_iota(jnp.int32, (TB, TB), 1)
            tri = col <= row
            items = [(u, r) for u in range(HU) for r in range(S // TQ)[::-1]]
            pend = {}
            for t in range(len(items) + 1):
                if t < len(items):
                    u, r = items[t]
                    hh = it * HU + u
                    pend[items[t]] = _attn_scores(q_s.at[hh], k_s.at[hh], r * TQ, tri)
                if t >= 1:
                    u, r = items[t - 1]
                    hh = it * HU + u
                    r0 = r * TQ
                    outs = _attn_values(v_s.at[hh], r0, *pend.pop(items[t - 1]))
                    for j, o in enumerate(outs):
                        ctx_s[g * HG + hh, r0 + j * TB:r0 + (j + 1) * TB, :] = o.astype(BF16)
            return c2

        with jax.named_scope("B_attn"):
            jax.lax.fori_loop(0, HG // HU, attn_body, 0)
        return carry

    def out_copy(i):
        r0 = i * RO
        if not isinstance(i, int):
            r0 = pl.multiple_of(r0, RO)
        return pltpu.make_async_copy(out_s.at[:, pl.ds(r0, RO)], out_hbm.at[0, :, pl.ds(r0, RO)], osems.at[i])

    def out_body(i, carry):
        r0 = pl.multiple_of(i * RO, RO)
        ctx = jnp.concatenate([ctx_s[h, pl.ds(r0, RO), :] for h in range(H)], axis=1)
        wo = jnp.concatenate([wob_s[h] for h in range(H)], axis=1)
        bt = _dot(wo, ctx, NT)
        omg = 1.0 - g_s[0:1, pl.ds(r0, RO)]
        out_s[:, pl.ds(r0, RO)] = (acc_s[:, pl.ds(r0, RO)] + omg * bt).astype(BF16)
        out_copy(i).start()
        return carry

    with jax.named_scope("A_prep"):
        a_prep()
    with jax.named_scope("A_main"):
        a_main()
        copies["c"].wait()
        for cp in pair_copies:
            cp.wait()
    jax.lax.fori_loop(0, NG, group_body, 0)
    with jax.named_scope("B_out"):
        copies["wob"].wait()
        jax.lax.fori_loop(0, S // RO, out_body, 0)
        for i in range(S // RO):
            out_copy(i).wait()


@jax.jit
def pallas_gated_mix__sliding_local_dilated__compressed_kv_cla__prompt_kernel(
    A_x: jax.Array,
    A_wqkv: jax.Array,
    A_wo: jax.Array,
    B_x: jax.Array,
    B_c_kv: jax.Array,
    B_w_q: jax.Array,
    B_w_uk: jax.Array,
    B_w_uv: jax.Array,
    B_w_o: jax.Array,
    gate_w: jax.Array,
):
    del B_x
    xt = jnp.swapaxes(A_x, 1, 2).reshape(M, S)
    c = B_c_kv.reshape(S, DC)
    wob = jnp.swapaxes(B_w_o, 1, 2)

    any_spec = pl.BlockSpec(memory_space=pl.ANY)
    scratch = [
        pltpu.VMEM((M, S), BF16),
        pltpu.VMEM((S, M), BF16),
        pltpu.VMEM((MP, 3 * M), BF16),
        pltpu.VMEM((M, M), BF16),
        pltpu.VMEM((S, DC), BF16),
        pltpu.VMEM((NPAIR, M, D), jnp.uint32),
        pltpu.VMEM((NPAIR, DC, D), jnp.uint32),
        pltpu.VMEM((NPAIR, DC, D), jnp.uint32),
        pltpu.VMEM((H, M, D), BF16),
        pltpu.VMEM((M,), BF16),
        pltpu.VMEM((NT_M, 14 * 128, 128), F32),
        pltpu.VMEM((3, MP, M), BF16),
        pltpu.VMEM((NT_M, M, 128), F32),
        pltpu.VMEM((MP, M), BF16),
        pltpu.VMEM((M, MP), BF16),
        pltpu.VMEM((NT_M, HALO + S, 128), F32),
        pltpu.VMEM((NT_M, HALO + S, 128), F32),
        pltpu.VMEM((M, S), F32),
        pltpu.VMEM((16, S), F32),
        pltpu.VMEM((HG, S, D), BF16),
        pltpu.VMEM((HG, S, D), BF16),
        pltpu.VMEM((HG, S, D), BF16),
        pltpu.VMEM((H, S, D), BF16),
        pltpu.VMEM((M, S), BF16),
        pltpu.SemaphoreType.DMA((6,)),
        pltpu.SemaphoreType.DMA((3 * NPAIR,)),
        pltpu.SemaphoreType.DMA((S // RO,)),
    ]
    out_t = pl.pallas_call(
        _kernel,
        out_shape=jax.ShapeDtypeStruct((1, M, S), BF16),
        in_specs=[any_spec] * 9,
        out_specs=any_spec,
        scratch_shapes=scratch,
        compiler_params=pltpu.CompilerParams(vmem_limit_bytes=120 * 1024 * 1024),
        name="gated_mix",
    )(xt, A_wqkv, A_wo, c, B_w_q, B_w_uk, B_w_uv, wob, gate_w)
    return jnp.swapaxes(out_t, 1, 2)
```

```python
import functools
import math

import jax
import jax.numpy as jnp
import jax.experimental.pallas as pl
import jax.experimental.pallas.tpu as pltpu

F32 = jnp.float32
BF16 = jnp.bfloat16

S = 2048
M = 576
MP = 640
NT_M = MP // 128
H = 32
D = 128
DC = 512
DHA = 18
WIN = 8
DIL = 2
HALO = 16
LOG2E = math.log2(math.e)
NEG = -1e9

RA = 256
RS = 32
HG = 8
NG = H // HG
RP = 1024
TQ = 256
TB = 128
HU = 2
RO = 512
NPAIR = H // 2

NN = (((1,), (0,)), ((), ()))
NT = (((1,), (1,)), ((), ()))


def _dot(a, b, dims=NN):
    return jax.lax.dot_general(a, b, dims, preferred_element_type=F32)


def _lane_partial(s, op):
    acc = s[:, 0:128]
    for j in range(1, s.shape[1] // 128):
        acc = op(acc, s[:, j * 128:(j + 1) * 128])
    return acc


def _recip(l):
    r = pl.reciprocal(l, approx=True)
    return r * (2.0 - l * r)


def _segments(r0):
    nsub = TQ // TB
    segs = []
    if r0 > 0:
        segs.append((0, TQ, 0, r0, False))
    for j in range(nsub):
        segs.append((j * TB, (j + 1) * TB, r0 + j * TB, r0 + (j + 1) * TB, True))
        if (j + 1) * TB < TQ:
            segs.append(((j + 1) * TB, TQ, r0 + j * TB, r0 + (j + 1) * TB, False))
    return segs


def _attn_scores(q_ref, k_ref, r0, tri):
    nsub = TQ // TB
    segs = _segments(r0)
    ss = []
    for (a, b, c, d, msk) in segs:
        s = _dot(q_ref[r0 + a:r0 + b, :], k_ref[c:d, :], NT)
        if msk:
            s = jnp.where(tri, s, NEG * LOG2E)
        ss.append(s)
    ms = []
    for i in range(nsub):
        m = None
        for (a, b, c, d, msk), s in zip(segs, ss):
            if a <= i * TB and (i + 1) * TB <= b:
                sm = _lane_partial(s[i * TB - a:(i + 1) * TB - a], jnp.maximum)
                m = sm if m is None else jnp.maximum(m, sm)
        ms.append(jnp.max(m, axis=1, keepdims=True))
    return ss, ms


def _attn_values(v_ref, r0, ss, ms):
    nsub = TQ // TB
    segs = _segments(r0)
    ls = [None] * nsub
    os_ = [None] * nsub
    for (a, b, c, d, msk), s in zip(segs, ss):
        m = jnp.concatenate(ms[a // TB:b // TB], axis=0) if b - a > TB else ms[a // TB]
        p = jnp.exp2(s - m)
        l = _lane_partial(p, jnp.add)
        o = _dot(p.astype(BF16), v_ref[c:d, :])
        for i in range(a // TB, b // TB):
            li = l[i * TB - a:(i + 1) * TB - a]
            oi = o[i * TB - a:(i + 1) * TB - a]
            ls[i] = li if ls[i] is None else ls[i] + li
            os_[i] = oi if os_[i] is None else os_[i] + oi
    return [o * _recip(jnp.sum(l, axis=1, keepdims=True)) for o, l in zip(os_, ls)]


def _kernel(xt_hbm, wqkv_hbm, woa_hbm, c_hbm, wq_hbm, wuk_hbm, wuv_hbm, wob_hbm, gate_hbm,
            out_hbm,
            xt_s, x_s, wqkv_s, woa_s, c_s, wq_raw, wuk_raw, wuv_raw, wob_s, gate_s,
            wt_s, wpt_s, wof_s, woap_s, woapt_s, kl_s, vl_s, acc_s, g_s,
            q_s, k_s, v_s, ctx_s, out_s, sems, wsems, osems):
    copies = {
        "wqkv": pltpu.make_async_copy(wqkv_hbm, wqkv_s.at[pl.ds(0, M)], sems.at[0]),
        "x": pltpu.make_async_copy(xt_hbm, xt_s, sems.at[1]),
        "gate": pltpu.make_async_copy(gate_hbm, gate_s, sems.at[2]),
        "woa": pltpu.make_async_copy(woa_hbm, woa_s, sems.at[3]),
        "c": pltpu.make_async_copy(c_hbm, c_s, sems.at[4]),
        "wob": pltpu.make_async_copy(wob_hbm, wob_s, sems.at[5]),
    }
    pair_copies = []
    for wi, (w_hbm, raw) in enumerate(((wq_hbm, wq_raw), (wuk_hbm, wuk_raw), (wuv_hbm, wuv_raw))):
        w32 = w_hbm.bitcast(jnp.uint32)
        for j in range(NPAIR):
            pair_copies.append(pltpu.make_async_copy(
                w32.at[:, j, :], raw.at[j], wsems.at[wi * NPAIR + j]))
    copies["gate"].start(priority=0)
    copies["wqkv"].start(priority=0)
    for name in ("x", "woa"):
        copies[name].start(priority=1)

    def make_eye():
        return (jax.lax.broadcasted_iota(jnp.int32, (128, 128), 0)
                == jax.lax.broadcasted_iota(jnp.int32, (128, 128), 1)).astype(BF16)

    def a_prep():
        wqkv_s[M:MP, :] = jnp.zeros((MP - M, 3 * M), BF16)
        zero_halo = jnp.zeros((HALO, 128), F32)
        for j in range(NT_M):
            kl_s[j, 0:HALO, :] = zero_halo
            vl_s[j, 0:HALO, :] = zero_halo
        for sec in range(3):
            wpt_s[sec, M:MP, :] = jnp.zeros((MP - M, M), BF16)
        woap_s[M:MP, :] = jnp.zeros((MP - M, M), BF16)
        eye = make_eye()

        copies["wqkv"].wait()
        ncol = 3 * M
        for t in range(pl.cdiv(ncol, 128)):
            c0 = t * 128
            wd = min(128, ncol - c0)
            wt = _dot(eye[0:wd, 0:wd], wqkv_s[:, c0:c0 + wd], NT)
            for j in range(NT_M):
                wt_s[j, c0:c0 + wd, :] = wt[:, j * 128:(j + 1) * 128]
        for sec in range(3):
            for d in range(DHA):
                for j in range(NT_M):
                    rows = wt_s[j, pl.ds(sec * M + d, H, stride=DHA), :]
                    wj = min(128, M - j * 128)
                    wpt_s[sec, d * H:(d + 1) * H, j * 128:j * 128 + wj] = rows[:, 0:wj].astype(BF16)
        copies["x"].wait()
        copies["woa"].wait()
        copies["c"].start()
        for j in range(NPAIR):
            for wi in range(3):
                pair_copies[wi * NPAIR + j].start()
        copies["wob"].start()
        copies["gate"].wait()

    def a_prep_wo():
        eye = make_eye()
        woa = woa_s[...].astype(F32)
        for j in range(NT_M):
            wj = min(128, M - j * 128)
            blk = woa[:, j * 128:j * 128 + wj]
            if wj < 128:
                blk = jnp.concatenate([blk, jnp.zeros((M, 128 - wj), F32)], axis=1)
            wof_s[j] = blk
        for d in range(DHA):
            for j in range(NT_M):
                wj = min(128, M - j * 128)
                rows = wof_s[j, pl.ds(d, H, stride=DHA), :]
                woap_s[d * H:(d + 1) * H, j * 128:j * 128 + wj] = rows[:, 0:wj].astype(BF16)
        for j in range(NT_M):
            wj = min(128, M - j * 128)
            woapt_s[j * 128:j * 128 + wj, :] = _dot(
                eye[0:wj, 0:wj], woap_s[:, j * 128:j * 128 + wj], NT).astype(BF16)

    def a_xpose(c):
        eye = make_eye()
        r0 = c * RA
        for t in range(r0 // 128, (r0 + RA) // 128):
            x_s[t * 128:(t + 1) * 128, :] = _dot(eye, xt_s[:, t * 128:(t + 1) * 128], NT).astype(BF16)
        gw = jnp.broadcast_to(gate_s[...].reshape(1, M), (16, M))
        g_s[:, r0:r0 + RA] = jax.nn.sigmoid(_dot(gw, xt_s[:, r0:r0 + RA]))

    a_scale = (DHA ** -0.5) * LOG2E

    def a_proj(c):
        r0 = c * RA
        xq = x_s[r0:r0 + RA, :]
        q = _dot(xq, wpt_s[0], NT)
        k = _dot(xq, wpt_s[1], NT)
        for j in range(NT_M):
            kl_s[j, HALO + r0:HALO + r0 + RA, :] = k[:, j * 128:(j + 1) * 128]
        v = _dot(xq, wpt_s[2], NT)
        for j in range(NT_M):
            vl_s[j, HALO + r0:HALO + r0 + RA, :] = v[:, j * 128:(j + 1) * 128]
        return [q[:, j * 128:(j + 1) * 128] * a_scale for j in range(NT_M)]

    def a_local_sub(r0, qt):
        logits = []
        for w in range(WIN):
            off = HALO + r0 - w * DIL
            s = None
            for j in range(NT_M):
                t = qt[j] * kl_s[j, off:off + RS, :]
                s = t if s is None else s + t
            s = s + pltpu.roll(s, 64, 1)
            s = s + pltpu.roll(s, 32, 1)
            if r0 < w * DIL:
                rowi = jax.lax.broadcasted_iota(jnp.int32, (RS, 128), 0)
                s = jnp.where(rowi + r0 >= w * DIL, s, NEG * LOG2E)
            logits.append(s)
        m = functools.reduce(jnp.maximum, logits)
        ps = [jnp.exp2(s - m) for s in logits]
        r = _recip(functools.reduce(jnp.add, ps))
        ot = []
        for j in range(NT_M):
            o = None
            for w in range(WIN):
                off = HALO + r0 - w * DIL
                t = ps[w] * vl_s[j, off:off + RS, :]
                o = t if o is None else o + t
            ot.append((o * r).astype(BF16))
        return jnp.concatenate(ot, axis=1)

    def a_local(c, qt):
        r0 = c * RA
        outs = []
        for sb in range(RA // RS):
            outs.append(a_local_sub(r0 + sb * RS, [q[sb * RS:(sb + 1) * RS] for q in qt]))
        return jnp.concatenate(outs, axis=0)

    def a_out(c, o):
        r0 = c * RA
        at = _dot(woapt_s[...], o, NT)
        acc_s[:, r0:r0 + RA] = at * g_s[0:1, r0:r0 + RA]

    def a_main():
        nca = S // RA
        st = {}
        a_xpose(0)
        for t in range(nca + 2):
            if t + 1 < nca:
                a_xpose(t + 1)
            if t < nca:
                st[t] = a_proj(t)
            if t == 0:
                a_prep_wo()
            if 0 <= t - 1 < nca:
                st[t - 1] = a_local(t - 1, st[t - 1])
            if 0 <= t - 2 < nca:
                a_out(t - 2, st.pop(t - 2))

    def group_weights(raw, g):
        cols = []
        for b in range(HG // 2):
            u = raw[g * (HG // 2) + b]
            cols.append(pltpu.bitcast(u << 16, F32).astype(BF16))
            cols.append(pltpu.bitcast(u & jnp.uint32(0xFFFF0000), F32).astype(BF16))
        return jnp.concatenate(cols, axis=1)

    b_scale = (D ** -0.5) * LOG2E

    def group_body(g, carry):
        def proj_body(rc, c2):
            r0 = pl.multiple_of(rc * RP, RP)
            wq = group_weights(wq_raw, g)
            wkv = jnp.concatenate([group_weights(wuk_raw, g), group_weights(wuv_raw, g)], axis=1)
            q = _dot(x_s[pl.ds(r0, RP), :], wq) * b_scale
            kv = _dot(c_s[pl.ds(r0, RP), :], wkv)
            for i in range(HG):
                q_s[i, pl.ds(r0, RP), :] = q[:, i * D:(i + 1) * D].astype(BF16)
                k_s[i, pl.ds(r0, RP), :] = kv[:, i * D:(i + 1) * D].astype(BF16)
                v_s[i, pl.ds(r0, RP), :] = kv[:, (HG + i) * D:(HG + i + 1) * D].astype(BF16)
            return c2

        with jax.named_scope("B_proj"):
            jax.lax.fori_loop(0, S // RP, proj_body, 0)

        def attn_body(it, c2):
            row = jax.lax.broadcasted_iota(jnp.int32, (TB, TB), 0)
            col = jax.lax.broadcasted_iota(jnp.int32, (TB, TB), 1)
            tri = col <= row
            items = [(u, r) for u in range(HU) for r in range(S // TQ)[::-1]]
            pend = {}
            for t in range(len(items) + 1):
                if t < len(items):
                    u, r = items[t]
                    hh = it * HU + u
                    pend[items[t]] = _attn_scores(q_s.at[hh], k_s.at[hh], r * TQ, tri)
                if t >= 1:
                    u, r = items[t - 1]
                    hh = it * HU + u
                    r0 = r * TQ
                    outs = _attn_values(v_s.at[hh], r0, *pend.pop(items[t - 1]))
                    for j, o in enumerate(outs):
                        ctx_s[g * HG + hh, r0 + j * TB:r0 + (j + 1) * TB, :] = o.astype(BF16)
            return c2

        with jax.named_scope("B_attn"):
            jax.lax.fori_loop(0, HG // HU, attn_body, 0)
        return carry

    def out_copy(i):
        r0 = i * RO
        if not isinstance(i, int):
            r0 = pl.multiple_of(r0, RO)
        return pltpu.make_async_copy(out_s.at[:, pl.ds(r0, RO)], out_hbm.at[0, :, pl.ds(r0, RO)], osems.at[i])

    def out_body(i, carry):
        r0 = pl.multiple_of(i * RO, RO)
        ctx = jnp.concatenate([ctx_s[h, pl.ds(r0, RO), :] for h in range(H)], axis=1)
        wo = jnp.concatenate([wob_s[h] for h in range(H)], axis=1)
        bt = _dot(wo, ctx, NT)
        omg = 1.0 - g_s[0:1, pl.ds(r0, RO)]
        out_s[:, pl.ds(r0, RO)] = (acc_s[:, pl.ds(r0, RO)] + omg * bt).astype(BF16)
        out_copy(i).start()
        return carry

    with jax.named_scope("A_prep"):
        a_prep()
    with jax.named_scope("A_main"):
        a_main()
        copies["c"].wait()
        for cp in pair_copies:
            cp.wait()
    jax.lax.fori_loop(0, NG, group_body, 0)
    with jax.named_scope("B_out"):
        copies["wob"].wait()
        jax.lax.fori_loop(0, S // RO, out_body, 0)
        for i in range(S // RO):
            out_copy(i).wait()


@jax.jit
def pallas_gated_mix__sliding_local_dilated__compressed_kv_cla__prompt_kernel(
    A_x: jax.Array,
    A_wqkv: jax.Array,
    A_wo: jax.Array,
    B_x: jax.Array,
    B_c_kv: jax.Array,
    B_w_q: jax.Array,
    B_w_uk: jax.Array,
    B_w_uv: jax.Array,
    B_w_o: jax.Array,
    gate_w: jax.Array,
):
    del B_x
    xt = jnp.swapaxes(A_x, 1, 2).reshape(M, S)
    c = B_c_kv.reshape(S, DC)
    wob = jnp.swapaxes(B_w_o, 1, 2)

    any_spec = pl.BlockSpec(memory_space=pl.ANY)
    scratch = [
        pltpu.VMEM((M, S), BF16),
        pltpu.VMEM((S, M), BF16),
        pltpu.VMEM((MP, 3 * M), BF16),
        pltpu.VMEM((M, M), BF16),
        pltpu.VMEM((S, DC), BF16),
        pltpu.VMEM((NPAIR, M, D), jnp.uint32),
        pltpu.VMEM((NPAIR, DC, D), jnp.uint32),
        pltpu.VMEM((NPAIR, DC, D), jnp.uint32),
        pltpu.VMEM((H, M, D), BF16),
        pltpu.VMEM((M,), BF16),
        pltpu.VMEM((NT_M, 14 * 128, 128), F32),
        pltpu.VMEM((3, MP, M), BF16),
        pltpu.VMEM((NT_M, M, 128), F32),
        pltpu.VMEM((MP, M), BF16),
        pltpu.VMEM((M, MP), BF16),
        pltpu.VMEM((NT_M, HALO + S, 128), F32),
        pltpu.VMEM((NT_M, HALO + S, 128), F32),
        pltpu.VMEM((M, S), F32),
        pltpu.VMEM((16, S), F32),
        pltpu.VMEM((HG, S, D), BF16),
        pltpu.VMEM((HG, S, D), BF16),
        pltpu.VMEM((HG, S, D), BF16),
        pltpu.VMEM((H, S, D), BF16),
        pltpu.VMEM((M, S), BF16),
        pltpu.SemaphoreType.DMA((6,)),
        pltpu.SemaphoreType.DMA((3 * NPAIR,)),
        pltpu.SemaphoreType.DMA((S // RO,)),
    ]
    out_t = pl.pallas_call(
        _kernel,
        out_shape=jax.ShapeDtypeStruct((1, M, S), BF16),
        in_specs=[any_spec] * 9,
        out_specs=any_spec,
        scratch_shapes=scratch,
        compiler_params=pltpu.CompilerParams(vmem_limit_bytes=120 * 1024 * 1024),
        name="gated_mix",
    )(xt, A_wqkv, A_wo, c, B_w_q, B_w_uk, B_w_uv, wob, gate_w)
    return jnp.swapaxes(out_t, 1, 2)
```

```python
import functools
import math

import jax
import jax.numpy as jnp
import jax.experimental.pallas as pl
import jax.experimental.pallas.tpu as pltpu

F32 = jnp.float32
BF16 = jnp.bfloat16

S = 2048
M = 576
MP = 640
NT_M = MP // 128
H = 32
D = 128
DC = 512
DHA = 18
WIN = 8
DIL = 2
HALO = 16
LOG2E = math.log2(math.e)
NEG = -1e9

RAP = 512
RA = 256
RS = 32
HG = 8
NG = H // HG
RP = 1024
TQ = 256
TB = 128
HU = 2
LAG = 1
RO = 256
assert NG * (S // RP) == S // RA
NSPLIT = 1
NPAIR = H // 2

NN = (((1,), (0,)), ((), ()))
NT = (((1,), (1,)), ((), ()))


def _dot(a, b, dims=NN):
    return jax.lax.dot_general(a, b, dims, preferred_element_type=F32)


def _lane_partial(s, op):
    acc = s[:, 0:128]
    for j in range(1, s.shape[1] // 128):
        acc = op(acc, s[:, j * 128:(j + 1) * 128])
    return acc


def _recip(l):
    r = pl.reciprocal(l, approx=True)
    return r * (2.0 - l * r)


def _segments(r0):
    nsub = TQ // TB
    segs = []
    if r0 > 0:
        segs.append((0, TQ, 0, r0, False))
    for j in range(nsub):
        segs.append((j * TB, (j + 1) * TB, r0 + j * TB, r0 + (j + 1) * TB, True))
        if (j + 1) * TB < TQ:
            segs.append(((j + 1) * TB, TQ, r0 + j * TB, r0 + (j + 1) * TB, False))
    return segs


def _attn_scores(q_ref, k_ref, r0, tri):
    nsub = TQ // TB
    segs = _segments(r0)
    ss = []
    for (a, b, c, d, msk) in segs:
        s = _dot(q_ref[r0 + a:r0 + b, :], k_ref[c:d, :], NT)
        if msk:
            s = jnp.where(tri, s, NEG * LOG2E)
        ss.append(s)
    ms = []
    for i in range(nsub):
        m = None
        for (a, b, c, d, msk), s in zip(segs, ss):
            if a <= i * TB and (i + 1) * TB <= b:
                sm = _lane_partial(s[i * TB - a:(i + 1) * TB - a], jnp.maximum)
                m = sm if m is None else jnp.maximum(m, sm)
        ms.append(jnp.max(m, axis=1, keepdims=True))
    return ss, ms


def _attn_values(v_ref, r0, ss, ms):
    nsub = TQ // TB
    segs = _segments(r0)
    ls = [None] * nsub
    os_ = [None] * nsub
    for (a, b, c, d, msk), s in zip(segs, ss):
        m = jnp.concatenate(ms[a // TB:b // TB], axis=0) if b - a > TB else ms[a // TB]
        p = jnp.exp2(s - m)
        l = _lane_partial(p, jnp.add)
        o = _dot(p.astype(BF16), v_ref[c:d, :])
        for i in range(a // TB, b // TB):
            li = l[i * TB - a:(i + 1) * TB - a]
            oi = o[i * TB - a:(i + 1) * TB - a]
            ls[i] = li if ls[i] is None else ls[i] + li
            os_[i] = oi if os_[i] is None else os_[i] + oi
    return [o * _recip(jnp.sum(l, axis=1, keepdims=True)) for o, l in zip(os_, ls)]


def attn_heads(qc_s, k_s, v_s, g, it):
    row = jax.lax.broadcasted_iota(jnp.int32, (TB, TB), 0)
    col = jax.lax.broadcasted_iota(jnp.int32, (TB, TB), 1)
    tri = col <= row
    items = [(u, r) for u in range(HU) for r in range(S // TQ)[::-1]]
    pend = {}
    done = {}

    def store(item):
        u, r = item
        for j, o in enumerate(done.pop(item)):
            r0 = r * TQ + j * TB
            qc_s[HG + g * HG + it * HU + u, r0:r0 + TB, :] = o.astype(BF16)

    for t in range(len(items) + 1):
        if t < len(items):
            u, r = items[t]
            hh = it * HU + u
            pend[items[t]] = _attn_scores(qc_s.at[hh], k_s.at[hh], r * TQ, tri)
        if t >= 1 + LAG:
            store(items[t - 1 - LAG])
        if t >= 1:
            u, r = items[t - 1]
            hh = it * HU + u
            done[items[t - 1]] = _attn_values(v_s.at[hh], r * TQ, *pend.pop(items[t - 1]))
    for item in list(done):
        store(item)


def _kernel(xt_hbm, wqkv_hbm, woa_hbm, c_hbm, wq_hbm, wuk_hbm, wuv_hbm, wob_hbm, gate_hbm,
            out_hbm,
            xt_s, x_s, wqkv_s, woa_s, c_s, wq_raw, wuk_raw, wuv_raw, wob_s, gate_s,
            wt_s, wpt_s, wof_s, woap_s, woapt_s, qa_s, kl_s, vl_s, oa_s, g_s,
            qc_s, k_s, v_s, out_s, sems, wsems, osems):
    copies = {
        "wqkv": pltpu.make_async_copy(wqkv_hbm, wqkv_s.at[pl.ds(0, M)], sems.at[0]),
        "x": pltpu.make_async_copy(xt_hbm, xt_s, sems.at[1]),
        "gate": pltpu.make_async_copy(gate_hbm, gate_s, sems.at[2]),
        "woa": pltpu.make_async_copy(woa_hbm, woa_s, sems.at[3]),
        "c": pltpu.make_async_copy(c_hbm, c_s, sems.at[4]),
        "wob": pltpu.make_async_copy(wob_hbm, wob_s, sems.at[5]),
    }
    def pair_copies(wi, j):
        w_hbm, raw = ((wq_hbm, wq_raw), (wuk_hbm, wuk_raw), (wuv_hbm, wuv_raw))[wi]
        n = w_hbm.shape[0] // NSPLIT
        return [pltpu.make_async_copy(
            w_hbm.bitcast(jnp.uint32).at[pl.ds(p * n, n), j, :], raw.at[j, pl.ds(p * n, n), :],
            wsems.at[wi * NPAIR + j]) for p in range(NSPLIT)]

    def group_copies(g):
        return [cp for b in range(HG // 2) for wi in range(3) for cp in pair_copies(wi, g * (HG // 2) + b)]

    copies["gate"].start(priority=0)
    copies["wqkv"].start(priority=0)
    for name in ("x", "woa"):
        copies[name].start(priority=1)

    def make_eye():
        return (jax.lax.broadcasted_iota(jnp.int32, (128, 128), 0)
                == jax.lax.broadcasted_iota(jnp.int32, (128, 128), 1)).astype(BF16)

    def a_prep():
        wqkv_s[M:MP, :] = jnp.zeros((MP - M, 3 * M), BF16)
        zero_halo = jnp.zeros((HALO, 128), F32)
        for j in range(NT_M):
            kl_s[j, 0:HALO, :] = zero_halo
            vl_s[j, 0:HALO, :] = zero_halo
        for sec in range(3):
            wpt_s[sec, M:MP, :] = jnp.zeros((MP - M, M), BF16)
        woap_s[M:MP, :] = jnp.zeros((MP - M, M), BF16)
        eye = make_eye()

        copies["wqkv"].wait()
        ncol = 3 * M
        for t in range(pl.cdiv(ncol, 128)):
            c0 = t * 128
            wd = min(128, ncol - c0)
            wt = _dot(eye[0:wd, 0:wd], wqkv_s[:, c0:c0 + wd], NT)
            for j in range(NT_M):
                wt_s[j, c0:c0 + wd, :] = wt[:, j * 128:(j + 1) * 128]
        for sec in range(3):
            for d in range(DHA):
                for j in range(NT_M):
                    rows = wt_s[j, pl.ds(sec * M + d, H, stride=DHA), :]
                    wj = min(128, M - j * 128)
                    wpt_s[sec, d * H:(d + 1) * H, j * 128:j * 128 + wj] = rows[:, 0:wj].astype(BF16)
        copies["x"].wait()
        copies["woa"].wait()
        copies["c"].start()
        for cp in group_copies(0):
            cp.start()
        copies["gate"].wait()

    def a_prep_wo():
        eye = make_eye()
        woa = woa_s[...].astype(F32)
        for j in range(NT_M):
            wj = min(128, M - j * 128)
            blk = woa[:, j * 128:j * 128 + wj]
            if wj < 128:
                blk = jnp.concatenate([blk, jnp.zeros((M, 128 - wj), F32)], axis=1)
            wof_s[j] = blk
        for d in range(DHA):
            for j in range(NT_M):
                wj = min(128, M - j * 128)
                rows = wof_s[j, pl.ds(d, H, stride=DHA), :]
                woap_s[d * H:(d + 1) * H, j * 128:j * 128 + wj] = rows[:, 0:wj].astype(BF16)
        for j in range(NT_M):
            wj = min(128, M - j * 128)
            woapt_s[j * 128:j * 128 + wj, :] = _dot(
                eye[0:wj, 0:wj], woap_s[:, j * 128:j * 128 + wj], NT).astype(BF16)

    def a_xpose():
        eye = make_eye()
        for t in range(S // 128):
            x_s[t * 128:(t + 1) * 128, :] = _dot(eye, xt_s[:, t * 128:(t + 1) * 128], NT).astype(BF16)
        gw = jnp.broadcast_to(gate_s[...].reshape(1, M), (16, M))
        g_s[...] = jax.nn.sigmoid(_dot(gw, xt_s[...]))

    a_scale = (DHA ** -0.5) * LOG2E

    def a_proj(c, carry):
        r0 = pl.multiple_of(c * RAP, RAP)
        rk = pl.multiple_of(HALO + c * RAP, HALO)
        xq = x_s[pl.ds(r0, RAP), :]
        q = _dot(xq, wpt_s[0], NT) * a_scale
        for j in range(NT_M):
            qa_s[j, pl.ds(r0, RAP), :] = q[:, j * 128:(j + 1) * 128]
        k = _dot(xq, wpt_s[1], NT)
        for j in range(NT_M):
            kl_s[j, pl.ds(rk, RAP), :] = k[:, j * 128:(j + 1) * 128]
        v = _dot(xq, wpt_s[2], NT)
        for j in range(NT_M):
            vl_s[j, pl.ds(rk, RAP), :] = v[:, j * 128:(j + 1) * 128]
        return carry

    def a_local(r0):
        qv = [qa_s.at[j, pl.ds(r0, RA), :] for j in range(NT_M)]
        kv = [kl_s.at[j, pl.ds(r0, HALO + RA), :] for j in range(NT_M)]
        vv = [vl_s.at[j, pl.ds(r0, HALO + RA), :] for j in range(NT_M)]
        for sb in range(RA // RS):
            b0 = sb * RS
            qt = [qv[j][b0:b0 + RS, :] for j in range(NT_M)]
            logits = []
            for w in range(WIN):
                off = HALO + b0 - w * DIL
                s = None
                for j in range(NT_M):
                    t = qt[j] * kv[j][off:off + RS, :]
                    s = t if s is None else s + t
                s = s + pltpu.roll(s, 64, 1)
                s = s + pltpu.roll(s, 32, 1)
                if b0 < w * DIL:
                    rowi = jax.lax.broadcasted_iota(jnp.int32, (RS, 128), 0) + (r0 + b0)
                    s = jnp.where(rowi >= w * DIL, s, NEG * LOG2E)
                logits.append(s)
            m = functools.reduce(jnp.maximum, logits)
            ps = [jnp.exp2(s - m) for s in logits]
            r = _recip(functools.reduce(jnp.add, ps))
            ot = []
            for j in range(NT_M):
                o = None
                for w in range(WIN):
                    off = HALO + b0 - w * DIL
                    t = ps[w] * vv[j][off:off + RS, :]
                    o = t if o is None else o + t
                ot.append((o * r).astype(BF16))
            oa_s[pl.ds(pl.multiple_of(r0 + b0, RS), RS), :] = jnp.concatenate(ot, axis=1)

    def a_main():
        a_xpose()
        a_prep_wo()
        jax.lax.fori_loop(0, S // RAP, a_proj, 0)

    def group_weights(raw, g):
        cols = []
        for b in range(HG // 2):
            u = raw[g * (HG // 2) + b]
            cols.append(pltpu.bitcast(u << 16, F32).astype(BF16))
            cols.append(pltpu.bitcast(u & jnp.uint32(0xFFFF0000), F32).astype(BF16))
        return jnp.concatenate(cols, axis=1)

    b_scale = (D ** -0.5) * LOG2E

    def group_body(g, carry):
        @pl.when(g > 0)
        def _():
            for cp in group_copies(g):
                cp.wait()

        def proj_body(rc, c2):
            r0 = pl.multiple_of(rc * RP, RP)
            wq = group_weights(wq_raw, g)
            wkv = jnp.concatenate([group_weights(wuk_raw, g), group_weights(wuv_raw, g)], axis=1)
            q = _dot(x_s[pl.ds(r0, RP), :], wq) * b_scale
            kv = _dot(c_s[pl.ds(r0, RP), :], wkv)
            for i in range(HG):
                qc_s[i, pl.ds(r0, RP), :] = q[:, i * D:(i + 1) * D].astype(BF16)
                k_s[i, pl.ds(r0, RP), :] = kv[:, i * D:(i + 1) * D].astype(BF16)
                v_s[i, pl.ds(r0, RP), :] = kv[:, (HG + i) * D:(HG + i + 1) * D].astype(BF16)
            a_local(pl.multiple_of((g * (S // RP) + rc) * RA, RA))
            return c2

        with jax.named_scope("B_proj"):
            jax.lax.fori_loop(0, S // RP, proj_body, 0)

        def attn_body(it, c2):
            attn_heads(qc_s, k_s, v_s, g, it)
            return c2

        with jax.named_scope("B_attn"):
            jax.lax.fori_loop(0, HG // HU, attn_body, 0)
        return carry

    def out_copy(i):
        r0 = i * RO
        if not isinstance(i, int):
            r0 = pl.multiple_of(r0, RO)
        return pltpu.make_async_copy(out_s.at[:, pl.ds(r0, RO)], out_hbm.at[0, :, pl.ds(r0, RO)], osems.at[i])

    def out_body(i, carry):
        r0 = pl.multiple_of(i * RO, RO)
        ctx = jnp.concatenate([qc_s[HG + h, pl.ds(r0, RO), :] for h in range(H)], axis=1)
        wo = jnp.concatenate([wob_s[h] for h in range(H)], axis=1)
        bt = _dot(wo, ctx, NT)
        at = _dot(woapt_s[...], oa_s[pl.ds(r0, RO), :], NT)
        gt = g_s[0:1, pl.ds(r0, RO)]
        out_s[:, pl.ds(r0, RO)] = (gt * at + (1.0 - gt) * bt).astype(BF16)
        out_copy(i).start()
        return carry

    with jax.named_scope("A_prep"):
        a_prep()
    with jax.named_scope("A_main"):
        a_main()
        copies["c"].wait()
        for cp in group_copies(0):
            cp.wait()
        for g in range(1, NG):
            for cp in group_copies(g):
                cp.start()
        copies["wob"].start()
    jax.lax.fori_loop(0, NG, group_body, 0)
    with jax.named_scope("B_out"):
        copies["wob"].wait()
        jax.lax.fori_loop(0, S // RO, out_body, 0)
        for i in range(S // RO):
            out_copy(i).wait()


@jax.jit
def pallas_gated_mix__sliding_local_dilated__compressed_kv_cla__prompt_kernel(
    A_x: jax.Array,
    A_wqkv: jax.Array,
    A_wo: jax.Array,
    B_x: jax.Array,
    B_c_kv: jax.Array,
    B_w_q: jax.Array,
    B_w_uk: jax.Array,
    B_w_uv: jax.Array,
    B_w_o: jax.Array,
    gate_w: jax.Array,
):
    del B_x
    xt = jnp.swapaxes(A_x, 1, 2).reshape(M, S)
    c = B_c_kv.reshape(S, DC)
    wob = jnp.swapaxes(B_w_o, 1, 2)

    any_spec = pl.BlockSpec(memory_space=pl.ANY)
    scratch = [
        pltpu.VMEM((M, S), BF16),
        pltpu.VMEM((S, M), BF16),
        pltpu.VMEM((MP, 3 * M), BF16),
        pltpu.VMEM((M, M), BF16),
        pltpu.VMEM((S, DC), BF16),
        pltpu.VMEM((NPAIR, M, D), jnp.uint32),
        pltpu.VMEM((NPAIR, DC, D), jnp.uint32),
        pltpu.VMEM((NPAIR, DC, D), jnp.uint32),
        pltpu.VMEM((H, M, D), BF16),
        pltpu.VMEM((M,), BF16),
        pltpu.VMEM((NT_M, 14 * 128, 128), F32),
        pltpu.VMEM((3, MP, M), BF16),
        pltpu.VMEM((NT_M, M, 128), F32),
        pltpu.VMEM((MP, M), BF16),
        pltpu.VMEM((M, MP), BF16),
        pltpu.VMEM((NT_M, S, 128), F32),
        pltpu.VMEM((NT_M, HALO + S, 128), F32),
        pltpu.VMEM((NT_M, HALO + S, 128), F32),
        pltpu.VMEM((S, MP), BF16),
        pltpu.VMEM((16, S), F32),
        pltpu.VMEM((HG + H, S, D), BF16),
        pltpu.VMEM((HG, S, D), BF16),
        pltpu.VMEM((HG, S, D), BF16),
        pltpu.VMEM((M, S), BF16),
        pltpu.SemaphoreType.DMA((6,)),
        pltpu.SemaphoreType.DMA((3 * NPAIR,)),
        pltpu.SemaphoreType.DMA((S // RO,)),
    ]
    out_t = pl.pallas_call(
        _kernel,
        out_shape=jax.ShapeDtypeStruct((1, M, S), BF16),
        in_specs=[any_spec] * 9,
        out_specs=any_spec,
        scratch_shapes=scratch,
        compiler_params=pltpu.CompilerParams(vmem_limit_bytes=120 * 1024 * 1024),
        name="gated_mix",
    )(xt, A_wqkv, A_wo, c, B_w_q, B_w_uk, B_w_uv, wob, gate_w)
    return jnp.swapaxes(out_t, 1, 2)
```

```python
import functools
import math

import jax
import jax.numpy as jnp
import jax.experimental.pallas as pl
import jax.experimental.pallas.tpu as pltpu

F32 = jnp.float32
BF16 = jnp.bfloat16

S = 2048
M = 576
MP = 640
NT_M = MP // 128
H = 32
D = 128
DC = 512
DHA = 18
WIN = 8
DIL = 2
HALO = 16
DF = 16
NPK = 14
LOG2E = math.log2(math.e)
NEG = -1e9

RAP = 512
RA = 256
RS = 32
HG = 8
NG = H // HG
RP = 1024
TQ = 256
TB = 128
HU = 2
BLOCK_ORDER = ((1, 3, 7, 6, 5, 4, 2, 0), (6, 7, 4, 5, 2, 3, 1, 0))
assert all(sorted(o) == list(range(S // TQ)) for o in BLOCK_ORDER) and len(BLOCK_ORDER) == HU
LAG = 1
RO = 256
assert NG * (S // RP) == S // RA
NSPLIT = 1
NPAIR = H // 2

NN = (((1,), (0,)), ((), ()))
NT = (((1,), (1,)), ((), ()))


def _dot(a, b, dims=NN):
    return jax.lax.dot_general(a, b, dims, preferred_element_type=F32)


def _packed_row(sec, d):
    if d < DF:
        return (sec * DF + d) * H
    return 3 * DF * H + ((0, 4, 2)[sec] + d - DF) * H


def _lane_partial(s, op):
    acc = s[:, 0:128]
    for j in range(1, s.shape[1] // 128):
        acc = op(acc, s[:, j * 128:(j + 1) * 128])
    return acc


def _recip(l):
    r = pl.reciprocal(l, approx=True)
    return r * (2.0 - l * r)


def _segments(r0):
    nsub = TQ // TB
    segs = []
    if r0 > 0:
        segs.append((0, TQ, 0, r0, False))
    for j in range(nsub):
        segs.append((j * TB, (j + 1) * TB, r0 + j * TB, r0 + (j + 1) * TB, True))
        if (j + 1) * TB < TQ:
            segs.append(((j + 1) * TB, TQ, r0 + j * TB, r0 + (j + 1) * TB, False))
    return segs


def _attn_scores(q_ref, k_ref, r0, tri):
    nsub = TQ // TB
    segs = _segments(r0)
    ss = []
    for (a, b, c, d, msk) in segs:
        s = _dot(q_ref[r0 + a:r0 + b, :], k_ref[c:d, :], NT)
        if msk:
            s = jnp.where(tri, s, NEG * LOG2E)
        ss.append(s)
    ms = []
    for i in range(nsub):
        m = None
        for (a, b, c, d, msk), s in zip(segs, ss):
            if a <= i * TB and (i + 1) * TB <= b:
                sm = _lane_partial(s[i * TB - a:(i + 1) * TB - a], jnp.maximum)
                m = sm if m is None else jnp.maximum(m, sm)
        ms.append(jnp.max(m, axis=1, keepdims=True))
    return ss, ms


def _attn_values(v_ref, r0, ss, ms):
    nsub = TQ // TB
    segs = _segments(r0)
    ls = [None] * nsub
    os_ = [None] * nsub
    for (a, b, c, d, msk), s in zip(segs, ss):
        m = jnp.concatenate(ms[a // TB:b // TB], axis=0) if b - a > TB else ms[a // TB]
        p = jnp.exp2(s - m)
        l = _lane_partial(p, jnp.add)
        o = _dot(p.astype(BF16), v_ref[c:d, :])
        for i in range(a // TB, b // TB):
            li = l[i * TB - a:(i + 1) * TB - a]
            oi = o[i * TB - a:(i + 1) * TB - a]
            ls[i] = li if ls[i] is None else ls[i] + li
            os_[i] = oi if os_[i] is None else os_[i] + oi
    return [o * _recip(jnp.sum(l, axis=1, keepdims=True)) for o, l in zip(os_, ls)]


def attn_heads(qc_s, k_s, v_s, g, it):
    row = jax.lax.broadcasted_iota(jnp.int32, (TB, TB), 0)
    col = jax.lax.broadcasted_iota(jnp.int32, (TB, TB), 1)
    tri = col <= row
    items = [(u, r) for u in range(HU) for r in BLOCK_ORDER[u]]
    pend = {}
    done = {}

    def store(item):
        u, r = item
        for j, o in enumerate(done.pop(item)):
            r0 = r * TQ + j * TB
            qc_s[HG + g * HG + it * HU + u, r0:r0 + TB, :] = o.astype(BF16)

    for t in range(len(items) + 1):
        if t < len(items):
            u, r = items[t]
            hh = it * HU + u
            pend[items[t]] = _attn_scores(qc_s.at[hh], k_s.at[hh], r * TQ, tri)
        if t >= 1 + LAG:
            store(items[t - 1 - LAG])
        if t >= 1:
            u, r = items[t - 1]
            hh = it * HU + u
            done[items[t - 1]] = _attn_values(v_s.at[hh], r * TQ, *pend.pop(items[t - 1]))
    for item in list(done):
        store(item)


def _kernel(xt_hbm, wqkv_hbm, woa_hbm, c_hbm, wq_hbm, wuk_hbm, wuv_hbm, wob_hbm, gate_hbm,
            out_hbm,
            xt_s, x_s, wqkv_s, woa_s, c_s, wq_raw, wuk_raw, wuv_raw, wob_s, gate_s,
            wt_s, wpt_s, wof_s, woap_s, woapt_s, qa_s, kl_s, vl_s, oa_s, g_s,
            qc_s, k_s, v_s, out_s, sems, wsems, osems):
    copies = {
        "wqkv": pltpu.make_async_copy(wqkv_hbm, wqkv_s.at[pl.ds(0, M)], sems.at[0]),
        "x": pltpu.make_async_copy(xt_hbm, xt_s, sems.at[1]),
        "gate": pltpu.make_async_copy(gate_hbm, gate_s, sems.at[2]),
        "woa": pltpu.make_async_copy(woa_hbm, woa_s, sems.at[3]),
        "c": pltpu.make_async_copy(c_hbm, c_s, sems.at[4]),
        "wob": pltpu.make_async_copy(wob_hbm, wob_s, sems.at[5]),
    }
    def pair_copies(wi, j):
        w_hbm, raw = ((wq_hbm, wq_raw), (wuk_hbm, wuk_raw), (wuv_hbm, wuv_raw))[wi]
        n = w_hbm.shape[0] // NSPLIT
        return [pltpu.make_async_copy(
            w_hbm.bitcast(jnp.uint32).at[pl.ds(p * n, n), j, :], raw.at[j, pl.ds(p * n, n), :],
            wsems.at[wi * NPAIR + j]) for p in range(NSPLIT)]

    def group_copies(g):
        return [cp for b in range(HG // 2) for wi in range(3) for cp in pair_copies(wi, g * (HG // 2) + b)]

    copies["gate"].start(priority=0)
    copies["wqkv"].start(priority=0)
    for name in ("x", "woa"):
        copies[name].start(priority=1)

    def make_eye():
        return (jax.lax.broadcasted_iota(jnp.int32, (128, 128), 0)
                == jax.lax.broadcasted_iota(jnp.int32, (128, 128), 1)).astype(BF16)

    def a_prep():
        wqkv_s[M:MP, :] = jnp.zeros((MP - M, 3 * M), BF16)
        zero_halo = jnp.zeros((HALO, 128), F32)
        for j in range(NT_M):
            kl_s[j, 0:HALO, :] = zero_halo
            vl_s[j, 0:HALO, :] = zero_halo
        wpt_s[3 * M:NPK * 128, :] = jnp.zeros((NPK * 128 - 3 * M, M), BF16)
        woap_s[DF * H:DF * H + 64, :] = jnp.zeros((64, M), BF16)
        eye = make_eye()

        copies["wqkv"].wait()
        ncol = 3 * M
        for t in range(pl.cdiv(ncol, 128)):
            c0 = t * 128
            wd = min(128, ncol - c0)
            wt = _dot(eye[0:wd, 0:wd], wqkv_s[:, c0:c0 + wd], NT)
            for j in range(NT_M):
                wt_s[j, c0:c0 + wd, :] = wt[:, j * 128:(j + 1) * 128]
        for sec in range(3):
            for d in range(DHA):
                for j in range(NT_M):
                    rows = wt_s[j, pl.ds(sec * M + d, H, stride=DHA), :]
                    wj = min(128, M - j * 128)
                    p0 = _packed_row(sec, d)
                    wpt_s[p0:p0 + H, j * 128:j * 128 + wj] = rows[:, 0:wj].astype(BF16)
        copies["x"].wait()
        copies["woa"].wait()
        copies["c"].start()
        for cp in group_copies(0):
            cp.start()
        copies["gate"].wait()

    def a_prep_wo():
        eye = make_eye()
        woa = woa_s[...].astype(F32)
        for j in range(NT_M):
            wj = min(128, M - j * 128)
            blk = woa[:, j * 128:j * 128 + wj]
            if wj < 128:
                blk = jnp.concatenate([blk, jnp.zeros((M, 128 - wj), F32)], axis=1)
            wof_s[j] = blk
        for d in range(DHA):
            for j in range(NT_M):
                wj = min(128, M - j * 128)
                rows = wof_s[j, pl.ds(d, H, stride=DHA), :]
                p0 = d * H if d < DF else d * H + 64
                woap_s[p0:p0 + H, j * 128:j * 128 + wj] = rows[:, 0:wj].astype(BF16)
        for j in range(NT_M):
            wj = min(128, M - j * 128)
            woapt_s[j * 128:j * 128 + wj, :] = _dot(
                eye[0:wj, 0:wj], woap_s[:, j * 128:j * 128 + wj], NT).astype(BF16)

    def a_xpose():
        eye = make_eye()
        for t in range(S // 128):
            x_s[t * 128:(t + 1) * 128, :] = _dot(eye, xt_s[:, t * 128:(t + 1) * 128], NT).astype(BF16)
        gw = jnp.broadcast_to(gate_s[...].reshape(1, M), (16, M))
        g_s[...] = jax.nn.sigmoid(_dot(gw, xt_s[...]))

    a_scale = (DHA ** -0.5) * LOG2E

    def a_proj(c, carry):
        r0 = pl.multiple_of(c * RAP, RAP)
        rk = pl.multiple_of(HALO + c * RAP, HALO)
        xq = x_s[pl.ds(r0, RAP), :]
        nf = DF * H
        q = _dot(xq, wpt_s[0:nf, :], NT)
        for j in range(NT_M - 1):
            qa_s[j, pl.ds(r0, RAP), :] = q[:, j * 128:(j + 1) * 128]
        k = _dot(xq, wpt_s[nf:2 * nf, :], NT) * a_scale
        for j in range(NT_M - 1):
            kl_s[j, pl.ds(rk, RAP), :] = k[:, j * 128:(j + 1) * 128]
        v = _dot(xq, wpt_s[2 * nf:3 * nf, :], NT)
        for j in range(NT_M - 1):
            vl_s[j, pl.ds(rk, RAP), :] = v[:, j * 128:(j + 1) * 128]
        t = _dot(xq, wpt_s[3 * nf:NPK * 128, :], NT)
        vl_s[NT_M - 1, pl.ds(rk, RAP), :] = t[:, 0:128]
        kl_s[NT_M - 1, pl.ds(rk, RAP), :] = t[:, 128:256] * a_scale
        return carry

    def a_local(r0):
        qv = [qa_s.at[j, pl.ds(r0, RA), :] for j in range(NT_M - 1)]
        kv = [kl_s.at[j, pl.ds(r0, HALO + RA), :] for j in range(NT_M)]
        vv = [vl_s.at[j, pl.ds(r0, HALO + RA), :] for j in range(NT_M)]
        for sb in range(RA // RS):
            b0 = sb * RS
            qt = [qv[j][b0:b0 + RS, :] for j in range(NT_M - 1)]
            qt.append(vv[NT_M - 1][HALO + b0:HALO + b0 + RS, :])
            logits = []
            for w in range(WIN):
                off = HALO + b0 - w * DIL
                s = None
                for j in range(NT_M):
                    t = qt[j] * kv[j][off:off + RS, :]
                    s = t if s is None else s + t
                s = s + pltpu.roll(s, 64, 1)
                s = s + pltpu.roll(s, 32, 1)
                if b0 < w * DIL:
                    rowi = jax.lax.broadcasted_iota(jnp.int32, (RS, 128), 0) + (r0 + b0)
                    s = jnp.where(rowi >= w * DIL, s, NEG * LOG2E)
                logits.append(s)
            m = functools.reduce(jnp.maximum, logits)
            ps = [jnp.exp2(s - m) for s in logits]
            r = _recip(functools.reduce(jnp.add, ps))
            ot = []
            for j in range(NT_M):
                o = None
                for w in range(WIN):
                    off = HALO + b0 - w * DIL
                    t = ps[w] * vv[j][off:off + RS, :]
                    o = t if o is None else o + t
                ot.append((o * r).astype(BF16))
            oa_s[pl.ds(pl.multiple_of(r0 + b0, RS), RS), :] = jnp.concatenate(ot, axis=1)

    def a_main():
        a_xpose()
        a_prep_wo()
        jax.lax.fori_loop(0, S // RAP, a_proj, 0)

    def group_weights(raw, g):
        cols = []
        for b in range(HG // 2):
            u = raw[g * (HG // 2) + b]
            cols.append(pltpu.bitcast(u << 16, F32).astype(BF16))
            cols.append(pltpu.bitcast(u & jnp.uint32(0xFFFF0000), F32).astype(BF16))
        return jnp.concatenate(cols, axis=1)

    b_scale = (D ** -0.5) * LOG2E

    def group_body(g, carry):
        @pl.when(g > 0)
        def _():
            for cp in group_copies(g):
                cp.wait()

        def proj_body(rc, c2):
            r0 = pl.multiple_of(rc * RP, RP)
            wq = group_weights(wq_raw, g)
            wkv = jnp.concatenate([group_weights(wuk_raw, g), group_weights(wuv_raw, g)], axis=1)
            q = _dot(x_s[pl.ds(r0, RP), :], wq) * b_scale
            kv = _dot(c_s[pl.ds(r0, RP), :], wkv)
            for i in range(HG):
                qc_s[i, pl.ds(r0, RP), :] = q[:, i * D:(i + 1) * D].astype(BF16)
                k_s[i, pl.ds(r0, RP), :] = kv[:, i * D:(i + 1) * D].astype(BF16)
                v_s[i, pl.ds(r0, RP), :] = kv[:, (HG + i) * D:(HG + i + 1) * D].astype(BF16)
            a_local(pl.multiple_of((g * (S // RP) + rc) * RA, RA))
            return c2

        with jax.named_scope("B_proj"):
            jax.lax.fori_loop(0, S // RP, proj_body, 0)

        def attn_body(it, c2):
            attn_heads(qc_s, k_s, v_s, g, it)
            return c2

        with jax.named_scope("B_attn"):
            jax.lax.fori_loop(0, HG // HU, attn_body, 0)
        return carry

    def out_copy(i):
        r0 = i * RO
        if not isinstance(i, int):
            r0 = pl.multiple_of(r0, RO)
        return pltpu.make_async_copy(out_s.at[:, pl.ds(r0, RO)], out_hbm.at[0, :, pl.ds(r0, RO)], osems.at[i])

    def out_body(i, carry):
        r0 = pl.multiple_of(i * RO, RO)
        ctx = jnp.concatenate([qc_s[HG + h, pl.ds(r0, RO), :] for h in range(H)], axis=1)
        wo = jnp.concatenate([wob_s[h] for h in range(H)], axis=1)
        bt = _dot(wo, ctx, NT)
        at = _dot(woapt_s[...], oa_s[pl.ds(r0, RO), :], NT)
        gt = g_s[0:1, pl.ds(r0, RO)]
        out_s[:, pl.ds(r0, RO)] = (gt * at + (1.0 - gt) * bt).astype(BF16)
        out_copy(i).start()
        return carry

    with jax.named_scope("A_prep"):
        a_prep()
    with jax.named_scope("A_main"):
        a_main()
        copies["c"].wait()
        for cp in group_copies(0):
            cp.wait()
        for g in range(1, NG):
            for cp in group_copies(g):
                cp.start()
        copies["wob"].start()
    jax.lax.fori_loop(0, NG, group_body, 0)
    with jax.named_scope("B_out"):
        copies["wob"].wait()
        jax.lax.fori_loop(0, S // RO, out_body, 0)
        for i in range(S // RO):
            out_copy(i).wait()


@jax.jit
def pallas_gated_mix__sliding_local_dilated__compressed_kv_cla__prompt_kernel(
    A_x: jax.Array,
    A_wqkv: jax.Array,
    A_wo: jax.Array,
    B_x: jax.Array,
    B_c_kv: jax.Array,
    B_w_q: jax.Array,
    B_w_uk: jax.Array,
    B_w_uv: jax.Array,
    B_w_o: jax.Array,
    gate_w: jax.Array,
):
    del B_x
    xt = jnp.swapaxes(A_x, 1, 2).reshape(M, S)
    c = B_c_kv.reshape(S, DC)
    wob = jnp.swapaxes(B_w_o, 1, 2)

    any_spec = pl.BlockSpec(memory_space=pl.ANY)
    scratch = [
        pltpu.VMEM((M, S), BF16),
        pltpu.VMEM((S, M), BF16),
        pltpu.VMEM((MP, 3 * M), BF16),
        pltpu.VMEM((M, M), BF16),
        pltpu.VMEM((S, DC), BF16),
        pltpu.VMEM((NPAIR, M, D), jnp.uint32),
        pltpu.VMEM((NPAIR, DC, D), jnp.uint32),
        pltpu.VMEM((NPAIR, DC, D), jnp.uint32),
        pltpu.VMEM((H, M, D), BF16),
        pltpu.VMEM((M,), BF16),
        pltpu.VMEM((NT_M, 14 * 128, 128), F32),
        pltpu.VMEM((NPK * 128, M), BF16),
        pltpu.VMEM((NT_M, M, 128), F32),
        pltpu.VMEM((MP, M), BF16),
        pltpu.VMEM((M, MP), BF16),
        pltpu.VMEM((NT_M - 1, S, 128), F32),
        pltpu.VMEM((NT_M, HALO + S, 128), F32),
        pltpu.VMEM((NT_M, HALO + S, 128), F32),
        pltpu.VMEM((S, MP), BF16),
        pltpu.VMEM((16, S), F32),
        pltpu.VMEM((HG + H, S, D), BF16),
        pltpu.VMEM((HG, S, D), BF16),
        pltpu.VMEM((HG, S, D), BF16),
        pltpu.VMEM((M, S), BF16),
        pltpu.SemaphoreType.DMA((6,)),
        pltpu.SemaphoreType.DMA((3 * NPAIR,)),
        pltpu.SemaphoreType.DMA((S // RO,)),
    ]
    out_t = pl.pallas_call(
        _kernel,
        out_shape=jax.ShapeDtypeStruct((1, M, S), BF16),
        in_specs=[any_spec] * 9,
        out_specs=any_spec,
        scratch_shapes=scratch,
        compiler_params=pltpu.CompilerParams(vmem_limit_bytes=120 * 1024 * 1024),
        name="gated_mix",
    )(xt, A_wqkv, A_wo, c, B_w_q, B_w_uk, B_w_uv, wob, gate_w)
    return jnp.swapaxes(out_t, 1, 2)
```

```python
import functools
import math

import jax
import jax.numpy as jnp
import jax.experimental.pallas as pl
import jax.experimental.pallas.tpu as pltpu

F32 = jnp.float32
BF16 = jnp.bfloat16

S = 2048
M = 576
MP = 640
NT_M = MP // 128
H = 32
D = 128
DC = 512
DHA = 18
WIN = 8
DIL = 2
HALO = 16
DF = 16
NPK = 14
LOG2E = math.log2(math.e)
NEG = -1e9

RAP = 512
RA = 256
RS = 32
HG = 8
NG = H // HG
RP = 1024
TQ = 256
TB = 128
HU = 2
BLOCK_ORDER = ((1, 3, 7, 6, 5, 4, 2, 0), (6, 7, 4, 5, 2, 3, 1, 0))
assert all(sorted(o) == list(range(S // TQ)) for o in BLOCK_ORDER) and len(BLOCK_ORDER) == HU
PSPLIT = 1
DYNZ = 0
PROJ_SEQ = "kvq01234567"
LAG = 1
RO = 256
assert NG * (S // RP) == S // RA
NSPLIT = 1
NPAIR = H // 2

NN = (((1,), (0,)), ((), ()))
NT = (((1,), (1,)), ((), ()))


def _dot(a, b, dims=NN):
    return jax.lax.dot_general(a, b, dims, preferred_element_type=F32)


def _packed_row(sec, d):
    if d < DF:
        return (sec * DF + d) * H
    return 3 * DF * H + ((0, 4, 2)[sec] + d - DF) * H


def _lane_partial(s, op):
    acc = s[:, 0:128]
    for j in range(1, s.shape[1] // 128):
        acc = op(acc, s[:, j * 128:(j + 1) * 128])
    return acc


def _recip(l):
    r = pl.reciprocal(l, approx=True)
    return r * (2.0 - l * r)


def _segments(r0):
    nsub = TQ // TB
    segs = []
    if r0 > 0:
        segs.append((0, TQ, 0, r0, False))
    for j in range(nsub):
        segs.append((j * TB, (j + 1) * TB, r0 + j * TB, r0 + (j + 1) * TB, True))
        if (j + 1) * TB < TQ:
            segs.append(((j + 1) * TB, TQ, r0 + j * TB, r0 + (j + 1) * TB, False))
    return segs


def _attn_scores(q_ref, k_ref, r0, tri):
    nsub = TQ // TB
    segs = _segments(r0)
    ss = []
    for (a, b, c, d, msk) in segs:
        s = _dot(q_ref[r0 + a:r0 + b, :], k_ref[c:d, :], NT)
        if msk:
            s = jnp.where(tri, s, NEG * LOG2E)
        ss.append(s)
    ms = []
    for i in range(nsub):
        m = None
        for (a, b, c, d, msk), s in zip(segs, ss):
            if a <= i * TB and (i + 1) * TB <= b:
                sm = _lane_partial(s[i * TB - a:(i + 1) * TB - a], jnp.maximum)
                m = sm if m is None else jnp.maximum(m, sm)
        ms.append(jnp.max(m, axis=1, keepdims=True))
    return ss, ms


def _attn_values(v_ref, r0, ss, ms):
    nsub = TQ // TB
    segs = _segments(r0)
    ls = [None] * nsub
    os_ = [None] * nsub
    for (a, b, c, d, msk), s in zip(segs, ss):
        m = jnp.concatenate(ms[a // TB:b // TB], axis=0) if b - a > TB else ms[a // TB]
        p = jnp.exp2(s - m)
        l = _lane_partial(p, jnp.add)
        o = _dot(p.astype(BF16), v_ref[c:d, :])
        for i in range(a // TB, b // TB):
            li = l[i * TB - a:(i + 1) * TB - a]
            oi = o[i * TB - a:(i + 1) * TB - a]
            ls[i] = li if ls[i] is None else ls[i] + li
            os_[i] = oi if os_[i] is None else os_[i] + oi
    return [o * _recip(jnp.sum(l, axis=1, keepdims=True)) for o, l in zip(os_, ls)]


def attn_heads(qc_s, k_s, v_s, g, it):
    row = jax.lax.broadcasted_iota(jnp.int32, (TB, TB), 0)
    col = jax.lax.broadcasted_iota(jnp.int32, (TB, TB), 1)
    tri = col <= row
    items = [(u, r) for u in range(HU) for r in BLOCK_ORDER[u]]
    pend = {}
    done = {}

    def store(item):
        u, r = item
        for j, o in enumerate(done.pop(item)):
            r0 = r * TQ + j * TB
            qc_s[HG + g * HG + it * HU + u, r0:r0 + TB, :] = o.astype(BF16)

    for t in range(len(items) + 1):
        if t < len(items):
            u, r = items[t]
            hh = it * HU + u
            pend[items[t]] = _attn_scores(qc_s.at[hh], k_s.at[hh], r * TQ, tri)
        if t >= 1 + LAG:
            store(items[t - 1 - LAG])
        if t >= 1:
            u, r = items[t - 1]
            hh = it * HU + u
            done[items[t - 1]] = _attn_values(v_s.at[hh], r * TQ, *pend.pop(items[t - 1]))
    for item in list(done):
        store(item)


def _kernel(xt_hbm, wqkv_hbm, woa_hbm, c_hbm, wq_hbm, wuk_hbm, wuv_hbm, wob_hbm, gate_hbm,
            out_hbm,
            xt_s, x_s, wqkv_s, woa_s, c_s, wq_raw, wuk_raw, wuv_raw, wob_s, gate_s,
            wt_s, wpt_s, wof_s, woap_s, woapt_s, qa_s, kl_s, vl_s, g_s,
            qc_s, k_s, v_s, out_s, sems, wsems, osems):
    copies = {
        "wqkv": pltpu.make_async_copy(wqkv_hbm, wqkv_s.at[pl.ds(0, M)], sems.at[0]),
        "x": pltpu.make_async_copy(xt_hbm, xt_s, sems.at[1]),
        "gate": pltpu.make_async_copy(gate_hbm, gate_s, sems.at[2]),
        "woa": pltpu.make_async_copy(woa_hbm, woa_s, sems.at[3]),
        "c": pltpu.make_async_copy(c_hbm, c_s, sems.at[4]),
        "wob": pltpu.make_async_copy(wob_hbm, wob_s, sems.at[5]),
    }
    def pair_copies(wi, j):
        w_hbm, raw = ((wq_hbm, wq_raw), (wuk_hbm, wuk_raw), (wuv_hbm, wuv_raw))[wi]
        n = w_hbm.shape[0] // NSPLIT
        return [pltpu.make_async_copy(
            w_hbm.bitcast(jnp.uint32).at[pl.ds(p * n, n), j, :], raw.at[j, pl.ds(p * n, n), :],
            wsems.at[wi * NPAIR + j]) for p in range(NSPLIT)]

    def group_copies(g):
        return [cp for b in range(HG // 2) for wi in range(3) for cp in pair_copies(wi, g * (HG // 2) + b)]

    copies["gate"].start(priority=0)
    copies["wqkv"].start(priority=0)
    for name in ("x", "woa"):
        copies[name].start(priority=1)

    def make_eye():
        return (jax.lax.broadcasted_iota(jnp.int32, (128, 128), 0)
                == jax.lax.broadcasted_iota(jnp.int32, (128, 128), 1)).astype(BF16)

    def a_prep():
        wqkv_s[M:MP, :] = jnp.zeros((MP - M, 3 * M), BF16)
        zero_halo = jnp.zeros((HALO, 128), F32)
        for j in range(NT_M):
            kl_s[j, 0:HALO, :] = zero_halo
            vl_s[j, 0:HALO, :] = zero_halo
        wpt_s[3 * M:NPK * 128, :] = jnp.zeros((NPK * 128 - 3 * M, M), BF16)
        woap_s[DF * H:DF * H + 64, :] = jnp.zeros((64, M), BF16)
        eye = make_eye()

        copies["wqkv"].wait()
        ncol = 3 * M
        for t in range(pl.cdiv(ncol, 128)):
            c0 = t * 128
            wd = min(128, ncol - c0)
            wt = _dot(eye[0:wd, 0:wd], wqkv_s[:, c0:c0 + wd], NT)
            for j in range(NT_M):
                wt_s[j, c0:c0 + wd, :] = wt[:, j * 128:(j + 1) * 128]
        for sec in range(3):
            for d in range(DHA):
                for j in range(NT_M):
                    rows = wt_s[j, pl.ds(sec * M + d, H, stride=DHA), :]
                    wj = min(128, M - j * 128)
                    p0 = _packed_row(sec, d)
                    wpt_s[p0:p0 + H, j * 128:j * 128 + wj] = rows[:, 0:wj].astype(BF16)
        copies["x"].wait()
        copies["woa"].wait()
        copies["c"].start()
        for cp in group_copies(0):
            cp.start()
        copies["gate"].wait()

    def a_prep_wo():
        eye = make_eye()
        woa = woa_s[...].astype(F32)
        for j in range(NT_M):
            wj = min(128, M - j * 128)
            blk = woa[:, j * 128:j * 128 + wj]
            if wj < 128:
                blk = jnp.concatenate([blk, jnp.zeros((M, 128 - wj), F32)], axis=1)
            wof_s[j] = blk
        for d in range(DHA):
            for j in range(NT_M):
                wj = min(128, M - j * 128)
                rows = wof_s[j, pl.ds(d, H, stride=DHA), :]
                p0 = d * H if d < DF else d * H + 64
                woap_s[p0:p0 + H, j * 128:j * 128 + wj] = rows[:, 0:wj].astype(BF16)
        for j in range(NT_M):
            wj = min(128, M - j * 128)
            woapt_s[j * 128:j * 128 + wj, :] = _dot(
                eye[0:wj, 0:wj], woap_s[:, j * 128:j * 128 + wj], NT).astype(BF16)

    def a_xpose():
        eye = make_eye()
        for t in range(S // 128):
            x_s[t * 128:(t + 1) * 128, :] = _dot(eye, xt_s[:, t * 128:(t + 1) * 128], NT).astype(BF16)
        gw = jnp.broadcast_to(gate_s[...].reshape(1, M), (16, M))
        g_s[...] = jax.nn.sigmoid(_dot(gw, xt_s[...]))

    a_scale = (DHA ** -0.5) * LOG2E

    def a_proj(c, carry):
        r0 = pl.multiple_of(c * RAP, RAP)
        rk = pl.multiple_of(HALO + c * RAP, HALO)
        xq = x_s[pl.ds(r0, RAP), :]
        nf = DF * H
        q = _dot(xq, wpt_s[0:nf, :], NT)
        for j in range(NT_M - 1):
            qa_s[j, pl.ds(r0, RAP), :] = q[:, j * 128:(j + 1) * 128]
        k = _dot(xq, wpt_s[nf:2 * nf, :], NT) * a_scale
        for j in range(NT_M - 1):
            kl_s[j, pl.ds(rk, RAP), :] = k[:, j * 128:(j + 1) * 128]
        v = _dot(xq, wpt_s[2 * nf:3 * nf, :], NT)
        for j in range(NT_M - 1):
            vl_s[j, pl.ds(rk, RAP), :] = v[:, j * 128:(j + 1) * 128]
        t = _dot(xq, wpt_s[3 * nf:NPK * 128, :], NT)
        vl_s[NT_M - 1, pl.ds(rk, RAP), :] = t[:, 0:128]
        kl_s[NT_M - 1, pl.ds(rk, RAP), :] = t[:, 128:256] * a_scale
        return carry

    def a_local(r0, sb, dz):
        qv = [qa_s.at[j, pl.ds(r0, RA), :] for j in range(NT_M - 1)]
        kv = [kl_s.at[j, pl.ds(r0, HALO + RA), :] for j in range(NT_M)]
        vv = [vl_s.at[j, pl.ds(r0, HALO + RA), :] for j in range(NT_M)]
        b0 = sb * RS
        qt = [qv[j][b0:b0 + RS, :] for j in range(NT_M - 1)]
        qt.append(vv[NT_M - 1][HALO + b0:HALO + b0 + RS, :])
        logits = []
        for w in range(WIN):
            off = HALO + b0 - w * DIL
            s = None
            for j in range(NT_M):
                t = qt[j] * kv[j][off:off + RS, :]
                s = t if s is None else s + t
            s = s + pltpu.roll(s, 64, 1)
            s = s + pltpu.roll(s, 32, 1)
            if b0 < w * DIL:
                rowi = jax.lax.broadcasted_iota(jnp.int32, (RS, 128), 0) + (r0 + b0)
                s = jnp.where(rowi >= w * DIL, s, NEG * LOG2E)
            logits.append(s)
        m = functools.reduce(jnp.maximum, logits)
        ps = [jnp.exp2(s - m) for s in logits]
        r = _recip(functools.reduce(jnp.add, ps))
        for j in range(NT_M):
            o = None
            for w in range(WIN):
                off = HALO + b0 - w * DIL
                t = ps[w] * vv[j][off:off + RS, :]
                o = t if o is None else o + t
            qc_s[HG + H + j + dz, pl.ds(pl.multiple_of(r0 + b0, RS), RS), :] = (o * r).astype(BF16)

    def a_main():
        a_xpose()
        a_prep_wo()
        jax.lax.fori_loop(0, S // RAP, a_proj, 0)

    def group_weights(raw, g):
        cols = []
        for b in range(HG // 2):
            u = raw[g * (HG // 2) + b]
            cols.append(pltpu.bitcast(u << 16, F32).astype(BF16))
            cols.append(pltpu.bitcast(u & jnp.uint32(0xFFFF0000), F32).astype(BF16))
        return jnp.concatenate(cols, axis=1)

    b_scale = (D ** -0.5) * LOG2E

    def group_body(g, carry):
        @pl.when(g > 0)
        def _():
            for cp in group_copies(g):
                cp.wait()

        def proj_body(rc, c2):
            r0 = pl.multiple_of(rc * RP, RP)
            ra = pl.multiple_of((g * (S // RP) + rc) * RA, RA)

            def proj(src, raw, dst, scale, part):
                n = RP // PSPLIT
                rows = pl.ds(pl.multiple_of(r0 + part * n, n), n)
                y = _dot(src[rows, :], group_weights(raw, g))
                if scale is not None:
                    y = y * scale
                for i in range(HG):
                    dst[i, rows, :] = y[:, i * D:(i + 1) * D].astype(BF16)

            count = {"q": 0, "k": 0, "v": 0}
            for ch in PROJ_SEQ:
                if ch in count:
                    src, raw, dst, scale = {"q": (x_s, wq_raw, qc_s, b_scale), "k": (c_s, wuk_raw, k_s, None),
                                            "v": (c_s, wuv_raw, v_s, None)}[ch]
                    proj(src, raw, dst, scale, count[ch])
                    count[ch] += 1
                else:
                    a_local(ra, int(ch), jnp.minimum(g, 0) if DYNZ else 0)
            return c2

        with jax.named_scope("B_proj"):
            jax.lax.fori_loop(0, S // RP, proj_body, 0)

        def attn_body(it, c2):
            attn_heads(qc_s, k_s, v_s, g, it)
            return c2

        with jax.named_scope("B_attn"):
            jax.lax.fori_loop(0, HG // HU, attn_body, 0)
        return carry

    def out_copy(i):
        r0 = i * RO
        if not isinstance(i, int):
            r0 = pl.multiple_of(r0, RO)
        return pltpu.make_async_copy(out_s.at[:, pl.ds(r0, RO)], out_hbm.at[0, :, pl.ds(r0, RO)], osems.at[i])

    def out_body(i, carry):
        r0 = pl.multiple_of(i * RO, RO)
        ctx = jnp.concatenate([qc_s[HG + h, pl.ds(r0, RO), :] for h in range(H)], axis=1)
        wo = jnp.concatenate([wob_s[h] for h in range(H)], axis=1)
        bt = _dot(wo, ctx, NT)
        oa = jnp.concatenate([qc_s[HG + H + j, pl.ds(r0, RO), :] for j in range(NT_M)], axis=1)
        at = _dot(woapt_s[...], oa, NT)
        gt = g_s[0:1, pl.ds(r0, RO)]
        out_s[:, pl.ds(r0, RO)] = (gt * at + (1.0 - gt) * bt).astype(BF16)
        out_copy(i).start()
        return carry

    with jax.named_scope("A_prep"):
        a_prep()
    with jax.named_scope("A_main"):
        a_main()
        copies["c"].wait()
        for cp in group_copies(0):
            cp.wait()
        for g in range(1, NG):
            for cp in group_copies(g):
                cp.start()
        copies["wob"].start()
    jax.lax.fori_loop(0, NG, group_body, 0)
    with jax.named_scope("B_out"):
        copies["wob"].wait()
        jax.lax.fori_loop(0, S // RO, out_body, 0)
        for i in range(S // RO):
            out_copy(i).wait()


@jax.jit
def pallas_gated_mix__sliding_local_dilated__compressed_kv_cla__prompt_kernel(
    A_x: jax.Array,
    A_wqkv: jax.Array,
    A_wo: jax.Array,
    B_x: jax.Array,
    B_c_kv: jax.Array,
    B_w_q: jax.Array,
    B_w_uk: jax.Array,
    B_w_uv: jax.Array,
    B_w_o: jax.Array,
    gate_w: jax.Array,
):
    del B_x
    xt = jnp.swapaxes(A_x, 1, 2).reshape(M, S)
    c = B_c_kv.reshape(S, DC)
    wob = jnp.swapaxes(B_w_o, 1, 2)

    any_spec = pl.BlockSpec(memory_space=pl.ANY)
    scratch = [
        pltpu.VMEM((M, S), BF16),
        pltpu.VMEM((S, M), BF16),
        pltpu.VMEM((MP, 3 * M), BF16),
        pltpu.VMEM((M, M), BF16),
        pltpu.VMEM((S, DC), BF16),
        pltpu.VMEM((NPAIR, M, D), jnp.uint32),
        pltpu.VMEM((NPAIR, DC, D), jnp.uint32),
        pltpu.VMEM((NPAIR, DC, D), jnp.uint32),
        pltpu.VMEM((H, M, D), BF16),
        pltpu.VMEM((M,), BF16),
        pltpu.VMEM((NT_M, 14 * 128, 128), F32),
        pltpu.VMEM((NPK * 128, M), BF16),
        pltpu.VMEM((NT_M, M, 128), F32),
        pltpu.VMEM((MP, M), BF16),
        pltpu.VMEM((M, MP), BF16),
        pltpu.VMEM((NT_M - 1, S, 128), F32),
        pltpu.VMEM((NT_M, HALO + S, 128), F32),
        pltpu.VMEM((NT_M, HALO + S, 128), F32),
        pltpu.VMEM((16, S), F32),
        pltpu.VMEM((HG + H + NT_M, S, D), BF16),
        pltpu.VMEM((HG, S, D), BF16),
        pltpu.VMEM((HG, S, D), BF16),
        pltpu.VMEM((M, S), BF16),
        pltpu.SemaphoreType.DMA((6,)),
        pltpu.SemaphoreType.DMA((3 * NPAIR,)),
        pltpu.SemaphoreType.DMA((S // RO,)),
    ]
    out_t = pl.pallas_call(
        _kernel,
        out_shape=jax.ShapeDtypeStruct((1, M, S), BF16),
        in_specs=[any_spec] * 9,
        out_specs=any_spec,
        scratch_shapes=scratch,
        compiler_params=pltpu.CompilerParams(vmem_limit_bytes=120 * 1024 * 1024),
        name="gated_mix",
    )(xt, A_wqkv, A_wo, c, B_w_q, B_w_uk, B_w_uv, wob, gate_w)
    return jnp.swapaxes(out_t, 1, 2)
```

```python
import functools
import math

import jax
import jax.numpy as jnp
import jax.experimental.pallas as pl
import jax.experimental.pallas.tpu as pltpu

F32 = jnp.float32
BF16 = jnp.bfloat16

S = 2048
M = 576
MP = 640
NT_M = MP // 128
H = 32
D = 128
DC = 512
DHA = 18
WIN = 8
DIL = 2
HALO = 16
DF = 16
NPK = 14
LOG2E = math.log2(math.e)
NEG = -1e9

RAP = 512
RA = 256
RS = 32
HG = 8
NG = H // HG
RP = 1024
TQ = 256
TB = 128
HU = 2
BLOCK_ORDER = ((1, 3, 7, 6, 5, 4, 2, 0), (6, 7, 4, 5, 2, 3, 1, 0))
assert all(sorted(o) == list(range(S // TQ)) for o in BLOCK_ORDER) and len(BLOCK_ORDER) == HU
PSPLIT = 1
DYNZ = 0
PROJ_SEQ = "kvq01234567"
LAG = 1
RO = 256
assert NG * (S // RP) == S // RA
NXC = 4
NSPLIT = 1
NPAIR = H // 2

NN = (((1,), (0,)), ((), ()))
NT = (((1,), (1,)), ((), ()))


def _dot(a, b, dims=NN):
    return jax.lax.dot_general(a, b, dims, preferred_element_type=F32)


def _packed_row(sec, d):
    if d < DF:
        return (sec * DF + d) * H
    return 3 * DF * H + ((0, 4, 2)[sec] + d - DF) * H


def _lane_partial(s, op):
    acc = s[:, 0:128]
    for j in range(1, s.shape[1] // 128):
        acc = op(acc, s[:, j * 128:(j + 1) * 128])
    return acc


def _recip(l):
    r = pl.reciprocal(l, approx=True)
    return r * (2.0 - l * r)


def _segments(r0):
    nsub = TQ // TB
    segs = []
    if r0 > 0:
        segs.append((0, TQ, 0, r0, False))
    for j in range(nsub):
        segs.append((j * TB, (j + 1) * TB, r0 + j * TB, r0 + (j + 1) * TB, True))
        if (j + 1) * TB < TQ:
            segs.append(((j + 1) * TB, TQ, r0 + j * TB, r0 + (j + 1) * TB, False))
    return segs


def _attn_scores(q_ref, k_ref, r0, tri):
    nsub = TQ // TB
    segs = _segments(r0)
    ss = []
    for (a, b, c, d, msk) in segs:
        s = _dot(q_ref[r0 + a:r0 + b, :], k_ref[c:d, :], NT)
        if msk:
            s = jnp.where(tri, s, NEG * LOG2E)
        ss.append(s)
    ms = []
    for i in range(nsub):
        m = None
        for (a, b, c, d, msk), s in zip(segs, ss):
            if a <= i * TB and (i + 1) * TB <= b:
                sm = _lane_partial(s[i * TB - a:(i + 1) * TB - a], jnp.maximum)
                m = sm if m is None else jnp.maximum(m, sm)
        ms.append(jnp.max(m, axis=1, keepdims=True))
    return ss, ms


def _attn_values(v_ref, r0, ss, ms):
    nsub = TQ // TB
    segs = _segments(r0)
    ls = [None] * nsub
    os_ = [None] * nsub
    for (a, b, c, d, msk), s in zip(segs, ss):
        m = jnp.concatenate(ms[a // TB:b // TB], axis=0) if b - a > TB else ms[a // TB]
        p = jnp.exp2(s - m)
        l = _lane_partial(p, jnp.add)
        o = _dot(p.astype(BF16), v_ref[c:d, :])
        for i in range(a // TB, b // TB):
            li = l[i * TB - a:(i + 1) * TB - a]
            oi = o[i * TB - a:(i + 1) * TB - a]
            ls[i] = li if ls[i] is None else ls[i] + li
            os_[i] = oi if os_[i] is None else os_[i] + oi
    return [o * _recip(jnp.sum(l, axis=1, keepdims=True)) for o, l in zip(os_, ls)]


def attn_heads(qc_s, k_s, v_s, g, it):
    row = jax.lax.broadcasted_iota(jnp.int32, (TB, TB), 0)
    col = jax.lax.broadcasted_iota(jnp.int32, (TB, TB), 1)
    tri = col <= row
    items = [(u, r) for u in range(HU) for r in BLOCK_ORDER[u]]
    pend = {}
    done = {}

    def store(item):
        u, r = item
        for j, o in enumerate(done.pop(item)):
            r0 = r * TQ + j * TB
            qc_s[HG + g * HG + it * HU + u, r0:r0 + TB, :] = o.astype(BF16)

    for t in range(len(items) + 1):
        if t < len(items):
            u, r = items[t]
            hh = it * HU + u
            pend[items[t]] = _attn_scores(qc_s.at[hh], k_s.at[hh], r * TQ, tri)
        if t >= 1 + LAG:
            store(items[t - 1 - LAG])
        if t >= 1:
            u, r = items[t - 1]
            hh = it * HU + u
            done[items[t - 1]] = _attn_values(v_s.at[hh], r * TQ, *pend.pop(items[t - 1]))
    for item in list(done):
        store(item)


def _kernel(xt_hbm, wqkv_hbm, woa_hbm, c_hbm, wq_hbm, wuk_hbm, wuv_hbm, wob_hbm, gate_hbm,
            out_hbm,
            xt_s, x_s, wqkv_s, woa_s, c_s, wq_raw, wuk_raw, wuv_raw, wob_s, gate_s,
            wt_s, wpt_s, wof_s, woap_s, woapt_s, qa_s, kl_s, vl_s, g_s,
            qc_s, k_s, v_s, out_s, sems, xsems, wsems, osems):
    copies = {
        "gate": pltpu.make_async_copy(gate_hbm, gate_s, sems.at[2]),
        "woa": pltpu.make_async_copy(woa_hbm, woa_s, sems.at[3]),
        "c": pltpu.make_async_copy(c_hbm, c_s, sems.at[4]),
        "wob": pltpu.make_async_copy(wob_hbm, wob_s, sems.at[5]),
    }
    w_cols = (0, 5 * 128, 9 * 128, 3 * M)
    w_copies = [pltpu.make_async_copy(wqkv_hbm.at[:, pl.ds(w_cols[i], w_cols[i + 1] - w_cols[i])],
                                      wqkv_s.at[pl.ds(0, M), pl.ds(w_cols[i], w_cols[i + 1] - w_cols[i])],
                                      xsems.at[NXC + i]) for i in range(3)]
    xw = S // NXC
    x_copies = [pltpu.make_async_copy(xt_hbm.at[:, pl.ds(i * xw, xw)], xt_s.at[:, pl.ds(i * xw, xw)], xsems.at[i])
                for i in range(NXC)]
    def pair_copies(wi, j):
        w_hbm, raw = ((wq_hbm, wq_raw), (wuk_hbm, wuk_raw), (wuv_hbm, wuv_raw))[wi]
        n = w_hbm.shape[0] // NSPLIT
        return [pltpu.make_async_copy(
            w_hbm.bitcast(jnp.uint32).at[pl.ds(p * n, n), j, :], raw.at[j, pl.ds(p * n, n), :],
            wsems.at[wi * NPAIR + j]) for p in range(NSPLIT)]

    def group_copies(g):
        return [cp for b in range(HG // 2) for wi in range(3) for cp in pair_copies(wi, g * (HG // 2) + b)]

    chain = w_copies + [copies["woa"]] + x_copies
    copies["gate"].start()
    chain[0].start()
    chain[1].start()

    def chain_wait(i):
        with jax.named_scope(f"W_{i}"):
            chain[i].wait()
        if i + 2 < len(chain):
            chain[i + 2].start()

    def make_eye():
        return (jax.lax.broadcasted_iota(jnp.int32, (128, 128), 0)
                == jax.lax.broadcasted_iota(jnp.int32, (128, 128), 1)).astype(BF16)

    def a_prep():
        wqkv_s[M:MP, :] = jnp.zeros((MP - M, 3 * M), BF16)
        zero_halo = jnp.zeros((HALO, 128), F32)
        for j in range(NT_M):
            kl_s[j, 0:HALO, :] = zero_halo
            vl_s[j, 0:HALO, :] = zero_halo
        wpt_s[3 * M:NPK * 128, :] = jnp.zeros((NPK * 128 - 3 * M, M), BF16)
        woap_s[DF * H:DF * H + 64, :] = jnp.zeros((64, M), BF16)
        eye = make_eye()

        for sec in range(3):
            chain_wait(sec)
            for c0 in range(w_cols[sec], w_cols[sec + 1], 128):
                wd = min(128, 3 * M - c0)
                wt = _dot(eye[0:wd, 0:wd], wqkv_s[:, c0:c0 + wd], NT)
                for j in range(NT_M):
                    wt_s[j, c0:c0 + wd, :] = wt[:, j * 128:(j + 1) * 128]
            for d in range(DHA):
                for j in range(NT_M):
                    rows = wt_s[j, pl.ds(sec * M + d, H, stride=DHA), :]
                    wj = min(128, M - j * 128)
                    p0 = _packed_row(sec, d)
                    wpt_s[p0:p0 + H, j * 128:j * 128 + wj] = rows[:, 0:wj].astype(BF16)
        copies["gate"].wait()
        chain_wait(3)
        a_prep_wo()
        for i in range(NXC):
            chain_wait(4 + i)
            if i == NXC - 2:
                copies["c"].start()
                for cp in group_copies(0):
                    cp.start()
            a_xpose(i * xw, (i + 1) * xw)

    def a_prep_wo():
        eye = make_eye()
        woa = woa_s[...].astype(F32)
        for j in range(NT_M):
            wj = min(128, M - j * 128)
            blk = woa[:, j * 128:j * 128 + wj]
            if wj < 128:
                blk = jnp.concatenate([blk, jnp.zeros((M, 128 - wj), F32)], axis=1)
            wof_s[j] = blk
        for d in range(DHA):
            for j in range(NT_M):
                wj = min(128, M - j * 128)
                rows = wof_s[j, pl.ds(d, H, stride=DHA), :]
                p0 = d * H if d < DF else d * H + 64
                woap_s[p0:p0 + H, j * 128:j * 128 + wj] = rows[:, 0:wj].astype(BF16)
        for j in range(NT_M):
            wj = min(128, M - j * 128)
            woapt_s[j * 128:j * 128 + wj, :] = _dot(
                eye[0:wj, 0:wj], woap_s[:, j * 128:j * 128 + wj], NT).astype(BF16)

    def a_xpose(t0, t1):
        eye = make_eye()
        for t in range(t0 // 128, t1 // 128):
            x_s[t * 128:(t + 1) * 128, :] = _dot(eye, xt_s[:, t * 128:(t + 1) * 128], NT).astype(BF16)
        gw = jnp.broadcast_to(gate_s[...].reshape(1, M), (16, M))
        g_s[:, t0:t1] = jax.nn.sigmoid(_dot(gw, xt_s[:, t0:t1]))

    a_scale = (DHA ** -0.5) * LOG2E

    def a_proj(c, carry):
        r0 = pl.multiple_of(c * RAP, RAP)
        rk = pl.multiple_of(HALO + c * RAP, HALO)
        xq = x_s[pl.ds(r0, RAP), :]
        nf = DF * H
        q = _dot(xq, wpt_s[0:nf, :], NT)
        for j in range(NT_M - 1):
            qa_s[j, pl.ds(r0, RAP), :] = q[:, j * 128:(j + 1) * 128]
        k = _dot(xq, wpt_s[nf:2 * nf, :], NT) * a_scale
        for j in range(NT_M - 1):
            kl_s[j, pl.ds(rk, RAP), :] = k[:, j * 128:(j + 1) * 128]
        v = _dot(xq, wpt_s[2 * nf:3 * nf, :], NT)
        for j in range(NT_M - 1):
            vl_s[j, pl.ds(rk, RAP), :] = v[:, j * 128:(j + 1) * 128]
        t = _dot(xq, wpt_s[3 * nf:NPK * 128, :], NT)
        vl_s[NT_M - 1, pl.ds(rk, RAP), :] = t[:, 0:128]
        kl_s[NT_M - 1, pl.ds(rk, RAP), :] = t[:, 128:256] * a_scale
        return carry

    def a_local(r0, sb, dz):
        qv = [qa_s.at[j, pl.ds(r0, RA), :] for j in range(NT_M - 1)]
        kv = [kl_s.at[j, pl.ds(r0, HALO + RA), :] for j in range(NT_M)]
        vv = [vl_s.at[j, pl.ds(r0, HALO + RA), :] for j in range(NT_M)]
        b0 = sb * RS
        qt = [qv[j][b0:b0 + RS, :] for j in range(NT_M - 1)]
        qt.append(vv[NT_M - 1][HALO + b0:HALO + b0 + RS, :])
        logits = []
        for w in range(WIN):
            off = HALO + b0 - w * DIL
            s = None
            for j in range(NT_M):
                t = qt[j] * kv[j][off:off + RS, :]
                s = t if s is None else s + t
            s = s + pltpu.roll(s, 64, 1)
            s = s + pltpu.roll(s, 32, 1)
            if b0 < w * DIL:
                rowi = jax.lax.broadcasted_iota(jnp.int32, (RS, 128), 0) + (r0 + b0)
                s = jnp.where(rowi >= w * DIL, s, NEG * LOG2E)
            logits.append(s)
        m = functools.reduce(jnp.maximum, logits)
        ps = [jnp.exp2(s - m) for s in logits]
        r = _recip(functools.reduce(jnp.add, ps))
        for j in range(NT_M):
            o = None
            for w in range(WIN):
                off = HALO + b0 - w * DIL
                t = ps[w] * vv[j][off:off + RS, :]
                o = t if o is None else o + t
            qc_s[HG + H + j + dz, pl.ds(pl.multiple_of(r0 + b0, RS), RS), :] = (o * r).astype(BF16)

    def a_main():
        jax.lax.fori_loop(0, S // RAP, a_proj, 0)

    def group_weights(raw, g):
        cols = []
        for b in range(HG // 2):
            u = raw[g * (HG // 2) + b]
            cols.append(pltpu.bitcast(u << 16, F32).astype(BF16))
            cols.append(pltpu.bitcast(u & jnp.uint32(0xFFFF0000), F32).astype(BF16))
        return jnp.concatenate(cols, axis=1)

    b_scale = (D ** -0.5) * LOG2E

    def group_body(g, carry):
        @pl.when(g > 0)
        def _():
            for cp in group_copies(g):
                cp.wait()

        def proj_body(rc, c2):
            r0 = pl.multiple_of(rc * RP, RP)
            ra = pl.multiple_of((g * (S // RP) + rc) * RA, RA)

            def proj(src, raw, dst, scale, part):
                n = RP // PSPLIT
                rows = pl.ds(pl.multiple_of(r0 + part * n, n), n)
                y = _dot(src[rows, :], group_weights(raw, g))
                if scale is not None:
                    y = y * scale
                for i in range(HG):
                    dst[i, rows, :] = y[:, i * D:(i + 1) * D].astype(BF16)

            count = {"q": 0, "k": 0, "v": 0}
            for ch in PROJ_SEQ:
                if ch in count:
                    src, raw, dst, scale = {"q": (x_s, wq_raw, qc_s, b_scale), "k": (c_s, wuk_raw, k_s, None),
                                            "v": (c_s, wuv_raw, v_s, None)}[ch]
                    proj(src, raw, dst, scale, count[ch])
                    count[ch] += 1
                else:
                    a_local(ra, int(ch), jnp.minimum(g, 0) if DYNZ else 0)
            return c2

        with jax.named_scope("B_proj"):
            jax.lax.fori_loop(0, S // RP, proj_body, 0)

        def attn_body(it, c2):
            attn_heads(qc_s, k_s, v_s, g, it)
            return c2

        with jax.named_scope("B_attn"):
            jax.lax.fori_loop(0, HG // HU, attn_body, 0)
        return carry

    def out_copy(i):
        r0 = i * RO
        if not isinstance(i, int):
            r0 = pl.multiple_of(r0, RO)
        return pltpu.make_async_copy(out_s.at[:, pl.ds(r0, RO)], out_hbm.at[0, :, pl.ds(r0, RO)], osems.at[i])

    def out_body(i, carry):
        r0 = pl.multiple_of(i * RO, RO)
        ctx = jnp.concatenate([qc_s[HG + h, pl.ds(r0, RO), :] for h in range(H)], axis=1)
        wo = jnp.concatenate([wob_s[h] for h in range(H)], axis=1)
        bt = _dot(wo, ctx, NT)
        oa = jnp.concatenate([qc_s[HG + H + j, pl.ds(r0, RO), :] for j in range(NT_M)], axis=1)
        at = _dot(woapt_s[...], oa, NT)
        gt = g_s[0:1, pl.ds(r0, RO)]
        out_s[:, pl.ds(r0, RO)] = (gt * at + (1.0 - gt) * bt).astype(BF16)
        out_copy(i).start()
        return carry

    with jax.named_scope("A_prep"):
        a_prep()
    with jax.named_scope("A_main"):
        a_main()
        copies["c"].wait()
        for cp in group_copies(0):
            cp.wait()
        for g in range(1, NG):
            for cp in group_copies(g):
                cp.start()
        copies["wob"].start()
    jax.lax.fori_loop(0, NG, group_body, 0)
    with jax.named_scope("B_out"):
        copies["wob"].wait()
        jax.lax.fori_loop(0, S // RO, out_body, 0)
        for i in range(S // RO):
            out_copy(i).wait()


@jax.jit
def pallas_gated_mix__sliding_local_dilated__compressed_kv_cla__prompt_kernel(
    A_x: jax.Array,
    A_wqkv: jax.Array,
    A_wo: jax.Array,
    B_x: jax.Array,
    B_c_kv: jax.Array,
    B_w_q: jax.Array,
    B_w_uk: jax.Array,
    B_w_uv: jax.Array,
    B_w_o: jax.Array,
    gate_w: jax.Array,
):
    del B_x
    xt = jnp.swapaxes(A_x, 1, 2).reshape(M, S)
    c = B_c_kv.reshape(S, DC)
    wob = jnp.swapaxes(B_w_o, 1, 2)

    any_spec = pl.BlockSpec(memory_space=pl.ANY)
    scratch = [
        pltpu.VMEM((M, S), BF16),
        pltpu.VMEM((S, M), BF16),
        pltpu.VMEM((MP, 3 * M), BF16),
        pltpu.VMEM((M, M), BF16),
        pltpu.VMEM((S, DC), BF16),
        pltpu.VMEM((NPAIR, M, D), jnp.uint32),
        pltpu.VMEM((NPAIR, DC, D), jnp.uint32),
        pltpu.VMEM((NPAIR, DC, D), jnp.uint32),
        pltpu.VMEM((H, M, D), BF16),
        pltpu.VMEM((M,), BF16),
        pltpu.VMEM((NT_M, 14 * 128, 128), F32),
        pltpu.VMEM((NPK * 128, M), BF16),
        pltpu.VMEM((NT_M, M, 128), F32),
        pltpu.VMEM((MP, M), BF16),
        pltpu.VMEM((M, MP), BF16),
        pltpu.VMEM((NT_M - 1, S, 128), F32),
        pltpu.VMEM((NT_M, HALO + S, 128), F32),
        pltpu.VMEM((NT_M, HALO + S, 128), F32),
        pltpu.VMEM((16, S), F32),
        pltpu.VMEM((HG + H + NT_M, S, D), BF16),
        pltpu.VMEM((HG, S, D), BF16),
        pltpu.VMEM((HG, S, D), BF16),
        pltpu.VMEM((M, S), BF16),
        pltpu.SemaphoreType.DMA((6,)),
        pltpu.SemaphoreType.DMA((NXC + 3,)),
        pltpu.SemaphoreType.DMA((3 * NPAIR,)),
        pltpu.SemaphoreType.DMA((S // RO,)),
    ]
    out_t = pl.pallas_call(
        _kernel,
        out_shape=jax.ShapeDtypeStruct((1, M, S), BF16),
        in_specs=[any_spec] * 9,
        out_specs=any_spec,
        scratch_shapes=scratch,
        compiler_params=pltpu.CompilerParams(vmem_limit_bytes=120 * 1024 * 1024),
        name="gated_mix",
    )(xt, A_wqkv, A_wo, c, B_w_q, B_w_uk, B_w_uv, wob, gate_w)
    return jnp.swapaxes(out_t, 1, 2)
```

```python
import functools
import math

import jax
import jax.numpy as jnp
import jax.experimental.pallas as pl
import jax.experimental.pallas.tpu as pltpu

F32 = jnp.float32
BF16 = jnp.bfloat16

S = 2048
M = 576
MP = 640
NT_M = MP // 128
H = 32
D = 128
DC = 512
DHA = 18
WIN = 8
DIL = 2
HALO = 16
DF = 16
NPK = 14
LOG2E = math.log2(math.e)
NEG = -1e9

RAP = 256
RA = 256
RG = 8
RS = 32
HG = 8
NG = H // HG
RP = 1024
TQ = 256
TB = 128
HU = 2
BLOCK_ORDER = ((1, 3, 7, 6, 5, 4, 2, 0), (6, 7, 4, 5, 2, 3, 1, 0))
assert all(sorted(o) == list(range(S // TQ)) for o in BLOCK_ORDER) and len(BLOCK_ORDER) == HU
PSPLIT = 1
DYNZ = 0
PROJ_SEQ = "01v234q56k7"
LAG = 1
RO = 256
assert NG * (S // RP) == S // RA
NXC = 4
NSPLIT = 1
NPAIR = H // 2

NN = (((1,), (0,)), ((), ()))
NT = (((1,), (1,)), ((), ()))


def _dot(a, b, dims=NN):
    return jax.lax.dot_general(a, b, dims, preferred_element_type=F32)


def _packed_row(sec, d):
    if d < DF:
        return (sec * DF + d) * H
    return 3 * DF * H + ((0, 4, 2)[sec] + d - DF) * H


def _lane_partial(s, op):
    acc = s[:, 0:128]
    for j in range(1, s.shape[1] // 128):
        acc = op(acc, s[:, j * 128:(j + 1) * 128])
    return acc


def _recip(l):
    r = pl.reciprocal(l, approx=True)
    return r * (2.0 - l * r)


def _segments(r0):
    nsub = TQ // TB
    segs = []
    if r0 > 0:
        segs.append((0, TQ, 0, r0, False))
    for j in range(nsub):
        segs.append((j * TB, (j + 1) * TB, r0 + j * TB, r0 + (j + 1) * TB, True))
        if (j + 1) * TB < TQ:
            segs.append(((j + 1) * TB, TQ, r0 + j * TB, r0 + (j + 1) * TB, False))
    return segs


def _attn_scores(q_ref, k_ref, r0, tri):
    nsub = TQ // TB
    segs = _segments(r0)
    ss = []
    for (a, b, c, d, msk) in segs:
        s = _dot(q_ref[r0 + a:r0 + b, :], k_ref[c:d, :], NT)
        if msk:
            s = jnp.where(tri, s, NEG * LOG2E)
        ss.append(s)
    ms = []
    for i in range(nsub):
        m = None
        for (a, b, c, d, msk), s in zip(segs, ss):
            if a <= i * TB and (i + 1) * TB <= b:
                sm = _lane_partial(s[i * TB - a:(i + 1) * TB - a], jnp.maximum)
                m = sm if m is None else jnp.maximum(m, sm)
        ms.append(jnp.max(m, axis=1, keepdims=True))
    return ss, ms


def _attn_values(v_ref, r0, ss, ms):
    nsub = TQ // TB
    segs = _segments(r0)
    ls = [None] * nsub
    os_ = [None] * nsub
    for (a, b, c, d, msk), s in zip(segs, ss):
        m = jnp.concatenate(ms[a // TB:b // TB], axis=0) if b - a > TB else ms[a // TB]
        p = jnp.exp2(s - m)
        l = _lane_partial(p, jnp.add)
        o = _dot(p.astype(BF16), v_ref[c:d, :])
        for i in range(a // TB, b // TB):
            li = l[i * TB - a:(i + 1) * TB - a]
            oi = o[i * TB - a:(i + 1) * TB - a]
            ls[i] = li if ls[i] is None else ls[i] + li
            os_[i] = oi if os_[i] is None else os_[i] + oi
    return [o * _recip(jnp.sum(l, axis=1, keepdims=True)) for o, l in zip(os_, ls)]


def attn_heads(qc_s, k_s, v_s, g, it):
    row = jax.lax.broadcasted_iota(jnp.int32, (TB, TB), 0)
    col = jax.lax.broadcasted_iota(jnp.int32, (TB, TB), 1)
    tri = col <= row
    items = [(u, r) for u in range(HU) for r in BLOCK_ORDER[u]]
    pend = {}
    done = {}

    def store(item):
        u, r = item
        for j, o in enumerate(done.pop(item)):
            r0 = r * TQ + j * TB
            qc_s[HG + g * HG + it * HU + u, r0:r0 + TB, :] = o.astype(BF16)

    for t in range(len(items) + 1):
        if t < len(items):
            u, r = items[t]
            hh = it * HU + u
            pend[items[t]] = _attn_scores(qc_s.at[hh], k_s.at[hh], r * TQ, tri)
        if t >= 1 + LAG:
            store(items[t - 1 - LAG])
        if t >= 1:
            u, r = items[t - 1]
            hh = it * HU + u
            done[items[t - 1]] = _attn_values(v_s.at[hh], r * TQ, *pend.pop(items[t - 1]))
    for item in list(done):
        store(item)


def _kernel(xt_hbm, wqkv_hbm, woa_hbm, c_hbm, wq_hbm, wuk_hbm, wuv_hbm, wob_hbm, gate_hbm,
            out_hbm,
            xt_s, x_s, wqkv_s, woa_s, c_s, wq_raw, wuk_raw, wuv_raw, wob_s, gate_s,
            wt_s, wpt_s, wof_s, woap_s, woapt_s, qa_s, kl_s, vl_s, g_s,
            qc_s, k_s, v_s, out_s, sems, xsems, wsems, osems):
    copies = {
        "gate": pltpu.make_async_copy(gate_hbm, gate_s, sems.at[2]),
        "woa": pltpu.make_async_copy(woa_hbm, woa_s, sems.at[3]),
        "c": pltpu.make_async_copy(c_hbm, c_s, sems.at[4]),
        "wob": pltpu.make_async_copy(wob_hbm, wob_s, sems.at[5]),
    }
    w_cols = (0, 5 * 128, 9 * 128, 3 * M)
    w_copies = [pltpu.make_async_copy(wqkv_hbm.at[:, pl.ds(w_cols[i], w_cols[i + 1] - w_cols[i])],
                                      wqkv_s.at[pl.ds(0, M), pl.ds(w_cols[i], w_cols[i + 1] - w_cols[i])],
                                      xsems.at[NXC + i]) for i in range(3)]
    xw = S // NXC
    x_copies = [pltpu.make_async_copy(xt_hbm.at[:, pl.ds(i * xw, xw)], xt_s.at[:, pl.ds(i * xw, xw)], xsems.at[i])
                for i in range(NXC)]
    def pair_copies(wi, j):
        w_hbm, raw = ((wq_hbm, wq_raw), (wuk_hbm, wuk_raw), (wuv_hbm, wuv_raw))[wi]
        n = w_hbm.shape[0] // NSPLIT
        return [pltpu.make_async_copy(
            w_hbm.bitcast(jnp.uint32).at[pl.ds(p * n, n), j, :], raw.at[j, pl.ds(p * n, n), :],
            wsems.at[wi * NPAIR + j]) for p in range(NSPLIT)]

    def group_copies(g):
        return [cp for b in range(HG // 2) for wi in range(3) for cp in pair_copies(wi, g * (HG // 2) + b)]

    chain = w_copies + [copies["woa"]] + x_copies
    copies["gate"].start()
    chain[0].start()
    chain[1].start()

    def chain_wait(i):
        with jax.named_scope(f"W_{i}"):
            chain[i].wait()
        if i + 2 < len(chain):
            chain[i + 2].start()

    def make_eye():
        return (jax.lax.broadcasted_iota(jnp.int32, (128, 128), 0)
                == jax.lax.broadcasted_iota(jnp.int32, (128, 128), 1)).astype(BF16)

    def a_prep():
        wqkv_s[M:MP, :] = jnp.zeros((MP - M, 3 * M), BF16)
        zero_halo = jnp.zeros((HALO, 128), F32)
        for j in range(NT_M):
            kl_s[j, 0:HALO, :] = zero_halo
            vl_s[j, 0:HALO, :] = zero_halo
        wpt_s[3 * M:NPK * 128, :] = jnp.zeros((NPK * 128 - 3 * M, M), BF16)
        woap_s[DF * H:DF * H + 64, :] = jnp.zeros((64, M), BF16)
        eye = make_eye()

        for sec in range(3):
            chain_wait(sec)
            for c0 in range(w_cols[sec], w_cols[sec + 1], 128):
                wd = min(128, 3 * M - c0)
                wt = _dot(eye[0:wd, 0:wd], wqkv_s[:, c0:c0 + wd], NT)
                for j in range(NT_M):
                    wt_s[j, c0:c0 + wd, :] = wt[:, j * 128:(j + 1) * 128]
            for d in range(DHA):
                for j in range(NT_M):
                    rows = wt_s[j, pl.ds(sec * M + d, H, stride=DHA), :]
                    wj = min(128, M - j * 128)
                    p0 = _packed_row(sec, d)
                    wpt_s[p0:p0 + H, j * 128:j * 128 + wj] = rows[:, 0:wj].astype(BF16)
        copies["gate"].wait()
        chain_wait(3)
        a_prep_wo()
        for i in range(NXC):
            chain_wait(4 + i)
            if i == NXC - 2:
                copies["c"].start()
                for cp in group_copies(0):
                    cp.start()
            a_xpose(i * xw, (i + 1) * xw)

    def a_prep_wo():
        eye = make_eye()
        woa = woa_s[...].astype(F32)
        for j in range(NT_M):
            wj = min(128, M - j * 128)
            blk = woa[:, j * 128:j * 128 + wj]
            if wj < 128:
                blk = jnp.concatenate([blk, jnp.zeros((M, 128 - wj), F32)], axis=1)
            wof_s[j] = blk
        for d in range(DHA):
            for j in range(NT_M):
                wj = min(128, M - j * 128)
                rows = wof_s[j, pl.ds(d, H, stride=DHA), :]
                p0 = d * H if d < DF else d * H + 64
                woap_s[p0:p0 + H, j * 128:j * 128 + wj] = rows[:, 0:wj].astype(BF16)
        for j in range(NT_M):
            wj = min(128, M - j * 128)
            woapt_s[j * 128:j * 128 + wj, :] = _dot(
                eye[0:wj, 0:wj], woap_s[:, j * 128:j * 128 + wj], NT).astype(BF16)

    def a_xpose(t0, t1):
        eye = make_eye()
        for t in range(t0 // 128, t1 // 128):
            x_s[t * 128:(t + 1) * 128, :] = _dot(eye, xt_s[:, t * 128:(t + 1) * 128], NT).astype(BF16)
        gw = jnp.broadcast_to(gate_s[...].reshape(1, M), (16, M))
        g_s[:, t0:t1] = jax.nn.sigmoid(_dot(gw, xt_s[:, t0:t1]))

    a_scale = (DHA ** -0.5) * LOG2E

    def a_proj(c, carry):
        r0 = pl.multiple_of(c * RAP, RAP)
        rk = pl.multiple_of(HALO + c * RAP, HALO)
        xq = x_s[pl.ds(r0, RAP), :]
        nf = DF * H
        q = _dot(xq, wpt_s[0:nf, :], NT)
        for j in range(NT_M - 1):
            qa_s[j, pl.ds(r0, RAP), :] = q[:, j * 128:(j + 1) * 128]
        k = _dot(xq, wpt_s[nf:2 * nf, :], NT) * a_scale
        for j in range(NT_M - 1):
            kl_s[j, pl.ds(rk, RAP), :] = k[:, j * 128:(j + 1) * 128]
        v = _dot(xq, wpt_s[2 * nf:3 * nf, :], NT)
        for j in range(NT_M - 1):
            vl_s[j, pl.ds(rk, RAP), :] = v[:, j * 128:(j + 1) * 128]
        t = _dot(xq, wpt_s[3 * nf:NPK * 128, :], NT)
        vl_s[NT_M - 1, pl.ds(rk, RAP), :] = t[:, 0:128]
        kl_s[NT_M - 1, pl.ds(rk, RAP), :] = t[:, 128:256] * a_scale
        return carry

    def a_local(r0, sb, dz):
        qv = [qa_s.at[j, pl.ds(r0, RA), :] for j in range(NT_M - 1)]
        kv = [kl_s.at[j, pl.ds(r0, HALO + RA), :] for j in range(NT_M)]
        vv = [vl_s.at[j, pl.ds(r0, HALO + RA), :] for j in range(NT_M)]
        outs = []
        for b0 in range(sb * RS, (sb + 1) * RS, RG):
            qt = [qv[j][b0:b0 + RG, :] for j in range(NT_M - 1)]
            qt.append(vv[NT_M - 1][HALO + b0:HALO + b0 + RG, :])
            logits = []
            for w in range(WIN):
                off = HALO + b0 - w * DIL
                s = None
                for j in range(NT_M):
                    t = qt[j] * kv[j][off:off + RG, :]
                    s = t if s is None else s + t
                s = s + pltpu.roll(s, 64, 1)
                s = s + pltpu.roll(s, 32, 1)
                if b0 < w * DIL:
                    rowi = jax.lax.broadcasted_iota(jnp.int32, (RG, 128), 0) + (r0 + b0)
                    s = jnp.where(rowi >= w * DIL, s, NEG * LOG2E)
                logits.append(s)
            m = functools.reduce(jnp.maximum, logits)
            ps = [jnp.exp2(s - m) for s in logits]
            r = _recip(functools.reduce(jnp.add, ps))
            ot = []
            for j in range(NT_M):
                o = None
                for w in range(WIN):
                    off = HALO + b0 - w * DIL
                    t = ps[w] * vv[j][off:off + RG, :]
                    o = t if o is None else o + t
                ot.append(o * r)
            outs.append(ot)
        for j in range(NT_M):
            o = jnp.concatenate([ot[j] for ot in outs], axis=0)
            qc_s[HG + H + j + dz, pl.ds(pl.multiple_of(r0 + sb * RS, RS), RS), :] = o.astype(BF16)

    def a_main():
        jax.lax.fori_loop(0, S // RAP, a_proj, 0)

    def group_weights(raw, g):
        cols = []
        for b in range(HG // 2):
            u = raw[g * (HG // 2) + b]
            cols.append(pltpu.bitcast(u << 16, F32).astype(BF16))
            cols.append(pltpu.bitcast(u & jnp.uint32(0xFFFF0000), F32).astype(BF16))
        return jnp.concatenate(cols, axis=1)

    b_scale = (D ** -0.5) * LOG2E

    def group_body(g, carry):
        @pl.when(g > 0)
        def _():
            for cp in group_copies(g):
                cp.wait()

        def proj_body(rc, c2):
            r0 = pl.multiple_of(rc * RP, RP)
            ra = pl.multiple_of((g * (S // RP) + rc) * RA, RA)

            def proj(src, raw, dst, scale, part):
                n = RP // PSPLIT
                rows = pl.ds(pl.multiple_of(r0 + part * n, n), n)
                y = _dot(src[rows, :], group_weights(raw, g))
                if scale is not None:
                    y = y * scale
                for i in range(HG):
                    dst[i, rows, :] = y[:, i * D:(i + 1) * D].astype(BF16)

            count = {"q": 0, "k": 0, "v": 0}
            for ch in PROJ_SEQ:
                if ch in count:
                    src, raw, dst, scale = {"q": (x_s, wq_raw, qc_s, b_scale), "k": (c_s, wuk_raw, k_s, None),
                                            "v": (c_s, wuv_raw, v_s, None)}[ch]
                    proj(src, raw, dst, scale, count[ch])
                    count[ch] += 1
                else:
                    a_local(ra, int(ch, 36), jnp.minimum(g, 0) if DYNZ else 0)
            return c2

        with jax.named_scope("B_proj"):
            jax.lax.fori_loop(0, S // RP, proj_body, 0)

        def attn_body(it, c2):
            attn_heads(qc_s, k_s, v_s, g, it)
            return c2

        with jax.named_scope("B_attn"):
            jax.lax.fori_loop(0, HG // HU, attn_body, 0)
        return carry

    def out_copy(i):
        r0 = i * RO
        if not isinstance(i, int):
            r0 = pl.multiple_of(r0, RO)
        return pltpu.make_async_copy(out_s.at[:, pl.ds(r0, RO)], out_hbm.at[0, :, pl.ds(r0, RO)], osems.at[i])

    def out_body(i, carry):
        r0 = pl.multiple_of(i * RO, RO)
        ctx = jnp.concatenate([qc_s[HG + h, pl.ds(r0, RO), :] for h in range(H)], axis=1)
        wo = jnp.concatenate([wob_s[h] for h in range(H)], axis=1)
        bt = _dot(wo, ctx, NT)
        oa = jnp.concatenate([qc_s[HG + H + j, pl.ds(r0, RO), :] for j in range(NT_M)], axis=1)
        at = _dot(woapt_s[...], oa, NT)
        gt = g_s[0:1, pl.ds(r0, RO)]
        out_s[:, pl.ds(r0, RO)] = (gt * at + (1.0 - gt) * bt).astype(BF16)
        out_copy(i).start()
        return carry

    with jax.named_scope("A_prep"):
        a_prep()
    with jax.named_scope("A_main"):
        a_main()
        copies["c"].wait()
        for cp in group_copies(0):
            cp.wait()
        for g in range(1, NG):
            for cp in group_copies(g):
                cp.start()
        copies["wob"].start()
    jax.lax.fori_loop(0, NG, group_body, 0)
    with jax.named_scope("B_out"):
        copies["wob"].wait()
        jax.lax.fori_loop(0, S // RO, out_body, 0)
        for i in range(S // RO):
            out_copy(i).wait()


@jax.jit
def pallas_gated_mix__sliding_local_dilated__compressed_kv_cla__prompt_kernel(
    A_x: jax.Array,
    A_wqkv: jax.Array,
    A_wo: jax.Array,
    B_x: jax.Array,
    B_c_kv: jax.Array,
    B_w_q: jax.Array,
    B_w_uk: jax.Array,
    B_w_uv: jax.Array,
    B_w_o: jax.Array,
    gate_w: jax.Array,
):
    del B_x
    xt = jnp.swapaxes(A_x, 1, 2).reshape(M, S)
    c = B_c_kv.reshape(S, DC)
    wob = jnp.swapaxes(B_w_o, 1, 2)

    any_spec = pl.BlockSpec(memory_space=pl.ANY)
    scratch = [
        pltpu.VMEM((M, S), BF16),
        pltpu.VMEM((S, M), BF16),
        pltpu.VMEM((MP, 3 * M), BF16),
        pltpu.VMEM((M, M), BF16),
        pltpu.VMEM((S, DC), BF16),
        pltpu.VMEM((NPAIR, M, D), jnp.uint32),
        pltpu.VMEM((NPAIR, DC, D), jnp.uint32),
        pltpu.VMEM((NPAIR, DC, D), jnp.uint32),
        pltpu.VMEM((H, M, D), BF16),
        pltpu.VMEM((M,), BF16),
        pltpu.VMEM((NT_M, 14 * 128, 128), F32),
        pltpu.VMEM((NPK * 128, M), BF16),
        pltpu.VMEM((NT_M, M, 128), F32),
        pltpu.VMEM((MP, M), BF16),
        pltpu.VMEM((M, MP), BF16),
        pltpu.VMEM((NT_M - 1, S, 128), F32),
        pltpu.VMEM((NT_M, HALO + S, 128), F32),
        pltpu.VMEM((NT_M, HALO + S, 128), F32),
        pltpu.VMEM((16, S), F32),
        pltpu.VMEM((HG + H + NT_M, S, D), BF16),
        pltpu.VMEM((HG, S, D), BF16),
        pltpu.VMEM((HG, S, D), BF16),
        pltpu.VMEM((M, S), BF16),
        pltpu.SemaphoreType.DMA((6,)),
        pltpu.SemaphoreType.DMA((NXC + 3,)),
        pltpu.SemaphoreType.DMA((3 * NPAIR,)),
        pltpu.SemaphoreType.DMA((S // RO,)),
    ]
    out_t = pl.pallas_call(
        _kernel,
        out_shape=jax.ShapeDtypeStruct((1, M, S), BF16),
        in_specs=[any_spec] * 9,
        out_specs=any_spec,
        scratch_shapes=scratch,
        compiler_params=pltpu.CompilerParams(vmem_limit_bytes=120 * 1024 * 1024),
        name="gated_mix",
    )(xt, A_wqkv, A_wo, c, B_w_q, B_w_uk, B_w_uv, wob, gate_w)
    return jnp.swapaxes(out_t, 1, 2)
```

```python
import functools
import math

import jax
import jax.numpy as jnp
import jax.experimental.pallas as pl
import jax.experimental.pallas.tpu as pltpu

F32 = jnp.float32
BF16 = jnp.bfloat16

S = 2048
M = 576
MP = 640
NT_M = MP // 128
H = 32
D = 128
DC = 512
DHA = 18
WIN = 8
DIL = 2
HALO = 16
DF = 16
NPK = 14
LOG2E = math.log2(math.e)
NEG = -1e9

RAP = 256
RA = 256
RG = 8
RS = 32
HG = 8
NG = H // HG
RP = 1024
TQ = 256
TB = 128
HU = 2
BLOCK_ORDER = ((1, 3, 7, 6, 5, 4, 2, 0), (6, 7, 4, 5, 2, 3, 1, 0))
assert all(sorted(o) == list(range(S // TQ)) for o in BLOCK_ORDER) and len(BLOCK_ORDER) == HU
PSPLIT = 1
DYNZ = 0
PROJ_SEQ = "01v234q56k7"
LAG = 1
RO = 256
assert NG * (S // RP) == S // RA
NXC = 4
NSPLIT = 1
NPAIR = H // 2

NN = (((1,), (0,)), ((), ()))
NT = (((1,), (1,)), ((), ()))


def _dot(a, b, dims=NN):
    return jax.lax.dot_general(a, b, dims, preferred_element_type=F32)


def _packed_row(sec, d):
    if d < DF:
        return (sec * DF + d) * H
    return 3 * DF * H + ((0, 4, 2)[sec] + d - DF) * H


def _lane_partial(s, op):
    acc = s[:, 0:128]
    for j in range(1, s.shape[1] // 128):
        acc = op(acc, s[:, j * 128:(j + 1) * 128])
    return acc


def _recip(l):
    r = pl.reciprocal(l, approx=True)
    return r * (2.0 - l * r)


def _segments(r0):
    nsub = TQ // TB
    segs = []
    if r0 > 0:
        segs.append((0, TQ, 0, r0, False))
    for j in range(nsub):
        segs.append((j * TB, (j + 1) * TB, r0 + j * TB, r0 + (j + 1) * TB, True))
        if (j + 1) * TB < TQ:
            segs.append(((j + 1) * TB, TQ, r0 + j * TB, r0 + (j + 1) * TB, False))
    return segs


def _attn_scores(q_ref, k_ref, r0, tri):
    nsub = TQ // TB
    segs = _segments(r0)
    ss = []
    for (a, b, c, d, msk) in segs:
        s = _dot(q_ref[r0 + a:r0 + b, :], k_ref[c:d, :], NT)
        if msk:
            s = jnp.where(tri, s, NEG * LOG2E)
        ss.append(s)
    ms = []
    for i in range(nsub):
        m = None
        for (a, b, c, d, msk), s in zip(segs, ss):
            if a <= i * TB and (i + 1) * TB <= b:
                sm = _lane_partial(s[i * TB - a:(i + 1) * TB - a], jnp.maximum)
                m = sm if m is None else jnp.maximum(m, sm)
        ms.append(jnp.max(m, axis=1, keepdims=True))
    return ss, ms


def _attn_values(v_ref, r0, ss, ms):
    nsub = TQ // TB
    segs = _segments(r0)
    ls = [None] * nsub
    os_ = [None] * nsub
    for (a, b, c, d, msk), s in zip(segs, ss):
        m = jnp.concatenate(ms[a // TB:b // TB], axis=0) if b - a > TB else ms[a // TB]
        p = jnp.exp2(s - m)
        l = _lane_partial(p, jnp.add)
        o = _dot(p.astype(BF16), v_ref[c:d, :])
        for i in range(a // TB, b // TB):
            li = l[i * TB - a:(i + 1) * TB - a]
            oi = o[i * TB - a:(i + 1) * TB - a]
            ls[i] = li if ls[i] is None else ls[i] + li
            os_[i] = oi if os_[i] is None else os_[i] + oi
    return [o * _recip(jnp.sum(l, axis=1, keepdims=True)) for o, l in zip(os_, ls)]


def attn_heads(qc_s, k_s, v_s, g, it):
    row = jax.lax.broadcasted_iota(jnp.int32, (TB, TB), 0)
    col = jax.lax.broadcasted_iota(jnp.int32, (TB, TB), 1)
    tri = col <= row
    items = [(u, r) for u in range(HU) for r in BLOCK_ORDER[u]]
    pend = {}
    done = {}

    def store(item):
        u, r = item
        for j, o in enumerate(done.pop(item)):
            r0 = r * TQ + j * TB
            qc_s[HG + g * HG + it * HU + u, r0:r0 + TB, :] = o.astype(BF16)

    for t in range(len(items) + 1):
        if t < len(items):
            u, r = items[t]
            hh = it * HU + u
            pend[items[t]] = _attn_scores(qc_s.at[hh], k_s.at[hh], r * TQ, tri)
        if t >= 1 + LAG:
            store(items[t - 1 - LAG])
        if t >= 1:
            u, r = items[t - 1]
            hh = it * HU + u
            done[items[t - 1]] = _attn_values(v_s.at[hh], r * TQ, *pend.pop(items[t - 1]))
    for item in list(done):
        store(item)


def _kernel(xt_hbm, wqkv_hbm, woa_hbm, c_hbm, wq_hbm, wuk_hbm, wuv_hbm, wob_hbm, gate_hbm,
            out_hbm,
            xt_s, x_s, wqkv_s, woa_s, c_s, wq_raw, wuk_raw, wuv_raw, wob_s, gate_s,
            wt_s, wpt_s, wof_s, woap_s, woapt_s, qa_s, kl_s, vl_s, g_s,
            qc_s, k_s, v_s, out_s, sems, xsems, wsems, osems):
    copies = {
        "gate": pltpu.make_async_copy(gate_hbm, gate_s, sems.at[2]),
        "woa": pltpu.make_async_copy(woa_hbm, woa_s, sems.at[3]),
        "c": pltpu.make_async_copy(c_hbm, c_s, sems.at[4]),
        "wob": pltpu.make_async_copy(wob_hbm, wob_s, sems.at[5]),
    }
    w_cols = (0, 5 * 128, 9 * 128, 3 * M)
    w_copies = [pltpu.make_async_copy(wqkv_hbm.at[:, pl.ds(w_cols[i], w_cols[i + 1] - w_cols[i])],
                                      wqkv_s.at[pl.ds(0, M), pl.ds(w_cols[i], w_cols[i + 1] - w_cols[i])],
                                      xsems.at[NXC + i]) for i in range(3)]
    xw = S // NXC
    x_copies = [pltpu.make_async_copy(xt_hbm.at[:, pl.ds(i * xw, xw)], xt_s.at[:, pl.ds(i * xw, xw)], xsems.at[i])
                for i in range(NXC)]
    def pair_copies(wi, j):
        w_hbm, raw = ((wq_hbm, wq_raw), (wuk_hbm, wuk_raw), (wuv_hbm, wuv_raw))[wi]
        n = w_hbm.shape[0] // NSPLIT
        return [pltpu.make_async_copy(
            w_hbm.bitcast(jnp.uint32).at[pl.ds(p * n, n), j, :], raw.at[j, pl.ds(p * n, n), :],
            wsems.at[wi * NPAIR + j]) for p in range(NSPLIT)]

    def group_copies(g):
        return [cp for b in range(HG // 2) for wi in range(3) for cp in pair_copies(wi, g * (HG // 2) + b)]

    chain = w_copies + x_copies + [copies["woa"]]
    copies["gate"].start()
    chain[0].start()
    chain[1].start()

    def chain_wait(i):
        chain[i].wait()
        chain[i + 2].start()

    def make_eye():
        return (jax.lax.broadcasted_iota(jnp.int32, (128, 128), 0)
                == jax.lax.broadcasted_iota(jnp.int32, (128, 128), 1)).astype(BF16)

    def a_prep():
        wqkv_s[M:MP, :] = jnp.zeros((MP - M, 3 * M), BF16)
        zero_halo = jnp.zeros((HALO, 128), F32)
        for j in range(NT_M):
            kl_s[j, 0:HALO, :] = zero_halo
            vl_s[j, 0:HALO, :] = zero_halo
        wpt_s[3 * M:NPK * 128, :] = jnp.zeros((NPK * 128 - 3 * M, M), BF16)
        woap_s[DF * H:DF * H + 64, :] = jnp.zeros((64, M), BF16)
        eye = make_eye()

        for sec in range(3):
            chain_wait(sec)
            for c0 in range(w_cols[sec], w_cols[sec + 1], 128):
                wd = min(128, 3 * M - c0)
                wt = _dot(eye[0:wd, 0:wd], wqkv_s[:, c0:c0 + wd], NT)
                for j in range(NT_M):
                    wt_s[j, c0:c0 + wd, :] = wt[:, j * 128:(j + 1) * 128]
            for d in range(DHA):
                for j in range(NT_M):
                    rows = wt_s[j, pl.ds(sec * M + d, H, stride=DHA), :]
                    wj = min(128, M - j * 128)
                    p0 = _packed_row(sec, d)
                    wpt_s[p0:p0 + H, j * 128:j * 128 + wj] = rows[:, 0:wj].astype(BF16)
        copies["gate"].wait()
        chain_wait(3)
        chain[6].start()
        chain[7].start()
        a_xpose(0, xw)

    def a_prep_rest(c):
        per = xw // RAP

        @pl.when(c == per - 1)
        def _():
            copies["c"].start()
            for cp in group_copies(0):
                cp.start()
            chain[4].wait()
            a_xpose(xw, 2 * xw)

        @pl.when(c == 2 * per - 1)
        def _():
            chain[5].wait()
            chain[7].wait()
            a_xpose(2 * xw, 3 * xw)
            a_prep_wo()

        @pl.when(c == 3 * per - 1)
        def _():
            chain[6].wait()
            a_xpose(3 * xw, 4 * xw)

    def a_prep_wo():
        eye = make_eye()
        woa = woa_s[...].astype(F32)
        for j in range(NT_M):
            wj = min(128, M - j * 128)
            blk = woa[:, j * 128:j * 128 + wj]
            if wj < 128:
                blk = jnp.concatenate([blk, jnp.zeros((M, 128 - wj), F32)], axis=1)
            wof_s[j] = blk
        for d in range(DHA):
            for j in range(NT_M):
                wj = min(128, M - j * 128)
                rows = wof_s[j, pl.ds(d, H, stride=DHA), :]
                p0 = d * H if d < DF else d * H + 64
                woap_s[p0:p0 + H, j * 128:j * 128 + wj] = rows[:, 0:wj].astype(BF16)
        for j in range(NT_M):
            wj = min(128, M - j * 128)
            woapt_s[j * 128:j * 128 + wj, :] = _dot(
                eye[0:wj, 0:wj], woap_s[:, j * 128:j * 128 + wj], NT).astype(BF16)

    def a_xpose(t0, t1):
        eye = make_eye()
        for t in range(t0 // 128, t1 // 128):
            x_s[t * 128:(t + 1) * 128, :] = _dot(eye, xt_s[:, t * 128:(t + 1) * 128], NT).astype(BF16)
        gw = jnp.broadcast_to(gate_s[...].reshape(1, M), (16, M))
        g_s[:, t0:t1] = jax.nn.sigmoid(_dot(gw, xt_s[:, t0:t1]))

    a_scale = (DHA ** -0.5) * LOG2E

    def a_proj(c, carry):
        a_prep_rest(c)
        r0 = pl.multiple_of(c * RAP, RAP)
        rk = pl.multiple_of(HALO + c * RAP, HALO)
        xq = x_s[pl.ds(r0, RAP), :]
        nf = DF * H
        q = _dot(xq, wpt_s[0:nf, :], NT)
        for j in range(NT_M - 1):
            qa_s[j, pl.ds(r0, RAP), :] = q[:, j * 128:(j + 1) * 128]
        k = _dot(xq, wpt_s[nf:2 * nf, :], NT) * a_scale
        for j in range(NT_M - 1):
            kl_s[j, pl.ds(rk, RAP), :] = k[:, j * 128:(j + 1) * 128]
        v = _dot(xq, wpt_s[2 * nf:3 * nf, :], NT)
        for j in range(NT_M - 1):
            vl_s[j, pl.ds(rk, RAP), :] = v[:, j * 128:(j + 1) * 128]
        t = _dot(xq, wpt_s[3 * nf:NPK * 128, :], NT)
        vl_s[NT_M - 1, pl.ds(rk, RAP), :] = t[:, 0:128]
        kl_s[NT_M - 1, pl.ds(rk, RAP), :] = t[:, 128:256] * a_scale
        return carry

    def a_local(r0, sb, dz):
        qv = [qa_s.at[j, pl.ds(r0, RA), :] for j in range(NT_M - 1)]
        kv = [kl_s.at[j, pl.ds(r0, HALO + RA), :] for j in range(NT_M)]
        vv = [vl_s.at[j, pl.ds(r0, HALO + RA), :] for j in range(NT_M)]
        outs = []
        for b0 in range(sb * RS, (sb + 1) * RS, RG):
            qt = [qv[j][b0:b0 + RG, :] for j in range(NT_M - 1)]
            qt.append(vv[NT_M - 1][HALO + b0:HALO + b0 + RG, :])
            logits = []
            for w in range(WIN):
                off = HALO + b0 - w * DIL
                s = None
                for j in range(NT_M):
                    t = qt[j] * kv[j][off:off + RG, :]
                    s = t if s is None else s + t
                s = s + pltpu.roll(s, 64, 1)
                s = s + pltpu.roll(s, 32, 1)
                if b0 < w * DIL:
                    rowi = jax.lax.broadcasted_iota(jnp.int32, (RG, 128), 0) + (r0 + b0)
                    s = jnp.where(rowi >= w * DIL, s, NEG * LOG2E)
                logits.append(s)
            m = functools.reduce(jnp.maximum, logits)
            ps = [jnp.exp2(s - m) for s in logits]
            r = _recip(functools.reduce(jnp.add, ps))
            ot = []
            for j in range(NT_M):
                o = None
                for w in range(WIN):
                    off = HALO + b0 - w * DIL
                    t = ps[w] * vv[j][off:off + RG, :]
                    o = t if o is None else o + t
                ot.append(o * r)
            outs.append(ot)
        for j in range(NT_M):
            o = jnp.concatenate([ot[j] for ot in outs], axis=0)
            qc_s[HG + H + j + dz, pl.ds(pl.multiple_of(r0 + sb * RS, RS), RS), :] = o.astype(BF16)

    def a_main():
        jax.lax.fori_loop(0, S // RAP, a_proj, 0)

    def group_weights(raw, g):
        cols = []
        for b in range(HG // 2):
            u = raw[g * (HG // 2) + b]
            cols.append(pltpu.bitcast(u << 16, F32).astype(BF16))
            cols.append(pltpu.bitcast(u & jnp.uint32(0xFFFF0000), F32).astype(BF16))
        return jnp.concatenate(cols, axis=1)

    b_scale = (D ** -0.5) * LOG2E

    def group_body(g, carry):
        @pl.when(g > 0)
        def _():
            for cp in group_copies(g):
                cp.wait()

        def proj_body(rc, c2):
            r0 = pl.multiple_of(rc * RP, RP)
            ra = pl.multiple_of((g * (S // RP) + rc) * RA, RA)

            def proj(src, raw, dst, scale, part):
                n = RP // PSPLIT
                rows = pl.ds(pl.multiple_of(r0 + part * n, n), n)
                y = _dot(src[rows, :], group_weights(raw, g))
                if scale is not None:
                    y = y * scale
                for i in range(HG):
                    dst[i, rows, :] = y[:, i * D:(i + 1) * D].astype(BF16)

            count = {"q": 0, "k": 0, "v": 0}
            for ch in PROJ_SEQ:
                if ch in count:
                    src, raw, dst, scale = {"q": (x_s, wq_raw, qc_s, b_scale), "k": (c_s, wuk_raw, k_s, None),
                                            "v": (c_s, wuv_raw, v_s, None)}[ch]
                    proj(src, raw, dst, scale, count[ch])
                    count[ch] += 1
                else:
                    a_local(ra, int(ch, 36), jnp.minimum(g, 0) if DYNZ else 0)
            return c2

        with jax.named_scope("B_proj"):
            jax.lax.fori_loop(0, S // RP, proj_body, 0)

        def attn_body(it, c2):
            attn_heads(qc_s, k_s, v_s, g, it)
            return c2

        with jax.named_scope("B_attn"):
            jax.lax.fori_loop(0, HG // HU, attn_body, 0)
        return carry

    def out_copy(i):
        r0 = i * RO
        if not isinstance(i, int):
            r0 = pl.multiple_of(r0, RO)
        return pltpu.make_async_copy(out_s.at[:, pl.ds(r0, RO)], out_hbm.at[0, :, pl.ds(r0, RO)], osems.at[i])

    def out_body(i, carry):
        r0 = pl.multiple_of(i * RO, RO)
        ctx = jnp.concatenate([qc_s[HG + h, pl.ds(r0, RO), :] for h in range(H)], axis=1)
        wo = jnp.concatenate([wob_s[h] for h in range(H)], axis=1)
        bt = _dot(wo, ctx, NT)
        oa = jnp.concatenate([qc_s[HG + H + j, pl.ds(r0, RO), :] for j in range(NT_M)], axis=1)
        at = _dot(woapt_s[...], oa, NT)
        gt = g_s[0:1, pl.ds(r0, RO)]
        out_s[:, pl.ds(r0, RO)] = (gt * at + (1.0 - gt) * bt).astype(BF16)
        out_copy(i).start()
        return carry

    with jax.named_scope("A_prep"):
        a_prep()
    with jax.named_scope("A_main"):
        a_main()
        copies["c"].wait()
        for cp in group_copies(0):
            cp.wait()
        for g in range(1, NG):
            for cp in group_copies(g):
                cp.start()
        copies["wob"].start()
    jax.lax.fori_loop(0, NG, group_body, 0)
    with jax.named_scope("B_out"):
        copies["wob"].wait()
        jax.lax.fori_loop(0, S // RO, out_body, 0)
        for i in range(S // RO):
            out_copy(i).wait()


@jax.jit
def pallas_gated_mix__sliding_local_dilated__compressed_kv_cla__prompt_kernel(
    A_x: jax.Array,
    A_wqkv: jax.Array,
    A_wo: jax.Array,
    B_x: jax.Array,
    B_c_kv: jax.Array,
    B_w_q: jax.Array,
    B_w_uk: jax.Array,
    B_w_uv: jax.Array,
    B_w_o: jax.Array,
    gate_w: jax.Array,
):
    del B_x
    xt = jnp.swapaxes(A_x, 1, 2).reshape(M, S)
    c = B_c_kv.reshape(S, DC)
    wob = jnp.swapaxes(B_w_o, 1, 2)

    any_spec = pl.BlockSpec(memory_space=pl.ANY)
    scratch = [
        pltpu.VMEM((M, S), BF16),
        pltpu.VMEM((S, M), BF16),
        pltpu.VMEM((MP, 3 * M), BF16),
        pltpu.VMEM((M, M), BF16),
        pltpu.VMEM((S, DC), BF16),
        pltpu.VMEM((NPAIR, M, D), jnp.uint32),
        pltpu.VMEM((NPAIR, DC, D), jnp.uint32),
        pltpu.VMEM((NPAIR, DC, D), jnp.uint32),
        pltpu.VMEM((H, M, D), BF16),
        pltpu.VMEM((M,), BF16),
        pltpu.VMEM((NT_M, 14 * 128, 128), F32),
        pltpu.VMEM((NPK * 128, M), BF16),
        pltpu.VMEM((NT_M, M, 128), F32),
        pltpu.VMEM((MP, M), BF16),
        pltpu.VMEM((M, MP), BF16),
        pltpu.VMEM((NT_M - 1, S, 128), F32),
        pltpu.VMEM((NT_M, HALO + S, 128), F32),
        pltpu.VMEM((NT_M, HALO + S, 128), F32),
        pltpu.VMEM((16, S), F32),
        pltpu.VMEM((HG + H + NT_M, S, D), BF16),
        pltpu.VMEM((HG, S, D), BF16),
        pltpu.VMEM((HG, S, D), BF16),
        pltpu.VMEM((M, S), BF16),
        pltpu.SemaphoreType.DMA((6,)),
        pltpu.SemaphoreType.DMA((NXC + 3,)),
        pltpu.SemaphoreType.DMA((3 * NPAIR,)),
        pltpu.SemaphoreType.DMA((S // RO,)),
    ]
    out_t = pl.pallas_call(
        _kernel,
        out_shape=jax.ShapeDtypeStruct((1, M, S), BF16),
        in_specs=[any_spec] * 9,
        out_specs=any_spec,
        scratch_shapes=scratch,
        compiler_params=pltpu.CompilerParams(vmem_limit_bytes=120 * 1024 * 1024),
        name="gated_mix",
    )(xt, A_wqkv, A_wo, c, B_w_q, B_w_uk, B_w_uv, wob, gate_w)
    return jnp.swapaxes(out_t, 1, 2)
```

```python
import functools
import math

import jax
import jax.numpy as jnp
import jax.experimental.pallas as pl
import jax.experimental.pallas.tpu as pltpu

F32 = jnp.float32
BF16 = jnp.bfloat16

S = 2048
M = 576
MP = 640
NT_M = MP // 128
H = 32
D = 128
DC = 512
DHA = 18
WIN = 8
DIL = 2
HALO = 16
DF = 16
NPK = 14
LOG2E = math.log2(math.e)
NEG = -1e9

RAP = 256
RA = 256
RG = 8
RS = 32
HG = 8
NG = H // HG
RP = 1024
TQ = 256
TB = 128
HU = 2
BLOCK_ORDER = ((1, 3, 7, 6, 5, 4, 2, 0), (6, 7, 4, 5, 2, 3, 1, 0))
assert all(sorted(o) == list(range(S // TQ)) for o in BLOCK_ORDER) and len(BLOCK_ORDER) == HU
OUT_ORDER = 0
PSPLIT = 1
DYNZ = 0
PROJ_SEQ = "01v234q56k7"
LAG = 1
RO = 256
assert NG * (S // RP) == S // RA
NXC = 4
NSPLIT = 1
NPAIR = H // 2

NN = (((1,), (0,)), ((), ()))
NT = (((1,), (1,)), ((), ()))


def _dot(a, b, dims=NN):
    return jax.lax.dot_general(a, b, dims, preferred_element_type=F32)


def _packed_row(sec, d):
    if d < DF:
        return (sec * DF + d) * H
    return 3 * DF * H + ((0, 4, 2)[sec] + d - DF) * H


def _lane_partial(s, op):
    acc = s[:, 0:128]
    for j in range(1, s.shape[1] // 128):
        acc = op(acc, s[:, j * 128:(j + 1) * 128])
    return acc


def _recip(l):
    r = pl.reciprocal(l, approx=True)
    return r * (2.0 - l * r)


def _segments(r0):
    nsub = TQ // TB
    segs = []
    if r0 > 0:
        segs.append((0, TQ, 0, r0, False))
    for j in range(nsub):
        segs.append((j * TB, (j + 1) * TB, r0 + j * TB, r0 + (j + 1) * TB, True))
        if (j + 1) * TB < TQ:
            segs.append(((j + 1) * TB, TQ, r0 + j * TB, r0 + (j + 1) * TB, False))
    return segs


def _attn_scores(q_ref, k_ref, r0, tri):
    nsub = TQ // TB
    segs = _segments(r0)
    ss = []
    for (a, b, c, d, msk) in segs:
        s = _dot(q_ref[r0 + a:r0 + b, :], k_ref[c:d, :], NT)
        if msk:
            s = jnp.where(tri, s, NEG * LOG2E)
        ss.append(s)
    ms = []
    for i in range(nsub):
        m = None
        for (a, b, c, d, msk), s in zip(segs, ss):
            if a <= i * TB and (i + 1) * TB <= b:
                sm = _lane_partial(s[i * TB - a:(i + 1) * TB - a], jnp.maximum)
                m = sm if m is None else jnp.maximum(m, sm)
        ms.append(jnp.max(m, axis=1, keepdims=True))
    return ss, ms


def _attn_values(v_ref, r0, ss, ms):
    nsub = TQ // TB
    segs = _segments(r0)
    ls = [None] * nsub
    os_ = [None] * nsub
    for (a, b, c, d, msk), s in zip(segs, ss):
        m = jnp.concatenate(ms[a // TB:b // TB], axis=0) if b - a > TB else ms[a // TB]
        p = jnp.exp2(s - m)
        l = _lane_partial(p, jnp.add)
        o = _dot(p.astype(BF16), v_ref[c:d, :])
        for i in range(a // TB, b // TB):
            li = l[i * TB - a:(i + 1) * TB - a]
            oi = o[i * TB - a:(i + 1) * TB - a]
            ls[i] = li if ls[i] is None else ls[i] + li
            os_[i] = oi if os_[i] is None else os_[i] + oi
    return [o * _recip(jnp.sum(l, axis=1, keepdims=True)) for o, l in zip(os_, ls)]


def attn_heads(qc_s, k_s, v_s, g, it):
    row = jax.lax.broadcasted_iota(jnp.int32, (TB, TB), 0)
    col = jax.lax.broadcasted_iota(jnp.int32, (TB, TB), 1)
    tri = col <= row
    items = [(u, r) for u in range(HU) for r in BLOCK_ORDER[u]]
    pend = {}
    done = {}

    def store(item):
        u, r = item
        for j, o in enumerate(done.pop(item)):
            r0 = r * TQ + j * TB
            qc_s[HG + g * HG + it * HU + u, r0:r0 + TB, :] = o.astype(BF16)

    for t in range(len(items) + 1):
        if t < len(items):
            u, r = items[t]
            hh = it * HU + u
            pend[items[t]] = _attn_scores(qc_s.at[hh], k_s.at[hh], r * TQ, tri)
        if t >= 1 + LAG:
            store(items[t - 1 - LAG])
        if t >= 1:
            u, r = items[t - 1]
            hh = it * HU + u
            done[items[t - 1]] = _attn_values(v_s.at[hh], r * TQ, *pend.pop(items[t - 1]))
    for item in list(done):
        store(item)


def _kernel(xt_hbm, wqkv_hbm, woa_hbm, c_hbm, wq_hbm, wuk_hbm, wuv_hbm, wob_hbm, gate_hbm,
            out_hbm,
            xt_s, x_s, wqkv_s, woa_s, c_s, wq_raw, wuk_raw, wuv_raw, wob_s, gate_s,
            wt_s, wpt_s, wof_s, woap_s, woapt_s, qa_s, kl_s, vl_s, g_s,
            qc_s, k_s, v_s, out_s, sems, xsems, wsems, osems):
    copies = {
        "gate": pltpu.make_async_copy(gate_hbm, gate_s, sems.at[2]),
        "woa": pltpu.make_async_copy(woa_hbm, woa_s, sems.at[3]),
        "c": pltpu.make_async_copy(c_hbm, c_s, sems.at[4]),
        "wob": pltpu.make_async_copy(wob_hbm, wob_s, sems.at[5]),
    }
    w_cols = (0, 5 * 128, 9 * 128, 3 * M)
    w_copies = [pltpu.make_async_copy(wqkv_hbm.at[:, pl.ds(w_cols[i], w_cols[i + 1] - w_cols[i])],
                                      wqkv_s.at[pl.ds(0, M), pl.ds(w_cols[i], w_cols[i + 1] - w_cols[i])],
                                      xsems.at[NXC + i]) for i in range(3)]
    xw = S // NXC
    x_copies = [pltpu.make_async_copy(xt_hbm.at[:, pl.ds(i * xw, xw)], xt_s.at[:, pl.ds(i * xw, xw)], xsems.at[i])
                for i in range(NXC)]
    def pair_copies(wi, j):
        w_hbm, raw = ((wq_hbm, wq_raw), (wuk_hbm, wuk_raw), (wuv_hbm, wuv_raw))[wi]
        n = w_hbm.shape[0] // NSPLIT
        return [pltpu.make_async_copy(
            w_hbm.bitcast(jnp.uint32).at[pl.ds(p * n, n), j, :], raw.at[j, pl.ds(p * n, n), :],
            wsems.at[wi * NPAIR + j]) for p in range(NSPLIT)]

    def group_copies(g):
        return [cp for b in range(HG // 2) for wi in range(3) for cp in pair_copies(wi, g * (HG // 2) + b)]

    chain = w_copies + x_copies + [copies["woa"]]
    copies["gate"].start()
    chain[0].start()
    chain[1].start()

    def chain_wait(i):
        chain[i].wait()
        chain[i + 2].start()

    def make_eye():
        return (jax.lax.broadcasted_iota(jnp.int32, (128, 128), 0)
                == jax.lax.broadcasted_iota(jnp.int32, (128, 128), 1)).astype(BF16)

    def a_prep():
        wqkv_s[M:MP, :] = jnp.zeros((MP - M, 3 * M), BF16)
        zero_halo = jnp.zeros((HALO, 128), F32)
        for j in range(NT_M):
            kl_s[j, 0:HALO, :] = zero_halo
            vl_s[j, 0:HALO, :] = zero_halo
        wpt_s[3 * M:NPK * 128, :] = jnp.zeros((NPK * 128 - 3 * M, M), BF16)
        woap_s[DF * H:DF * H + 64, :] = jnp.zeros((64, M), BF16)
        eye = make_eye()

        for sec in range(3):
            chain_wait(sec)
            for c0 in range(w_cols[sec], w_cols[sec + 1], 128):
                wd = min(128, 3 * M - c0)
                wt = _dot(eye[0:wd, 0:wd], wqkv_s[:, c0:c0 + wd], NT)
                for j in range(NT_M):
                    wt_s[j, c0:c0 + wd, :] = wt[:, j * 128:(j + 1) * 128]
            for d in range(DHA):
                for j in range(NT_M):
                    rows = wt_s[j, pl.ds(sec * M + d, H, stride=DHA), :]
                    wj = min(128, M - j * 128)
                    p0 = _packed_row(sec, d)
                    wpt_s[p0:p0 + H, j * 128:j * 128 + wj] = rows[:, 0:wj].astype(BF16)
        copies["gate"].wait()
        chain_wait(3)
        chain[6].start()
        chain[7].start()
        a_xpose(0, xw)

    def a_prep_rest(c):
        per = xw // RAP

        @pl.when(c == per - 1)
        def _():
            copies["c"].start()
            for cp in group_copies(0):
                cp.start()
            chain[4].wait()
            a_xpose(xw, 2 * xw)

        @pl.when(c == 2 * per - 1)
        def _():
            chain[5].wait()
            chain[7].wait()
            a_xpose(2 * xw, 3 * xw)
            a_prep_wo()

        @pl.when(c == 3 * per - 1)
        def _():
            chain[6].wait()
            a_xpose(3 * xw, 4 * xw)

    def a_prep_wo():
        eye = make_eye()
        woa = woa_s[...].astype(F32)
        for j in range(NT_M):
            wj = min(128, M - j * 128)
            blk = woa[:, j * 128:j * 128 + wj]
            if wj < 128:
                blk = jnp.concatenate([blk, jnp.zeros((M, 128 - wj), F32)], axis=1)
            wof_s[j] = blk
        for d in range(DHA):
            for j in range(NT_M):
                wj = min(128, M - j * 128)
                rows = wof_s[j, pl.ds(d, H, stride=DHA), :]
                p0 = d * H if d < DF else d * H + 64
                woap_s[p0:p0 + H, j * 128:j * 128 + wj] = rows[:, 0:wj].astype(BF16)
        for j in range(NT_M):
            wj = min(128, M - j * 128)
            woapt_s[j * 128:j * 128 + wj, :] = _dot(
                eye[0:wj, 0:wj], woap_s[:, j * 128:j * 128 + wj], NT).astype(BF16)

    def a_xpose(t0, t1):
        eye = make_eye()
        for t in range(t0 // 128, t1 // 128):
            x_s[t * 128:(t + 1) * 128, :] = _dot(eye, xt_s[:, t * 128:(t + 1) * 128], NT).astype(BF16)
        gw = jnp.broadcast_to(gate_s[...].reshape(1, M), (16, M))
        g_s[:, t0:t1] = jax.nn.sigmoid(_dot(gw, xt_s[:, t0:t1]))

    a_scale = (DHA ** -0.5) * LOG2E

    def a_proj(c, carry):
        a_prep_rest(c)
        r0 = pl.multiple_of(c * RAP, RAP)
        rk = pl.multiple_of(HALO + c * RAP, HALO)
        xq = x_s[pl.ds(r0, RAP), :]
        nf = DF * H
        q = _dot(xq, wpt_s[0:nf, :], NT)
        for j in range(NT_M - 1):
            qa_s[j, pl.ds(r0, RAP), :] = q[:, j * 128:(j + 1) * 128]
        k = _dot(xq, wpt_s[nf:2 * nf, :], NT) * a_scale
        for j in range(NT_M - 1):
            kl_s[j, pl.ds(rk, RAP), :] = k[:, j * 128:(j + 1) * 128]
        v = _dot(xq, wpt_s[2 * nf:3 * nf, :], NT)
        for j in range(NT_M - 1):
            vl_s[j, pl.ds(rk, RAP), :] = v[:, j * 128:(j + 1) * 128]
        t = _dot(xq, wpt_s[3 * nf:NPK * 128, :], NT)
        vl_s[NT_M - 1, pl.ds(rk, RAP), :] = t[:, 0:128]
        kl_s[NT_M - 1, pl.ds(rk, RAP), :] = t[:, 128:256] * a_scale
        return carry

    def a_local(r0, sb, dz):
        qv = [qa_s.at[j, pl.ds(r0, RA), :] for j in range(NT_M - 1)]
        kv = [kl_s.at[j, pl.ds(r0, HALO + RA), :] for j in range(NT_M)]
        vv = [vl_s.at[j, pl.ds(r0, HALO + RA), :] for j in range(NT_M)]
        outs = []
        for b0 in range(sb * RS, (sb + 1) * RS, RG):
            qt = [qv[j][b0:b0 + RG, :] for j in range(NT_M - 1)]
            qt.append(vv[NT_M - 1][HALO + b0:HALO + b0 + RG, :])
            logits = []
            for w in range(WIN):
                off = HALO + b0 - w * DIL
                s = None
                for j in range(NT_M):
                    t = qt[j] * kv[j][off:off + RG, :]
                    s = t if s is None else s + t
                s = s + pltpu.roll(s, 64, 1)
                s = s + pltpu.roll(s, 32, 1)
                if b0 < w * DIL:
                    rowi = jax.lax.broadcasted_iota(jnp.int32, (RG, 128), 0) + (r0 + b0)
                    s = jnp.where(rowi >= w * DIL, s, NEG * LOG2E)
                logits.append(s)
            m = functools.reduce(jnp.maximum, logits)
            ps = [jnp.exp2(s - m) for s in logits]
            r = _recip(functools.reduce(jnp.add, ps))
            ot = []
            for j in range(NT_M):
                o = None
                for w in range(WIN):
                    off = HALO + b0 - w * DIL
                    t = ps[w] * vv[j][off:off + RG, :]
                    o = t if o is None else o + t
                ot.append(o * r)
            outs.append(ot)
        for j in range(NT_M):
            o = jnp.concatenate([ot[j] for ot in outs], axis=0)
            qc_s[HG + H + j + dz, pl.ds(pl.multiple_of(r0 + sb * RS, RS), RS), :] = o.astype(BF16)

    def a_main():
        jax.lax.fori_loop(0, S // RAP, a_proj, 0)

    def group_weights(raw, g):
        cols = []
        for b in range(HG // 2):
            u = raw[g * (HG // 2) + b]
            cols.append(pltpu.bitcast(u << 16, F32).astype(BF16))
            cols.append(pltpu.bitcast(u & jnp.uint32(0xFFFF0000), F32).astype(BF16))
        return jnp.concatenate(cols, axis=1)

    b_scale = (D ** -0.5) * LOG2E

    def group_body(g, carry):
        @pl.when(g > 0)
        def _():
            for cp in group_copies(g):
                cp.wait()

        def proj_body(rc, c2):
            r0 = pl.multiple_of(rc * RP, RP)
            ra = pl.multiple_of((g * (S // RP) + rc) * RA, RA)

            def proj(src, raw, dst, scale, part):
                n = RP // PSPLIT
                rows = pl.ds(pl.multiple_of(r0 + part * n, n), n)
                y = _dot(src[rows, :], group_weights(raw, g))
                if scale is not None:
                    y = y * scale
                for i in range(HG):
                    dst[i, rows, :] = y[:, i * D:(i + 1) * D].astype(BF16)

            count = {"q": 0, "k": 0, "v": 0}
            for ch in PROJ_SEQ:
                if ch in count:
                    src, raw, dst, scale = {"q": (x_s, wq_raw, qc_s, b_scale), "k": (c_s, wuk_raw, k_s, None),
                                            "v": (c_s, wuv_raw, v_s, None)}[ch]
                    proj(src, raw, dst, scale, count[ch])
                    count[ch] += 1
                else:
                    a_local(ra, int(ch, 36), jnp.minimum(g, 0) if DYNZ else 0)
            return c2

        with jax.named_scope("B_proj"):
            jax.lax.fori_loop(0, S // RP, proj_body, 0)

        def attn_body(it, c2):
            attn_heads(qc_s, k_s, v_s, g, it)
            return c2

        with jax.named_scope("B_attn"):
            jax.lax.fori_loop(0, HG // HU, attn_body, 0)
        return carry

    def out_copy(i):
        r0 = i * RO
        if not isinstance(i, int):
            r0 = pl.multiple_of(r0, RO)
        return pltpu.make_async_copy(out_s.at[:, pl.ds(r0, RO)], out_hbm.at[0, :, pl.ds(r0, RO)], osems.at[i])

    def out_body(i, carry):
        r0 = pl.multiple_of(i * RO, RO)

        def branch_b():
            ctx = jnp.concatenate([qc_s[HG + h, pl.ds(r0, RO), :] for h in range(H)], axis=1)
            wo = jnp.concatenate([wob_s[h] for h in range(H)], axis=1)
            return _dot(wo, ctx, NT)

        def branch_a():
            oa = jnp.concatenate([qc_s[HG + H + j, pl.ds(r0, RO), :] for j in range(NT_M)], axis=1)
            return _dot(woapt_s[...], oa, NT)

        gt = g_s[0:1, pl.ds(r0, RO)]
        if OUT_ORDER == 0:
            bt = branch_b()
            at = branch_a()
        else:
            at = branch_a() * gt
            bt = branch_b()
        if OUT_ORDER == 0:
            out = gt * at + (1.0 - gt) * bt
        else:
            out = at + (1.0 - gt) * bt
        out_s[:, pl.ds(r0, RO)] = out.astype(BF16)
        out_copy(i).start()
        return carry

    with jax.named_scope("A_prep"):
        a_prep()
    with jax.named_scope("A_main"):
        a_main()
        copies["c"].wait()
        for cp in group_copies(0):
            cp.wait()
        for g in range(1, NG):
            for cp in group_copies(g):
                cp.start()
        copies["wob"].start()
    jax.lax.fori_loop(0, NG, group_body, 0)
    with jax.named_scope("B_out"):
        copies["wob"].wait()
        jax.lax.fori_loop(0, S // RO, out_body, 0)
        for i in range(S // RO):
            out_copy(i).wait()


@jax.jit
def pallas_gated_mix__sliding_local_dilated__compressed_kv_cla__prompt_kernel(
    A_x: jax.Array,
    A_wqkv: jax.Array,
    A_wo: jax.Array,
    B_x: jax.Array,
    B_c_kv: jax.Array,
    B_w_q: jax.Array,
    B_w_uk: jax.Array,
    B_w_uv: jax.Array,
    B_w_o: jax.Array,
    gate_w: jax.Array,
):
    del B_x
    xt = jnp.swapaxes(A_x, 1, 2).reshape(M, S)
    c = B_c_kv.reshape(S, DC)
    wob = jnp.swapaxes(B_w_o, 1, 2)

    any_spec = pl.BlockSpec(memory_space=pl.ANY)
    scratch = [
        pltpu.VMEM((M, S), BF16),
        pltpu.VMEM((S, M), BF16),
        pltpu.VMEM((MP, 3 * M), BF16),
        pltpu.VMEM((M, M), BF16),
        pltpu.VMEM((S, DC), BF16),
        pltpu.VMEM((NPAIR, M, D), jnp.uint32),
        pltpu.VMEM((NPAIR, DC, D), jnp.uint32),
        pltpu.VMEM((NPAIR, DC, D), jnp.uint32),
        pltpu.VMEM((H, M, D), BF16),
        pltpu.VMEM((M,), BF16),
        pltpu.VMEM((NT_M, 14 * 128, 128), F32),
        pltpu.VMEM((NPK * 128, M), BF16),
        pltpu.VMEM((NT_M, M, 128), F32),
        pltpu.VMEM((MP, M), BF16),
        pltpu.VMEM((M, MP), BF16),
        pltpu.VMEM((NT_M - 1, S, 128), F32),
        pltpu.VMEM((NT_M, HALO + S, 128), F32),
        pltpu.VMEM((NT_M, HALO + S, 128), F32),
        pltpu.VMEM((16, S), F32),
        pltpu.VMEM((HG + H + NT_M, S, D), BF16),
        pltpu.VMEM((HG, S, D), BF16),
        pltpu.VMEM((HG, S, D), BF16),
        pltpu.VMEM((M, S), BF16),
        pltpu.SemaphoreType.DMA((6,)),
        pltpu.SemaphoreType.DMA((NXC + 3,)),
        pltpu.SemaphoreType.DMA((3 * NPAIR,)),
        pltpu.SemaphoreType.DMA((S // RO,)),
    ]
    out_t = pl.pallas_call(
        _kernel,
        out_shape=jax.ShapeDtypeStruct((1, M, S), BF16),
        in_specs=[any_spec] * 9,
        out_specs=any_spec,
        scratch_shapes=scratch,
        compiler_params=pltpu.CompilerParams(vmem_limit_bytes=120 * 1024 * 1024),
        name="gated_mix",
    )(xt, A_wqkv, A_wo, c, B_w_q, B_w_uk, B_w_uv, wob, gate_w)
    return jnp.swapaxes(out_t, 1, 2)
```

```python
import functools
import math

import jax
import jax.numpy as jnp
import jax.experimental.pallas as pl
import jax.experimental.pallas.tpu as pltpu

F32 = jnp.float32
BF16 = jnp.bfloat16

S = 2048
M = 576
MP = 640
NT_M = MP // 128
H = 32
D = 128
DC = 512
DHA = 18
WIN = 8
DIL = 2
HALO = 16
DF = 16
NPK = 14
LOG2E = math.log2(math.e)
NEG = -1e9

RAP = 512
RA = 256
RG = 8
RS = 32
HG = 8
NG = H // HG
RP = 1024
TQ = 256
TB = 128
HU = 2
BLOCK_ORDER = ((1, 3, 7, 6, 5, 4, 2, 0), (6, 7, 4, 5, 2, 3, 1, 0))
assert all(sorted(o) == list(range(S // TQ)) for o in BLOCK_ORDER) and len(BLOCK_ORDER) == HU
OUT_ORDER = 0
PSPLIT = 1
DYNZ = 0
PROJ_SEQ = "01v234q56k7"
LAG = 1
RO = 256
assert NG * (S // RP) == S // RA
NXC = 4
A_SEQ = "qkvt"
CB_AT = 1
WO_AT = 2
assert S // NXC == RAP
NSPLIT = 1
NPAIR = H // 2

NN = (((1,), (0,)), ((), ()))
NT = (((1,), (1,)), ((), ()))


def _dot(a, b, dims=NN):
    return jax.lax.dot_general(a, b, dims, preferred_element_type=F32)


def _packed_row(sec, d):
    if d < DF:
        return (sec * DF + d) * H
    return 3 * DF * H + ((0, 4, 2)[sec] + d - DF) * H


def _lane_partial(s, op):
    acc = s[:, 0:128]
    for j in range(1, s.shape[1] // 128):
        acc = op(acc, s[:, j * 128:(j + 1) * 128])
    return acc


def _recip(l):
    r = pl.reciprocal(l, approx=True)
    return r * (2.0 - l * r)


def _segments(r0):
    nsub = TQ // TB
    segs = []
    if r0 > 0:
        segs.append((0, TQ, 0, r0, False))
    for j in range(nsub):
        segs.append((j * TB, (j + 1) * TB, r0 + j * TB, r0 + (j + 1) * TB, True))
        if (j + 1) * TB < TQ:
            segs.append(((j + 1) * TB, TQ, r0 + j * TB, r0 + (j + 1) * TB, False))
    return segs


def _attn_scores(q_ref, k_ref, r0, tri):
    nsub = TQ // TB
    segs = _segments(r0)
    ss = []
    for (a, b, c, d, msk) in segs:
        s = _dot(q_ref[r0 + a:r0 + b, :], k_ref[c:d, :], NT)
        if msk:
            s = jnp.where(tri, s, NEG * LOG2E)
        ss.append(s)
    ms = []
    for i in range(nsub):
        m = None
        for (a, b, c, d, msk), s in zip(segs, ss):
            if a <= i * TB and (i + 1) * TB <= b:
                sm = _lane_partial(s[i * TB - a:(i + 1) * TB - a], jnp.maximum)
                m = sm if m is None else jnp.maximum(m, sm)
        ms.append(jnp.max(m, axis=1, keepdims=True))
    return ss, ms


def _attn_values(v_ref, r0, ss, ms):
    nsub = TQ // TB
    segs = _segments(r0)
    ls = [None] * nsub
    os_ = [None] * nsub
    for (a, b, c, d, msk), s in zip(segs, ss):
        m = jnp.concatenate(ms[a // TB:b // TB], axis=0) if b - a > TB else ms[a // TB]
        p = jnp.exp2(s - m)
        l = _lane_partial(p, jnp.add)
        o = _dot(p.astype(BF16), v_ref[c:d, :])
        for i in range(a // TB, b // TB):
            li = l[i * TB - a:(i + 1) * TB - a]
            oi = o[i * TB - a:(i + 1) * TB - a]
            ls[i] = li if ls[i] is None else ls[i] + li
            os_[i] = oi if os_[i] is None else os_[i] + oi
    return [o * _recip(jnp.sum(l, axis=1, keepdims=True)) for o, l in zip(os_, ls)]


def attn_heads(qc_s, k_s, v_s, g, it):
    row = jax.lax.broadcasted_iota(jnp.int32, (TB, TB), 0)
    col = jax.lax.broadcasted_iota(jnp.int32, (TB, TB), 1)
    tri = col <= row
    items = [(u, r) for u in range(HU) for r in BLOCK_ORDER[u]]
    pend = {}
    done = {}

    def store(item):
        u, r = item
        for j, o in enumerate(done.pop(item)):
            r0 = r * TQ + j * TB
            qc_s[HG + g * HG + it * HU + u, r0:r0 + TB, :] = o.astype(BF16)

    for t in range(len(items) + 1):
        if t < len(items):
            u, r = items[t]
            hh = it * HU + u
            pend[items[t]] = _attn_scores(qc_s.at[hh], k_s.at[hh], r * TQ, tri)
        if t >= 1 + LAG:
            store(items[t - 1 - LAG])
        if t >= 1:
            u, r = items[t - 1]
            hh = it * HU + u
            done[items[t - 1]] = _attn_values(v_s.at[hh], r * TQ, *pend.pop(items[t - 1]))
    for item in list(done):
        store(item)


def _kernel(xt_hbm, wqkv_hbm, woa_hbm, c_hbm, wq_hbm, wuk_hbm, wuv_hbm, wob_hbm, gate_hbm,
            out_hbm,
            xt_s, x_s, wqkv_s, woa_s, c_s, wq_raw, wuk_raw, wuv_raw, wob_s, gate_s,
            wt_s, wpt_s, wof_s, woap_s, woapt_s, qa_s, kl_s, vl_s, g_s,
            qc_s, k_s, v_s, out_s, sems, xsems, wsems, osems):
    copies = {
        "gate": pltpu.make_async_copy(gate_hbm, gate_s, sems.at[2]),
        "woa": pltpu.make_async_copy(woa_hbm, woa_s, sems.at[3]),
        "c": pltpu.make_async_copy(c_hbm, c_s, sems.at[4]),
        "wob": pltpu.make_async_copy(wob_hbm, wob_s, sems.at[5]),
    }
    w_cols = (0, 5 * 128, 9 * 128, 3 * M)
    w_copies = [pltpu.make_async_copy(wqkv_hbm.at[:, pl.ds(w_cols[i], w_cols[i + 1] - w_cols[i])],
                                      wqkv_s.at[pl.ds(0, M), pl.ds(w_cols[i], w_cols[i + 1] - w_cols[i])],
                                      xsems.at[NXC + i]) for i in range(3)]
    xw = S // NXC
    x_copies = [pltpu.make_async_copy(xt_hbm.at[:, pl.ds(i * xw, xw)], xt_s.at[:, pl.ds(i * xw, xw)], xsems.at[i])
                for i in range(NXC)]
    def pair_copies(wi, j):
        w_hbm, raw = ((wq_hbm, wq_raw), (wuk_hbm, wuk_raw), (wuv_hbm, wuv_raw))[wi]
        n = w_hbm.shape[0] // NSPLIT
        return [pltpu.make_async_copy(
            w_hbm.bitcast(jnp.uint32).at[pl.ds(p * n, n), j, :], raw.at[j, pl.ds(p * n, n), :],
            wsems.at[wi * NPAIR + j]) for p in range(NSPLIT)]

    def group_copies(g):
        return [cp for b in range(HG // 2) for wi in range(3) for cp in pair_copies(wi, g * (HG // 2) + b)]

    chain = w_copies + x_copies + [copies["woa"]]
    copies["gate"].start()
    chain[0].start()
    chain[1].start()

    def chain_wait(i):
        chain[i].wait()
        chain[i + 2].start()

    def make_eye():
        return (jax.lax.broadcasted_iota(jnp.int32, (128, 128), 0)
                == jax.lax.broadcasted_iota(jnp.int32, (128, 128), 1)).astype(BF16)

    def a_prep():
        wqkv_s[M:MP, :] = jnp.zeros((MP - M, 3 * M), BF16)
        zero_halo = jnp.zeros((HALO, 128), F32)
        for j in range(NT_M):
            kl_s[j, 0:HALO, :] = zero_halo
            vl_s[j, 0:HALO, :] = zero_halo
        wpt_s[3 * M:NPK * 128, :] = jnp.zeros((NPK * 128 - 3 * M, M), BF16)
        woap_s[DF * H:DF * H + 64, :] = jnp.zeros((64, M), BF16)
        eye = make_eye()

        for sec in range(3):
            chain_wait(sec)
            for c0 in range(w_cols[sec], w_cols[sec + 1], 128):
                wd = min(128, 3 * M - c0)
                wt = _dot(eye[0:wd, 0:wd], wqkv_s[:, c0:c0 + wd], NT)
                for j in range(NT_M):
                    wt_s[j, c0:c0 + wd, :] = wt[:, j * 128:(j + 1) * 128]
            for d in range(DHA):
                for j in range(NT_M):
                    rows = wt_s[j, pl.ds(sec * M + d, H, stride=DHA), :]
                    wj = min(128, M - j * 128)
                    p0 = _packed_row(sec, d)
                    wpt_s[p0:p0 + H, j * 128:j * 128 + wj] = rows[:, 0:wj].astype(BF16)
        copies["gate"].wait()
        for cp in chain[5:]:
            cp.start()

    def a_prep_rest(c):
        @pl.when(c == CB_AT)
        def _():
            copies["c"].start()
            for cp in group_copies(0):
                cp.start()

        @pl.when(c == WO_AT)
        def _():
            chain[3 + NXC].wait()
            a_prep_wo()

    def a_prep_wo():
        eye = make_eye()
        woa = woa_s[...].astype(F32)
        for j in range(NT_M):
            wj = min(128, M - j * 128)
            blk = woa[:, j * 128:j * 128 + wj]
            if wj < 128:
                blk = jnp.concatenate([blk, jnp.zeros((M, 128 - wj), F32)], axis=1)
            wof_s[j] = blk
        for d in range(DHA):
            for j in range(NT_M):
                wj = min(128, M - j * 128)
                rows = wof_s[j, pl.ds(d, H, stride=DHA), :]
                p0 = d * H if d < DF else d * H + 64
                woap_s[p0:p0 + H, j * 128:j * 128 + wj] = rows[:, 0:wj].astype(BF16)
        for j in range(NT_M):
            wj = min(128, M - j * 128)
            woapt_s[j * 128:j * 128 + wj, :] = _dot(
                eye[0:wj, 0:wj], woap_s[:, j * 128:j * 128 + wj], NT).astype(BF16)

    def a_xpose(t0, n):
        eye = make_eye()
        tiles = []
        for t in range(n // 128):
            tt = pl.multiple_of(t0 + t * 128, 128)
            xr = _dot(eye, xt_s[:, pl.ds(tt, 128)], NT).astype(BF16)
            x_s[pl.ds(tt, 128), :] = xr
            tiles.append(xr)
        gw = jnp.broadcast_to(gate_s[...].reshape(1, M), (16, M))
        g_s[:, pl.ds(t0, n)] = jax.nn.sigmoid(_dot(gw, xt_s[:, pl.ds(t0, n)]))
        return jnp.concatenate(tiles, axis=0)

    a_scale = (DHA ** -0.5) * LOG2E

    def a_proj(c, carry):
        a_prep_rest(c)
        r0 = pl.multiple_of(c * RAP, RAP)
        rk = pl.multiple_of(HALO + c * RAP, HALO)
        pltpu.make_async_copy(xt_hbm.at[:, pl.ds(r0, RAP)], xt_s.at[:, pl.ds(r0, RAP)], xsems.at[c]).wait()
        xq = a_xpose(r0, RAP)
        nf = DF * H
        def do_q():
            q = _dot(xq, wpt_s[0:nf, :], NT)
            for j in range(NT_M - 1):
                qa_s[j, pl.ds(r0, RAP), :] = q[:, j * 128:(j + 1) * 128]

        def do_k():
            k = _dot(xq, wpt_s[nf:2 * nf, :], NT) * a_scale
            for j in range(NT_M - 1):
                kl_s[j, pl.ds(rk, RAP), :] = k[:, j * 128:(j + 1) * 128]

        def do_v():
            v = _dot(xq, wpt_s[2 * nf:3 * nf, :], NT)
            for j in range(NT_M - 1):
                vl_s[j, pl.ds(rk, RAP), :] = v[:, j * 128:(j + 1) * 128]

        def do_t():
            t = _dot(xq, wpt_s[3 * nf:NPK * 128, :], NT)
            vl_s[NT_M - 1, pl.ds(rk, RAP), :] = t[:, 0:128]
            kl_s[NT_M - 1, pl.ds(rk, RAP), :] = t[:, 128:256] * a_scale

        for ch in A_SEQ:
            {"q": do_q, "k": do_k, "v": do_v, "t": do_t}[ch]()
        return carry

    def a_local(r0, sb, dz):
        qv = [qa_s.at[j, pl.ds(r0, RA), :] for j in range(NT_M - 1)]
        kv = [kl_s.at[j, pl.ds(r0, HALO + RA), :] for j in range(NT_M)]
        vv = [vl_s.at[j, pl.ds(r0, HALO + RA), :] for j in range(NT_M)]
        outs = []
        for b0 in range(sb * RS, (sb + 1) * RS, RG):
            qt = [qv[j][b0:b0 + RG, :] for j in range(NT_M - 1)]
            qt.append(vv[NT_M - 1][HALO + b0:HALO + b0 + RG, :])
            logits = []
            for w in range(WIN):
                off = HALO + b0 - w * DIL
                s = None
                for j in range(NT_M):
                    t = qt[j] * kv[j][off:off + RG, :]
                    s = t if s is None else s + t
                s = s + pltpu.roll(s, 64, 1)
                s = s + pltpu.roll(s, 32, 1)
                if b0 < w * DIL:
                    rowi = jax.lax.broadcasted_iota(jnp.int32, (RG, 128), 0) + (r0 + b0)
                    s = jnp.where(rowi >= w * DIL, s, NEG * LOG2E)
                logits.append(s)
            m = functools.reduce(jnp.maximum, logits)
            ps = [jnp.exp2(s - m) for s in logits]
            r = _recip(functools.reduce(jnp.add, ps))
            ot = []
            for j in range(NT_M):
                o = None
                for w in range(WIN):
                    off = HALO + b0 - w * DIL
                    t = ps[w] * vv[j][off:off + RG, :]
                    o = t if o is None else o + t
                ot.append(o * r)
            outs.append(ot)
        for j in range(NT_M):
            o = jnp.concatenate([ot[j] for ot in outs], axis=0)
            qc_s[HG + H + j + dz, pl.ds(pl.multiple_of(r0 + sb * RS, RS), RS), :] = o.astype(BF16)

    def a_main():
        jax.lax.fori_loop(0, S // RAP, a_proj, 0)

    def group_weights(raw, g):
        cols = []
        for b in range(HG // 2):
            u = raw[g * (HG // 2) + b]
            cols.append(pltpu.bitcast(u << 16, F32).astype(BF16))
            cols.append(pltpu.bitcast(u & jnp.uint32(0xFFFF0000), F32).astype(BF16))
        return jnp.concatenate(cols, axis=1)

    b_scale = (D ** -0.5) * LOG2E

    def group_body(g, carry):
        @pl.when(g > 0)
        def _():
            for cp in group_copies(g):
                cp.wait()

        def proj_body(rc, c2):
            r0 = pl.multiple_of(rc * RP, RP)
            ra = pl.multiple_of((g * (S // RP) + rc) * RA, RA)

            def proj(src, raw, dst, scale, part):
                n = RP // PSPLIT
                rows = pl.ds(pl.multiple_of(r0 + part * n, n), n)
                y = _dot(src[rows, :], group_weights(raw, g))
                if scale is not None:
                    y = y * scale
                for i in range(HG):
                    dst[i, rows, :] = y[:, i * D:(i + 1) * D].astype(BF16)

            count = {"q": 0, "k": 0, "v": 0}
            for ch in PROJ_SEQ:
                if ch in count:
                    src, raw, dst, scale = {"q": (x_s, wq_raw, qc_s, b_scale), "k": (c_s, wuk_raw, k_s, None),
                                            "v": (c_s, wuv_raw, v_s, None)}[ch]
                    proj(src, raw, dst, scale, count[ch])
                    count[ch] += 1
                else:
                    a_local(ra, int(ch, 36), jnp.minimum(g, 0) if DYNZ else 0)
            return c2

        with jax.named_scope("B_proj"):
            jax.lax.fori_loop(0, S // RP, proj_body, 0)

        def attn_body(it, c2):
            attn_heads(qc_s, k_s, v_s, g, it)
            return c2

        with jax.named_scope("B_attn"):
            jax.lax.fori_loop(0, HG // HU, attn_body, 0)
        return carry

    def out_copy(i):
        r0 = i * RO
        if not isinstance(i, int):
            r0 = pl.multiple_of(r0, RO)
        return pltpu.make_async_copy(out_s.at[:, pl.ds(r0, RO)], out_hbm.at[0, :, pl.ds(r0, RO)], osems.at[i])

    def out_body(i, carry):
        r0 = pl.multiple_of(i * RO, RO)

        def branch_b():
            ctx = jnp.concatenate([qc_s[HG + h, pl.ds(r0, RO), :] for h in range(H)], axis=1)
            wo = jnp.concatenate([wob_s[h] for h in range(H)], axis=1)
            return _dot(wo, ctx, NT)

        def branch_a():
            oa = jnp.concatenate([qc_s[HG + H + j, pl.ds(r0, RO), :] for j in range(NT_M)], axis=1)
            return _dot(woapt_s[...], oa, NT)

        gt = g_s[0:1, pl.ds(r0, RO)]
        if OUT_ORDER == 0:
            bt = branch_b()
            at = branch_a()
        else:
            at = branch_a() * gt
            bt = branch_b()
        if OUT_ORDER == 0:
            out = gt * at + (1.0 - gt) * bt
        else:
            out = at + (1.0 - gt) * bt
        out_s[:, pl.ds(r0, RO)] = out.astype(BF16)
        out_copy(i).start()
        return carry

    with jax.named_scope("A_prep"):
        a_prep()
    with jax.named_scope("A_main"):
        a_main()
        copies["c"].wait()
        for cp in group_copies(0):
            cp.wait()
        for g in range(1, NG):
            for cp in group_copies(g):
                cp.start()
        copies["wob"].start()
    jax.lax.fori_loop(0, NG, group_body, 0)
    with jax.named_scope("B_out"):
        copies["wob"].wait()
        jax.lax.fori_loop(0, S // RO, out_body, 0)
        for i in range(S // RO):
            out_copy(i).wait()


@jax.jit
def pallas_gated_mix__sliding_local_dilated__compressed_kv_cla__prompt_kernel(
    A_x: jax.Array,
    A_wqkv: jax.Array,
    A_wo: jax.Array,
    B_x: jax.Array,
    B_c_kv: jax.Array,
    B_w_q: jax.Array,
    B_w_uk: jax.Array,
    B_w_uv: jax.Array,
    B_w_o: jax.Array,
    gate_w: jax.Array,
):
    del B_x
    xt = jnp.swapaxes(A_x, 1, 2).reshape(M, S)
    c = B_c_kv.reshape(S, DC)
    wob = jnp.swapaxes(B_w_o, 1, 2)

    any_spec = pl.BlockSpec(memory_space=pl.ANY)
    scratch = [
        pltpu.VMEM((M, S), BF16),
        pltpu.VMEM((S, M), BF16),
        pltpu.VMEM((MP, 3 * M), BF16),
        pltpu.VMEM((M, M), BF16),
        pltpu.VMEM((S, DC), BF16),
        pltpu.VMEM((NPAIR, M, D), jnp.uint32),
        pltpu.VMEM((NPAIR, DC, D), jnp.uint32),
        pltpu.VMEM((NPAIR, DC, D), jnp.uint32),
        pltpu.VMEM((H, M, D), BF16),
        pltpu.VMEM((M,), BF16),
        pltpu.VMEM((NT_M, 14 * 128, 128), F32),
        pltpu.VMEM((NPK * 128, M), BF16),
        pltpu.VMEM((NT_M, M, 128), F32),
        pltpu.VMEM((MP, M), BF16),
        pltpu.VMEM((M, MP), BF16),
        pltpu.VMEM((NT_M - 1, S, 128), F32),
        pltpu.VMEM((NT_M, HALO + S, 128), F32),
        pltpu.VMEM((NT_M, HALO + S, 128), F32),
        pltpu.VMEM((16, S), F32),
        pltpu.VMEM((HG + H + NT_M, S, D), BF16),
        pltpu.VMEM((HG, S, D), BF16),
        pltpu.VMEM((HG, S, D), BF16),
        pltpu.VMEM((M, S), BF16),
        pltpu.SemaphoreType.DMA((6,)),
        pltpu.SemaphoreType.DMA((NXC + 3,)),
        pltpu.SemaphoreType.DMA((3 * NPAIR,)),
        pltpu.SemaphoreType.DMA((S // RO,)),
    ]
    out_t = pl.pallas_call(
        _kernel,
        out_shape=jax.ShapeDtypeStruct((1, M, S), BF16),
        in_specs=[any_spec] * 9,
        out_specs=any_spec,
        scratch_shapes=scratch,
        compiler_params=pltpu.CompilerParams(vmem_limit_bytes=120 * 1024 * 1024),
        name="gated_mix",
    )(xt, A_wqkv, A_wo, c, B_w_q, B_w_uk, B_w_uv, wob, gate_w)
    return jnp.swapaxes(out_t, 1, 2)
```

```python
import functools
import math

import jax
import jax.numpy as jnp
import jax.experimental.pallas as pl
import jax.experimental.pallas.tpu as pltpu

F32 = jnp.float32
BF16 = jnp.bfloat16

S = 2048
M = 576
MP = 640
NT_M = MP // 128
H = 32
D = 128
DC = 512
DHA = 18
WIN = 8
DIL = 2
HALO = 16
DF = 16
NPK = 14
LOG2E = math.log2(math.e)
NEG = -1e9

RAP = 512
RA = 256
RG = 8
RS = 32
HG = 8
NG = H // HG
RP = 1024
TQ = 256
TB = 128
HU = 2
BLOCK_ORDER = ((1, 3, 7, 6, 5, 4, 2, 0), (6, 7, 4, 5, 2, 3, 1, 0))
assert all(sorted(o) == list(range(S // TQ)) for o in BLOCK_ORDER) and len(BLOCK_ORDER) == HU
OUT_ORDER = 0
PSPLIT = 1
DYNZ = 0
PROJ_SEQ = "01v234q56k7"
LAG = 1
RO = 256
assert NG * (S // RP) == S // RA
NXC = 4
FILL_R = (1, 3, 7, 6, 5, 4, 2, 0)
FILL_AT = (14, 14, 14, 14, 16, 16, 16, 16)
FILL_POS = 0
assert HU == 2 and sorted(FILL_R) == list(range(S // TQ))
assert all(BLOCK_ORDER[0].index(r) + 1 + LAG <= a <= 16 for r, a in zip(FILL_R, FILL_AT))
A_SEQ = "qkvt"
CB_AT = 1
WO_AT = 2
assert S // NXC == RAP
NSPLIT = 1
NPAIR = H // 2

NN = (((1,), (0,)), ((), ()))
NT = (((1,), (1,)), ((), ()))


def _dot(a, b, dims=NN):
    return jax.lax.dot_general(a, b, dims, preferred_element_type=F32)


def _packed_row(sec, d):
    if d < DF:
        return (sec * DF + d) * H
    return 3 * DF * H + ((0, 4, 2)[sec] + d - DF) * H


def _lane_partial(s, op):
    acc = s[:, 0:128]
    for j in range(1, s.shape[1] // 128):
        acc = op(acc, s[:, j * 128:(j + 1) * 128])
    return acc


def _recip(l):
    r = pl.reciprocal(l, approx=True)
    return r * (2.0 - l * r)


def _segments(r0):
    nsub = TQ // TB
    segs = []
    if r0 > 0:
        segs.append((0, TQ, 0, r0, False))
    for j in range(nsub):
        segs.append((j * TB, (j + 1) * TB, r0 + j * TB, r0 + (j + 1) * TB, True))
        if (j + 1) * TB < TQ:
            segs.append(((j + 1) * TB, TQ, r0 + j * TB, r0 + (j + 1) * TB, False))
    return segs


def _attn_scores(q_ref, k_ref, r0, tri):
    nsub = TQ // TB
    segs = _segments(r0)
    ss = []
    for (a, b, c, d, msk) in segs:
        s = _dot(q_ref[r0 + a:r0 + b, :], k_ref[c:d, :], NT)
        if msk:
            s = jnp.where(tri, s, NEG * LOG2E)
        ss.append(s)
    ms = []
    for i in range(nsub):
        m = None
        for (a, b, c, d, msk), s in zip(segs, ss):
            if a <= i * TB and (i + 1) * TB <= b:
                sm = _lane_partial(s[i * TB - a:(i + 1) * TB - a], jnp.maximum)
                m = sm if m is None else jnp.maximum(m, sm)
        ms.append(jnp.max(m, axis=1, keepdims=True))
    return ss, ms


def _attn_values(v_ref, r0, ss, ms):
    nsub = TQ // TB
    segs = _segments(r0)
    ls = [None] * nsub
    os_ = [None] * nsub
    for (a, b, c, d, msk), s in zip(segs, ss):
        m = jnp.concatenate(ms[a // TB:b // TB], axis=0) if b - a > TB else ms[a // TB]
        p = jnp.exp2(s - m)
        l = _lane_partial(p, jnp.add)
        o = _dot(p.astype(BF16), v_ref[c:d, :])
        for i in range(a // TB, b // TB):
            li = l[i * TB - a:(i + 1) * TB - a]
            oi = o[i * TB - a:(i + 1) * TB - a]
            ls[i] = li if ls[i] is None else ls[i] + li
            os_[i] = oi if os_[i] is None else os_[i] + oi
    return [o * _recip(jnp.sum(l, axis=1, keepdims=True)) for o, l in zip(os_, ls)]


def attn_heads(qc_s, k_s, v_s, wob_s, acc_s, g, it):
    row = jax.lax.broadcasted_iota(jnp.int32, (TB, TB), 0)
    col = jax.lax.broadcasted_iota(jnp.int32, (TB, TB), 1)
    tri = col <= row
    items = [(u, r) for u in range(HU) for r in BLOCK_ORDER[u]]
    pend = {}
    done = {}

    def store(item):
        u, r = item
        for j, o in enumerate(done.pop(item)):
            r0 = r * TQ + j * TB
            qc_s[HG + g * HG + it * HU + u, r0:r0 + TB, :] = o.astype(BF16)

    def fill(r):
        h0 = g * HG + it * HU
        ctx = qc_s[HG + h0, r * TQ:(r + 1) * TQ, :]
        acc_s[:, r * TQ:(r + 1) * TQ] = acc_s[:, r * TQ:(r + 1) * TQ] + _dot(wob_s[h0], ctx, NT)

    def fills(t):
        for r, at in zip(FILL_R, FILL_AT):
            if at == t:
                fill(r)

    for t in range(len(items) + 1):
        if t < len(items):
            u, r = items[t]
            hh = it * HU + u
            pend[items[t]] = _attn_scores(qc_s.at[hh], k_s.at[hh], r * TQ, tri)
        if t >= 1 + LAG:
            store(items[t - 1 - LAG])
        if t >= 1:
            u, r = items[t - 1]
            hh = it * HU + u
            if FILL_POS == 0:
                fills(t)
            done[items[t - 1]] = _attn_values(v_s.at[hh], r * TQ, *pend.pop(items[t - 1]))
            if FILL_POS == 1:
                fills(t)
    for item in list(done):
        store(item)


def _kernel(xt_hbm, wqkv_hbm, woa_hbm, c_hbm, wq_hbm, wuk_hbm, wuv_hbm, wob_hbm, gate_hbm,
            out_hbm,
            xt_s, x_s, wqkv_s, woa_s, c_s, wq_raw, wuk_raw, wuv_raw, wob_s, gate_s,
            wt_s, wpt_s, wof_s, woap_s, woapt_s, qa_s, kl_s, vl_s, g_s,
            qc_s, k_s, v_s, out_s, acc_s, sems, xsems, wsems, osems):
    copies = {
        "gate": pltpu.make_async_copy(gate_hbm, gate_s, sems.at[2]),
        "woa": pltpu.make_async_copy(woa_hbm, woa_s, sems.at[3]),
        "c": pltpu.make_async_copy(c_hbm, c_s, sems.at[4]),
        "wob": pltpu.make_async_copy(wob_hbm, wob_s, sems.at[5]),
    }
    w_cols = (0, 5 * 128, 9 * 128, 3 * M)
    w_copies = [pltpu.make_async_copy(wqkv_hbm.at[:, pl.ds(w_cols[i], w_cols[i + 1] - w_cols[i])],
                                      wqkv_s.at[pl.ds(0, M), pl.ds(w_cols[i], w_cols[i + 1] - w_cols[i])],
                                      xsems.at[NXC + i]) for i in range(3)]
    xw = S // NXC
    x_copies = [pltpu.make_async_copy(xt_hbm.at[:, pl.ds(i * xw, xw)], xt_s.at[:, pl.ds(i * xw, xw)], xsems.at[i])
                for i in range(NXC)]
    def pair_copies(wi, j):
        w_hbm, raw = ((wq_hbm, wq_raw), (wuk_hbm, wuk_raw), (wuv_hbm, wuv_raw))[wi]
        n = w_hbm.shape[0] // NSPLIT
        return [pltpu.make_async_copy(
            w_hbm.bitcast(jnp.uint32).at[pl.ds(p * n, n), j, :], raw.at[j, pl.ds(p * n, n), :],
            wsems.at[wi * NPAIR + j]) for p in range(NSPLIT)]

    def group_copies(g):
        return [cp for b in range(HG // 2) for wi in range(3) for cp in pair_copies(wi, g * (HG // 2) + b)]

    chain = w_copies + x_copies + [copies["woa"]]
    copies["gate"].start()
    chain[0].start()
    chain[1].start()

    def chain_wait(i):
        chain[i].wait()
        chain[i + 2].start()

    def make_eye():
        return (jax.lax.broadcasted_iota(jnp.int32, (128, 128), 0)
                == jax.lax.broadcasted_iota(jnp.int32, (128, 128), 1)).astype(BF16)

    def a_prep():
        wqkv_s[M:MP, :] = jnp.zeros((MP - M, 3 * M), BF16)
        zero_halo = jnp.zeros((HALO, 128), F32)
        for j in range(NT_M):
            kl_s[j, 0:HALO, :] = zero_halo
            vl_s[j, 0:HALO, :] = zero_halo
        wpt_s[3 * M:NPK * 128, :] = jnp.zeros((NPK * 128 - 3 * M, M), BF16)
        woap_s[DF * H:DF * H + 64, :] = jnp.zeros((64, M), BF16)
        acc_s[...] = jnp.zeros((M, S), F32)
        eye = make_eye()

        for sec in range(3):
            chain_wait(sec)
            for c0 in range(w_cols[sec], w_cols[sec + 1], 128):
                wd = min(128, 3 * M - c0)
                wt = _dot(eye[0:wd, 0:wd], wqkv_s[:, c0:c0 + wd], NT)
                for j in range(NT_M):
                    wt_s[j, c0:c0 + wd, :] = wt[:, j * 128:(j + 1) * 128]
            for d in range(DHA):
                for j in range(NT_M):
                    rows = wt_s[j, pl.ds(sec * M + d, H, stride=DHA), :]
                    wj = min(128, M - j * 128)
                    p0 = _packed_row(sec, d)
                    wpt_s[p0:p0 + H, j * 128:j * 128 + wj] = rows[:, 0:wj].astype(BF16)
        copies["gate"].wait()
        for cp in chain[5:]:
            cp.start()

    def a_prep_rest(c):
        @pl.when(c == CB_AT)
        def _():
            copies["c"].start()
            for cp in group_copies(0):
                cp.start()
            copies["wob"].start()

        @pl.when(c == WO_AT)
        def _():
            chain[3 + NXC].wait()
            a_prep_wo()

    def a_prep_wo():
        eye = make_eye()
        woa = woa_s[...].astype(F32)
        for j in range(NT_M):
            wj = min(128, M - j * 128)
            blk = woa[:, j * 128:j * 128 + wj]
            if wj < 128:
                blk = jnp.concatenate([blk, jnp.zeros((M, 128 - wj), F32)], axis=1)
            wof_s[j] = blk
        for d in range(DHA):
            for j in range(NT_M):
                wj = min(128, M - j * 128)
                rows = wof_s[j, pl.ds(d, H, stride=DHA), :]
                p0 = d * H if d < DF else d * H + 64
                woap_s[p0:p0 + H, j * 128:j * 128 + wj] = rows[:, 0:wj].astype(BF16)
        for j in range(NT_M):
            wj = min(128, M - j * 128)
            woapt_s[j * 128:j * 128 + wj, :] = _dot(
                eye[0:wj, 0:wj], woap_s[:, j * 128:j * 128 + wj], NT).astype(BF16)

    def a_xpose(t0, n):
        eye = make_eye()
        tiles = []
        for t in range(n // 128):
            tt = pl.multiple_of(t0 + t * 128, 128)
            xr = _dot(eye, xt_s[:, pl.ds(tt, 128)], NT).astype(BF16)
            x_s[pl.ds(tt, 128), :] = xr
            tiles.append(xr)
        gw = jnp.broadcast_to(gate_s[...].reshape(1, M), (16, M))
        g_s[:, pl.ds(t0, n)] = jax.nn.sigmoid(_dot(gw, xt_s[:, pl.ds(t0, n)]))
        return jnp.concatenate(tiles, axis=0)

    a_scale = (DHA ** -0.5) * LOG2E

    def a_proj(c, carry):
        a_prep_rest(c)
        r0 = pl.multiple_of(c * RAP, RAP)
        rk = pl.multiple_of(HALO + c * RAP, HALO)
        pltpu.make_async_copy(xt_hbm.at[:, pl.ds(r0, RAP)], xt_s.at[:, pl.ds(r0, RAP)], xsems.at[c]).wait()
        xq = a_xpose(r0, RAP)
        nf = DF * H
        def do_q():
            q = _dot(xq, wpt_s[0:nf, :], NT)
            for j in range(NT_M - 1):
                qa_s[j, pl.ds(r0, RAP), :] = q[:, j * 128:(j + 1) * 128]

        def do_k():
            k = _dot(xq, wpt_s[nf:2 * nf, :], NT) * a_scale
            for j in range(NT_M - 1):
                kl_s[j, pl.ds(rk, RAP), :] = k[:, j * 128:(j + 1) * 128]

        def do_v():
            v = _dot(xq, wpt_s[2 * nf:3 * nf, :], NT)
            for j in range(NT_M - 1):
                vl_s[j, pl.ds(rk, RAP), :] = v[:, j * 128:(j + 1) * 128]

        def do_t():
            t = _dot(xq, wpt_s[3 * nf:NPK * 128, :], NT)
            vl_s[NT_M - 1, pl.ds(rk, RAP), :] = t[:, 0:128]
            kl_s[NT_M - 1, pl.ds(rk, RAP), :] = t[:, 128:256] * a_scale

        for ch in A_SEQ:
            {"q": do_q, "k": do_k, "v": do_v, "t": do_t}[ch]()
        return carry

    def a_local(r0, sb, dz):
        qv = [qa_s.at[j, pl.ds(r0, RA), :] for j in range(NT_M - 1)]
        kv = [kl_s.at[j, pl.ds(r0, HALO + RA), :] for j in range(NT_M)]
        vv = [vl_s.at[j, pl.ds(r0, HALO + RA), :] for j in range(NT_M)]
        outs = []
        for b0 in range(sb * RS, (sb + 1) * RS, RG):
            qt = [qv[j][b0:b0 + RG, :] for j in range(NT_M - 1)]
            qt.append(vv[NT_M - 1][HALO + b0:HALO + b0 + RG, :])
            logits = []
            for w in range(WIN):
                off = HALO + b0 - w * DIL
                s = None
                for j in range(NT_M):
                    t = qt[j] * kv[j][off:off + RG, :]
                    s = t if s is None else s + t
                s = s + pltpu.roll(s, 64, 1)
                s = s + pltpu.roll(s, 32, 1)
                if b0 < w * DIL:
                    rowi = jax.lax.broadcasted_iota(jnp.int32, (RG, 128), 0) + (r0 + b0)
                    s = jnp.where(rowi >= w * DIL, s, NEG * LOG2E)
                logits.append(s)
            m = functools.reduce(jnp.maximum, logits)
            ps = [jnp.exp2(s - m) for s in logits]
            r = _recip(functools.reduce(jnp.add, ps))
            ot = []
            for j in range(NT_M):
                o = None
                for w in range(WIN):
                    off = HALO + b0 - w * DIL
                    t = ps[w] * vv[j][off:off + RG, :]
                    o = t if o is None else o + t
                ot.append(o * r)
            outs.append(ot)
        for j in range(NT_M):
            o = jnp.concatenate([ot[j] for ot in outs], axis=0)
            qc_s[HG + H + j + dz, pl.ds(pl.multiple_of(r0 + sb * RS, RS), RS), :] = o.astype(BF16)

    def a_main():
        jax.lax.fori_loop(0, S // RAP, a_proj, 0)

    def group_weights(raw, g):
        cols = []
        for b in range(HG // 2):
            u = raw[g * (HG // 2) + b]
            cols.append(pltpu.bitcast(u << 16, F32).astype(BF16))
            cols.append(pltpu.bitcast(u & jnp.uint32(0xFFFF0000), F32).astype(BF16))
        return jnp.concatenate(cols, axis=1)

    b_scale = (D ** -0.5) * LOG2E

    def group_body(g, carry):
        @pl.when(g > 0)
        def _():
            for cp in group_copies(g):
                cp.wait()

        def proj_body(rc, c2):
            r0 = pl.multiple_of(rc * RP, RP)
            ra = pl.multiple_of((g * (S // RP) + rc) * RA, RA)

            def proj(src, raw, dst, scale, part):
                n = RP // PSPLIT
                rows = pl.ds(pl.multiple_of(r0 + part * n, n), n)
                y = _dot(src[rows, :], group_weights(raw, g))
                if scale is not None:
                    y = y * scale
                for i in range(HG):
                    dst[i, rows, :] = y[:, i * D:(i + 1) * D].astype(BF16)

            count = {"q": 0, "k": 0, "v": 0}
            for ch in PROJ_SEQ:
                if ch in count:
                    src, raw, dst, scale = {"q": (x_s, wq_raw, qc_s, b_scale), "k": (c_s, wuk_raw, k_s, None),
                                            "v": (c_s, wuv_raw, v_s, None)}[ch]
                    proj(src, raw, dst, scale, count[ch])
                    count[ch] += 1
                else:
                    a_local(ra, int(ch, 36), jnp.minimum(g, 0) if DYNZ else 0)
            return c2

        with jax.named_scope("B_proj"):
            jax.lax.fori_loop(0, S // RP, proj_body, 0)

        def attn_body(it, c2):
            attn_heads(qc_s, k_s, v_s, wob_s, acc_s, g, it)
            return c2

        with jax.named_scope("B_attn"):
            jax.lax.fori_loop(0, HG // HU, attn_body, 0)
        return carry

    def out_copy(i):
        r0 = i * RO
        if not isinstance(i, int):
            r0 = pl.multiple_of(r0, RO)
        return pltpu.make_async_copy(out_s.at[:, pl.ds(r0, RO)], out_hbm.at[0, :, pl.ds(r0, RO)], osems.at[i])

    def out_body(i, carry):
        r0 = pl.multiple_of(i * RO, RO)

        def branch_b():
            ctx = jnp.concatenate([qc_s[HG + h, pl.ds(r0, RO), :] for h in range(1, H, HU)], axis=1)
            wo = jnp.concatenate([wob_s[h] for h in range(1, H, HU)], axis=1)
            return _dot(wo, ctx, NT) + acc_s[:, pl.ds(r0, RO)]

        def branch_a():
            oa = jnp.concatenate([qc_s[HG + H + j, pl.ds(r0, RO), :] for j in range(NT_M)], axis=1)
            return _dot(woapt_s[...], oa, NT)

        gt = g_s[0:1, pl.ds(r0, RO)]
        if OUT_ORDER == 0:
            bt = branch_b()
            at = branch_a()
        else:
            at = branch_a() * gt
            bt = branch_b()
        if OUT_ORDER == 0:
            out = gt * at + (1.0 - gt) * bt
        else:
            out = at + (1.0 - gt) * bt
        out_s[:, pl.ds(r0, RO)] = out.astype(BF16)
        out_copy(i).start()
        return carry

    with jax.named_scope("A_prep"):
        a_prep()
    with jax.named_scope("A_main"):
        a_main()
        copies["c"].wait()
        for cp in group_copies(0):
            cp.wait()
        copies["wob"].wait()
        for g in range(1, NG):
            for cp in group_copies(g):
                cp.start()
    jax.lax.fori_loop(0, NG, group_body, 0)
    with jax.named_scope("B_out"):
        jax.lax.fori_loop(0, S // RO, out_body, 0)
        for i in range(S // RO):
            out_copy(i).wait()


@jax.jit
def pallas_gated_mix__sliding_local_dilated__compressed_kv_cla__prompt_kernel(
    A_x: jax.Array,
    A_wqkv: jax.Array,
    A_wo: jax.Array,
    B_x: jax.Array,
    B_c_kv: jax.Array,
    B_w_q: jax.Array,
    B_w_uk: jax.Array,
    B_w_uv: jax.Array,
    B_w_o: jax.Array,
    gate_w: jax.Array,
):
    del B_x
    xt = jnp.swapaxes(A_x, 1, 2).reshape(M, S)
    c = B_c_kv.reshape(S, DC)
    wob = jnp.swapaxes(B_w_o, 1, 2)

    any_spec = pl.BlockSpec(memory_space=pl.ANY)
    scratch = [
        pltpu.VMEM((M, S), BF16),
        pltpu.VMEM((S, M), BF16),
        pltpu.VMEM((MP, 3 * M), BF16),
        pltpu.VMEM((M, M), BF16),
        pltpu.VMEM((S, DC), BF16),
        pltpu.VMEM((NPAIR, M, D), jnp.uint32),
        pltpu.VMEM((NPAIR, DC, D), jnp.uint32),
        pltpu.VMEM((NPAIR, DC, D), jnp.uint32),
        pltpu.VMEM((H, M, D), BF16),
        pltpu.VMEM((M,), BF16),
        pltpu.VMEM((NT_M, 14 * 128, 128), F32),
        pltpu.VMEM((NPK * 128, M), BF16),
        pltpu.VMEM((NT_M, M, 128), F32),
        pltpu.VMEM((MP, M), BF16),
        pltpu.VMEM((M, MP), BF16),
        pltpu.VMEM((NT_M - 1, S, 128), F32),
        pltpu.VMEM((NT_M, HALO + S, 128), F32),
        pltpu.VMEM((NT_M, HALO + S, 128), F32),
        pltpu.VMEM((16, S), F32),
        pltpu.VMEM((HG + H + NT_M, S, D), BF16),
        pltpu.VMEM((HG, S, D), BF16),
        pltpu.VMEM((HG, S, D), BF16),
        pltpu.VMEM((M, S), BF16),
        pltpu.VMEM((M, S), F32),
        pltpu.SemaphoreType.DMA((6,)),
        pltpu.SemaphoreType.DMA((NXC + 3,)),
        pltpu.SemaphoreType.DMA((3 * NPAIR,)),
        pltpu.SemaphoreType.DMA((S // RO,)),
    ]
    out_t = pl.pallas_call(
        _kernel,
        out_shape=jax.ShapeDtypeStruct((1, M, S), BF16),
        in_specs=[any_spec] * 9,
        out_specs=any_spec,
        scratch_shapes=scratch,
        compiler_params=pltpu.CompilerParams(vmem_limit_bytes=120 * 1024 * 1024),
        name="gated_mix",
    )(xt, A_wqkv, A_wo, c, B_w_q, B_w_uk, B_w_uv, wob, gate_w)
    return jnp.swapaxes(out_t, 1, 2)
```
